```python
import jax
import jax.numpy as jnp

def _softmax(x, axis=-1):
    return jax.nn.softmax(x, axis=axis)

def _gelu(x):
    return jax.nn.gelu(x, approximate=True)

def _silu(x):
    return jax.nn.silu(x)

def _sigmoid(x):
    return jax.nn.sigmoid(x)

def _layernorm(x, axis=-1, eps=1e-05):
    m = jnp.mean(x, axis=axis, keepdims=True)
    v = jnp.var(x, axis=axis, keepdims=True)
    return (x - m) / jnp.sqrt(v + eps)

def _scatter_add(tgt, idx, src, axis=0):
    return tgt.at[idx].add(src)

def _segment_sum(src, seg, n):
    return jax.ops.segment_sum(src, seg, n)

class _Rng:

    def __init__(self, key):
        self._k = key

    def _next(self):
        self._k, sub = jax.random.split(self._k)
        return sub

    def normal(self, shape):
        return jax.random.normal(self._next(), shape, dtype=jnp.bfloat16)

    def randint(self, lo, hi, shape):
        return jax.random.randint(self._next(), shape, lo, hi, dtype=jnp.int32)

    def uniform(self, shape, lo=0.0, hi=1.0):
        return jax.random.uniform(self._next(), shape, jnp.bfloat16, lo, hi)

    def permutation(self, n):
        return jax.random.permutation(self._next(), n)
kernel_name = 'gated_mix__ssm_conv_h3__memory_aug_recurrent_mem_tr__prompt'

def setup_inputs():
    _rng = _Rng(jax.random.key(int.from_bytes(__import__("os").urandom(4), "little")))
    _w = lambda a: (lambda t: t.astype(jnp.bfloat16) if jnp.issubdtype(t.dtype, jnp.floating) else t)(jnp.asarray(a))

    def _A_setup():
        B, S, D = (1, 2048, 1024)
        ks = 4
        return {'q': _w((lambda *s: _rng.normal(s) * 0.05)(B, S, D)), 'k': _w((lambda *s: _rng.normal(s) * 0.05)(B, S, D)), 'v': _w((lambda *s: _rng.normal(s) * 0.05)(B, S, D)), 'shift_k': _w((lambda *s: _rng.normal(s) * 0.05)(D, ks) * 0.5), 'ssm_k': _w((lambda *s: _rng.normal(s) * 0.05)(D, S) * (1.0 / S ** 0.5)), 'ssm_D': _w((lambda *s: _rng.normal(s) * 0.05)(D))}
    _A_in = _A_setup()

    def _B_setup():
        B, S, Dm = (1, 2048, 1024)
        H, Dh = (32, 128)
        M, seg = (8, 32)
        seg = min(seg, S)
        S = S // seg * seg
        return {'x': _w((lambda *s: _rng.normal(s) * 0.05)(B, S, Dm)), 'mem0': _w((lambda *s: _rng.normal(s) * 0.05)(B, M, Dm)), 'Wq': _w((lambda *s: _rng.normal(s) * 0.05)(Dm, H, Dh) * Dm ** (-0.5)), 'Wk': _w((lambda *s: _rng.normal(s) * 0.05)(Dm, H, Dh) * Dm ** (-0.5)), 'Wv': _w((lambda *s: _rng.normal(s) * 0.05)(Dm, H, Dh) * Dm ** (-0.5)), 'Wo': _w((lambda *s: _rng.normal(s) * 0.05)(H, Dh, Dm) * (H * Dh) ** (-0.5)), 'seg_len': seg}
    _B_in = _B_setup()
    return {'A_q': _A_in['q'], 'A_k': _A_in['k'], 'A_v': _A_in['v'], 'A_shift_k': _A_in['shift_k'], 'A_ssm_k': _A_in['ssm_k'], 'A_ssm_D': _A_in['ssm_D'], 'B_x': _B_in['x'], 'B_mem0': _B_in['mem0'], 'B_Wq': _B_in['Wq'], 'B_Wk': _B_in['Wk'], 'B_Wv': _B_in['Wv'], 'B_Wo': _B_in['Wo'], 'B_seg_len': _B_in['seg_len'], 'gate_w': _w((lambda *s: _rng.normal(s) * 0.05)(1024))}

def reference(A_q, A_k, A_v, A_shift_k, A_ssm_k, A_ssm_D, B_x, B_mem0, B_Wq, B_Wk, B_Wv, B_Wo, B_seg_len, gate_w):

    def _A_ref(q, k, v, shift_k, ssm_k, ssm_D):
        B, S, D = q.shape
        ks = shift_k.shape[-1]
        k_pad = jnp.pad(k, ((0, 0), (ks - 1, 0), (0, 0)))
        k_shift = jnp.zeros_like(k)
        for t in range(ks):
            k_shift = k_shift + k_pad[:, t:t + S, :] * shift_k[:, ks - 1 - t][None, None, :]
        kv = k_shift * v
        L = 2 * S
        kv_pad = jnp.pad(kv, ((0, 0), (0, S), (0, 0)))
        kf_pad = jnp.pad(ssm_k, ((0, 0), (0, S)))
        kv_f = (lambda x, axes=(-2, -1): jnp.fft.rfft2(x.astype(jnp.float32), axes=axes))(kv_pad[:, None, :, :], axes=(1, 2))
        kf_f = (lambda x, axes=(-2, -1): jnp.fft.rfft2(x.astype(jnp.float32), axes=axes))(kf_pad[:, None, :], axes=(1, 2))
        kf_f = (lambda x, *d: x.transpose(*d))(kf_f, 1, 2, 0)
        y_f = kv_f * kf_f[None, :, :, :]
        y = (lambda x, s, axes=(-2, -1): jnp.fft.irfft2(x, s=s, axes=axes).astype(jnp.bfloat16))(y_f, (1, L), axes=(1, 2))[:, 0, :S, :]
        y = y + kv * ssm_D[None, None, :]
        return q * y

    def _B_ref(x, mem0, Wq, Wk, Wv, Wo, seg_len):
        B, S, Dm = x.shape
        H, Dh = (Wq.shape[1], Wq.shape[2])
        M = mem0.shape[1]
        scale = Dh ** (-0.5)
        n_seg = S // seg_len
        L = M + seg_len
        idx = jnp.arange(L)
        mask = (idx[:, None] < M) | (idx[:, None] >= idx[None, :])
        mem = mem0
        outs = []
        for s in range(n_seg):
            xs = x[:, s * seg_len:(s + 1) * seg_len, :].copy()
            h = jnp.concatenate([mem, xs], axis=1)
            q = jnp.einsum('btd,dhe->bhte', h, Wq)
            k = jnp.einsum('btd,dhe->bhte', h, Wk)
            v = jnp.einsum('btd,dhe->bhte', h, Wv)
            scores = jnp.einsum('bhqe,bhke->bhqk', q, k) * scale
            scores = jnp.where(mask[None, None], scores, -1000000000.0)
            p = _softmax(scores, axis=-1)
            o = jnp.einsum('bhqk,bhke->bhqe', p, v)
            o = jnp.einsum('bhte,hed->btd', o, Wo)
            mem = o[:, :M, :].copy()
            outs.append(o[:, M:, :])
        return jnp.concatenate(outs, axis=1)
    x = A_q
    g = _sigmoid((x * gate_w).sum(-1, keepdims=True))
    a = _A_ref(x, A_k, A_v, A_shift_k, A_ssm_k, A_ssm_D)
    b = _B_ref(x, B_mem0, B_Wq, B_Wk, B_Wv, B_Wo, B_seg_len)
    return g * a + (1 - g) * b
```

```python
import functools

import jax
import jax.numpy as jnp
import numpy as np
import jax.experimental.pallas as pl
import jax.experimental.pallas.tpu as pltpu

F32 = jnp.float32
BF16 = jnp.bfloat16

S = 2048
D = 1024
NC = D // 128
H = 32
DH = 128
MEM = 8
SEG = 32
NSEG = S // SEG
XR = 24
PRE = S - NSEG * XR
RING = PRE + SEG
CB = 128
NB = S // CB
KS = 4


def _dft_tables():
    f = np.concatenate([np.arange(0, CB, 2), np.arange(1, CB, 2)]).astype(np.float64)
    t = np.arange(CB, dtype=np.float64)
    ang = 2.0 * np.pi * (f[:, None] + 0.5) * t[None, :] / (2 * CB)
    fwd = np.concatenate([np.cos(ang), -np.sin(ang)], axis=0)
    inv = np.concatenate([np.cos(ang).T, -np.sin(ang).T], axis=1) / CB
    return fwd, inv


def _dot(a, b):
    return jnp.dot(a, b, preferred_element_type=F32)


def _dot_nt(a, b):
    return jax.lax.dot_general(a, b, (((1,), (1,)), ((), ())), preferred_element_type=F32)


def _kernel(x_hbm, k_hbm, v_hbm, ssm_hbm, wq_hbm, wk_hbm, wv_hbm, wo_hbm,
            shift_ref, dskip_ref, gate_ref, mem0_ref, fwd_ref, inv_ref,
            out_hbm,
            xs, ks, vs, ssm, wraw, stage, wqkv, wo, ring, obuf, olhs, bbuf, abuf,
            kf, kvb, uspec, kspec, zspec, outbuf, mem,
            sem_x, sem_k, sem_v, sem_s, sem_w, sem_o, sem_out):
    w_hbm = (wq_hbm, wk_hbm, wv_hbm)

    def slab_copy(src, dst, sem, c):
        return pltpu.make_async_copy(src.at[:, pl.ds(c * 128, 128)], dst.at[c], sem.at[c])

    def w_copy(c):
        t, g = divmod(c, 4)
        return pltpu.make_async_copy(w_hbm[t].at[:, pl.ds(g * 8, 8), :], wraw.at[c % 2], sem_w.at[c % 2])

    for c in range(NC):
        slab_copy(k_hbm, ks, sem_k, c).start()
        slab_copy(v_hbm, vs, sem_v, c).start()
        pltpu.make_async_copy(ssm_hbm.at[pl.ds(c * 128, 128), :], ssm.at[c], sem_s.at[c]).start()
        slab_copy(x_hbm, xs, sem_x, c).start()
    w_copy(0).start()
    w_copy(1).start()
    for c in range(NC):
        slab_copy(wo_hbm, wo, sem_o, c).start()

    kf[0:8, :] = jnp.zeros((8, 128), F32)
    for c in range(NC):
        slab_copy(k_hbm, ks, sem_k, c).wait()
        slab_copy(v_hbm, vs, sem_v, c).wait()
        pltpu.make_async_copy(ssm_hbm.at[pl.ds(c * 128, 128), :], ssm.at[c], sem_s.at[c]).wait()
        slab_copy(x_hbm, xs, sem_x, c).wait()

    def conv_tile(c, carry):
        shift = shift_ref[c].astype(F32)
        dsk = dskip_ref[pl.ds(c, 1), :]
        kf[8:8 + S, :] = ks[c].astype(F32)
        fwd = fwd_ref[...]
        for b in range(NB):
            r = b * CB
            acc = kf[8 + r:8 + r + CB, :] * shift[0:1, :]
            for l in range(1, KS):
                acc = acc + kf[8 + r - l:8 + r - l + CB, :] * shift[l:l + 1, :]
            kv = (acc * vs[c, r:r + CB, :].astype(F32)).astype(BF16)
            kvb[r:r + CB, :] = kv
            uspec[b] = _dot(fwd, kv)
        prev = None
        h = CB // 2
        for b in range(NB):
            kb = _dot_nt(fwd, ssm[c, :, b * CB:(b + 1) * CB])
            if prev is None:
                kspec[b] = kb
            else:
                kspec[b, 0:h] = kb[0:h] - prev[CB:CB + h]
                kspec[b, h:CB] = kb[h:CB] + prev[CB + h:2 * CB]
                kspec[b, CB:CB + h] = kb[CB:CB + h] + prev[0:h]
                kspec[b, CB + h:2 * CB] = kb[CB + h:2 * CB] - prev[h:CB]
            prev = kb

        def mac(fr, carry2):
            r = pl.multiple_of(fr * 16, 16)
            for i in range(NB):
                zr = None
                for j in range(i + 1):
                    ur = uspec[j, pl.ds(r, 16), :]
                    ui = uspec[j, pl.ds(CB + r, 16), :]
                    kr = kspec[i - j, pl.ds(r, 16), :]
                    ki = kspec[i - j, pl.ds(CB + r, 16), :]
                    tr = ur * kr - ui * ki
                    ti = ur * ki + ui * kr
                    if zr is None:
                        zr, zi = tr, ti
                    else:
                        zr, zi = zr + tr, zi + ti
                zspec[i, pl.ds(r, 16), :] = zr.astype(BF16)
                zspec[i, pl.ds(CB + r, 16), :] = zi.astype(BF16)
            return carry2
        jax.lax.fori_loop(0, CB // 16, mac, 0)

        inv = inv_ref[...]
        for b in range(NB):
            r = b * CB
            y = _dot(inv, zspec[b])
            y = y + kvb[r:r + CB, :].astype(F32) * dsk
            abuf[c, r:r + CB, :] = (xs[c, r:r + CB, :].astype(F32) * y).astype(BF16)
        return carry
    jax.lax.fori_loop(0, NC, conv_tile, 0)

    xpre = jnp.concatenate([xs[c, 0:PRE, :] for c in range(NC)], axis=1)
    for c in range(12):
        w_copy(c).wait()
        for db in range(D // 128):
            blk = wraw[c % 2, db * 128:(db + 1) * 128]
            stage[...] = blk.astype(F32).reshape(128 * 8, 128)
            for j in range(8):
                wqkv[c * 8 + j, db * 128:(db + 1) * 128, :] = stage[pl.ds(j, 128, stride=8), :].astype(BF16)
        if c + 2 < 12:
            w_copy(c + 2).start()
        for j in range(8):
            ring[c * 8 + j, 0:PRE, :] = _dot(xpre, wqkv[c * 8 + j]).astype(BF16)

    for c in range(NC):
        slab_copy(wo_hbm, wo, sem_o, c).wait()

    mem[...] = mem0_ref[...].astype(F32)
    scale = float(DH) ** -0.5
    NR = 2 * (SEG + MEM)

    def step(s, carry):
        ri = jax.lax.broadcasted_iota(jnp.int32, (NR, NR), 0)
        ci = jax.lax.broadcasted_iota(jnp.int32, (NR, NR), 1)
        r_mem = ri >= 2 * SEG
        c_mem = ci >= 2 * SEG
        r_head = jnp.where(r_mem, (ri - 2 * SEG) // MEM, ri // SEG)
        c_head = jnp.where(c_mem, (ci - 2 * SEG) // MEM, ci // SEG)
        same = r_head == c_head
        allowed = same & (r_mem | c_mem | (ci <= ri))
        fill = jnp.where(same, -1000000000.0, -jnp.inf).astype(F32)

        xr0 = pl.multiple_of(PRE + s * XR, 8)
        h_lhs = jnp.concatenate(
            [jnp.concatenate([mem[:, c * 128:(c + 1) * 128], xs[c, pl.ds(xr0, XR), :].astype(F32)],
                             axis=0).astype(BF16) for c in range(NC)], axis=1)
        wr = [pl.multiple_of(jax.lax.rem(xr0 + 8 * i, RING), 8) for i in range(XR // 8)]
        rd = pl.multiple_of(jax.lax.rem(s * SEG, RING), SEG)
        orow = pl.multiple_of(s * SEG, SEG)
        lag = pl.multiple_of(s * XR, 8)

        def proj(p):
            res = []
            for t in range(3):
                ms = []
                for hh in (2 * p, 2 * p + 1):
                    y = _dot(h_lhs, wqkv[t * H + hh])
                    for i in range(XR // 8):
                        ring[t * H + hh, pl.ds(wr[i], 8), :] = y[MEM + 8 * i:MEM + 8 * (i + 1)].astype(BF16)
                    ms.append(y[0:MEM])
                res.append(jnp.concatenate(ms, axis=0).astype(BF16))
            return res

        def attend(p, mrows):
            q, k, v = [jnp.concatenate([ring[t * H + 2 * p, pl.ds(rd, SEG), :],
                                        ring[t * H + 2 * p + 1, pl.ds(rd, SEG), :],
                                        mrows[t]], axis=0) for t in range(3)]
            sc = _dot_nt(q, k) * scale
            sc = jnp.where(allowed, sc, fill)
            m = jnp.max(sc, axis=1, keepdims=True)
            e = jnp.exp(sc - m)
            l = jnp.sum(e, axis=1, keepdims=True)
            o = _dot(e.astype(BF16), v) / l
            for i, hh in enumerate((2 * p, 2 * p + 1)):
                obuf[hh, pl.ds(orow, SEG), :] = o[i * SEG:(i + 1) * SEG].astype(BF16)
                lagged = obuf[hh, pl.ds(lag, XR), :].astype(F32)
                om = o[2 * SEG + i * MEM:2 * SEG + (i + 1) * MEM]
                olhs[hh] = jnp.concatenate([om, lagged], axis=0).astype(BF16)

        pend = None
        for p in range(H // 2):
            cur = proj(p)
            if pend is not None:
                attend(p - 1, pend)
            pend = cur
        HA = H - 4
        oa = jnp.concatenate([olhs[hh] for hh in range(HA)], axis=1)
        parts = [_dot(oa, wo[n, 0:HA * DH, :]) for n in range(NC)]
        attend(H // 2 - 1, pend)
        ob = jnp.concatenate([olhs[hh] for hh in range(HA, H)], axis=1)
        for n in range(NC):
            y = parts[n] + _dot(ob, wo[n, HA * DH:H * DH, :])
            mem[:, n * 128:(n + 1) * 128] = y[0:MEM].astype(BF16).astype(F32)
            bbuf[n, pl.ds(lag, XR), :] = y[MEM:].astype(BF16)
        return carry
    jax.lax.fori_loop(0, NSEG, step, 0)

    opost = jnp.concatenate([obuf[hh, S - PRE:S, :] for hh in range(H)], axis=1)
    for n in range(NC):
        bbuf[n, S - PRE:S, :] = _dot(opost, wo[n]).astype(BF16)

    RB = 256

    def out_copy(i):
        return pltpu.make_async_copy(outbuf.at[pl.ds(i * RB, RB), :], out_hbm.at[pl.ds(i * RB, RB), :],
                                     sem_out.at[i])

    for i in range(S // RB):
        r = i * RB
        z = None
        for c in range(NC):
            t = xs[c, r:r + RB, :].astype(F32) * gate_ref[c:c + 1, :]
            z = t if z is None else z + t
        g = jax.nn.sigmoid(jnp.sum(z, axis=1, keepdims=True))
        for c in range(NC):
            a = abuf[c, r:r + RB, :].astype(F32)
            b = bbuf[c, r:r + RB, :].astype(F32)
            outbuf[r:r + RB, c * 128:(c + 1) * 128] = (g * a + (1.0 - g) * b).astype(BF16)
        out_copy(i).start()
    for i in range(S // RB):
        out_copy(i).wait()


@functools.partial(jax.jit, static_argnames=("B_seg_len",))
def pallas_gated_mix__ssm_conv_h3__memory_aug_recurrent_mem_tr__prompt_kernel(
    A_q, A_k, A_v, A_shift_k, A_ssm_k, A_ssm_D, B_x, B_mem0, B_Wq, B_Wk, B_Wv, B_Wo,
    B_seg_len, gate_w,
):
    del B_x
    assert B_seg_len == SEG and A_q.shape == (1, S, D) and B_Wq.shape == (D, H, DH)
    fwd, inv = _dft_tables()
    hbm = pl.BlockSpec(memory_space=pl.ANY)
    vmem = pl.BlockSpec(memory_space=pltpu.VMEM)
    out = pl.pallas_call(
        _kernel,
        out_shape=jax.ShapeDtypeStruct((S, D), BF16),
        in_specs=[hbm] * 8 + [vmem] * 6,
        out_specs=hbm,
        scratch_shapes=[
            pltpu.VMEM((NC, S, 128), BF16),
            pltpu.VMEM((NC, S, 128), BF16),
            pltpu.VMEM((NC, S, 128), BF16),
            pltpu.VMEM((NC, 128, S), BF16),
            pltpu.VMEM((2, D, 8, 128), BF16),
            pltpu.VMEM((128 * 8, 128), F32),
            pltpu.VMEM((3 * H, D, 128), BF16),
            pltpu.VMEM((NC, H * DH, 128), BF16),
            pltpu.VMEM((3 * H, RING, 128), BF16),
            pltpu.VMEM((H, S, 128), BF16),
            pltpu.VMEM((H, MEM + XR, 128), BF16),
            pltpu.VMEM((NC, S, 128), BF16),
            pltpu.VMEM((NC, S, 128), BF16),
            pltpu.VMEM((S + 8, 128), F32),
            pltpu.VMEM((S, 128), BF16),
            pltpu.VMEM((NB, 2 * CB, 128), F32),
            pltpu.VMEM((NB, 2 * CB, 128), F32),
            pltpu.VMEM((NB, 2 * CB, 128), BF16),
            pltpu.VMEM((S, D), BF16),
            pltpu.VMEM((MEM, D), F32),
            pltpu.SemaphoreType.DMA((NC,)),
            pltpu.SemaphoreType.DMA((NC,)),
            pltpu.SemaphoreType.DMA((NC,)),
            pltpu.SemaphoreType.DMA((NC,)),
            pltpu.SemaphoreType.DMA((2,)),
            pltpu.SemaphoreType.DMA((NC,)),
            pltpu.SemaphoreType.DMA((S // 256,)),
        ],
        compiler_params=pltpu.CompilerParams(vmem_limit_bytes=120 * 1024 * 1024),
    )(
        A_q.reshape(S, D), A_k.reshape(S, D), A_v.reshape(S, D), A_ssm_k,
        B_Wq, B_Wk, B_Wv, B_Wo.reshape(H * DH, D),
        A_shift_k.T.reshape(KS, NC, 128).transpose(1, 0, 2),
        A_ssm_D.reshape(NC, 128).astype(F32), gate_w.reshape(NC, 128).astype(F32),
        B_mem0.reshape(MEM, D),
        jnp.asarray(fwd, BF16), jnp.asarray(inv, BF16),
    )
    return out.reshape(1, S, D)
```

```python
import functools

import jax
import jax.numpy as jnp
import numpy as np
import jax.experimental.pallas as pl
import jax.experimental.pallas.tpu as pltpu

F32 = jnp.float32
BF16 = jnp.bfloat16
U32 = jnp.uint32

S = 2048
D = 1024
NC = D // 128
H = 32
DH = 128
MEM = 8
SEG = 32
NSEG = S // SEG
XR = 24
PRE = S - NSEG * XR
RING = PRE + SEG
CB = 128
NB = S // CB
KS = 4
KPAD = 16
MB = 128
NCH = 12
NSLOT = 3
STG = 3 * H
WO0 = 3 * H + 1
G0 = WO0 + 4 * NC
UB = 0
KB = 2 * NB * 2 * CB
ZB = 2 * KB
TOKD = 100
LINK = 1
MAC_T0 = 4
MAC_G = 4
def _program(kind):
    seq = []
    if kind == 0:
        g = 0
        for tick in range(18):
            if 1 <= tick <= 16:
                seq.append(f"q{tick - 1}")
            if tick >= 2:
                seq.append(f"v{tick - 2}")
            if tick < 16:
                seq.append(f"P{tick}")
            else:
                seq.append(f"O{g}"); g += 1
            if 1 <= tick <= 16:
                seq.append(f"S{tick - 1}")
            if tick >= 2:
                seq.append(f"V{tick - 2}")
            if 8 <= tick < 16 and tick % 2 == 0:
                seq.append(f"O{g}"); g += 1
            if tick == 1:
                seq.append("I")
            if tick == 3:
                seq.append("F")
        seq += ["O6", "O7"]
    elif kind == 1:
        seq = "P0 P1 I q0 q1 P2 S0 S1 P3 F".split()
        g = 0
        for k in range(1, 7):
            a, b = 2 * k, 2 * k + 1
            seq += [f"q{a}", f"q{b}", f"v{a - 2}", f"v{b - 2}", f"P{a + 2}", f"S{a}", f"S{b}", f"V{a - 2}", f"V{b - 2}", f"P{b + 2}"]
            if k >= 3:
                seq.append(f"O{g}"); g += 1
        seq += "q14 q15 v12 v13 O4 S14 S15 V12 V13 v14 v15 O5 V14 V15 O6 O7".split()
    return " ".join(seq)


PROGRAM = _program(1)
GATE_OPS = 0
GATE_ALL = 0
DEADL = 0
MIDW = 0
TAILD = 0
NST = NSEG
CONV_IN = 7


def _dft_tables():
    f = np.concatenate([np.arange(0, CB, 2), np.arange(1, CB, 2)]).astype(np.float64)
    t = np.arange(CB, dtype=np.float64)
    ang = 2.0 * np.pi * (f[:, None] + 0.5) * t[None, :] / (2 * CB)
    fwd = np.concatenate([np.cos(ang), -np.sin(ang)], axis=0)
    inv = np.concatenate([np.cos(ang).T, -np.sin(ang).T], axis=1) / CB
    return fwd, inv


def _dot(a, b):
    return jnp.dot(a, b, preferred_element_type=F32)


def _dot_nt(a, b):
    return jax.lax.dot_general(a, b, (((1,), (1,)), ((), ())), preferred_element_type=F32)


def _mo(x, m):
    return x if isinstance(x, int) else pl.multiple_of(x, m)


def _kernel(x_hbm, k_hbm, v_hbm, ssm_hbm, wq_hbm, wk_hbm, wv_hbm, wo_hbm,
            shift_hbm, dskip_hbm, gate_hbm, mem0_hbm, fwd_hbm, inv_hbm,
            out_hbm,
            xs, ks, vs, ssm, wraw, wts, ring, obuf, outb, olhs, oacc, mem, small,
            kf, spec, zspec, gbuf, shift_ref, dskip_ref, gate_ref, mem0_ref, fwd_ref, inv_ref,
            zero_ref, sems, sem_w):
    w_hbm = (wq_hbm, wk_hbm, wv_hbm)

    def x_copy(c, part):
        r0, n = (0, PRE) if part == 0 else (PRE, S - PRE)
        return pltpu.make_async_copy(x_hbm.at[pl.ds(r0, n), pl.ds(_mo(c * 128, 128), 128)],
                                     xs.at[c, pl.ds(r0, n), :], sems.at[part])

    def conv_copies(c):
        col = pl.ds(c * 128, 128)
        sem = sems.at[2 if c < 2 else 3]
        return [pltpu.make_async_copy(k_hbm.at[:, col], ks.at[c, pl.ds(KPAD, S), :], sem),
                pltpu.make_async_copy(v_hbm.at[:, col], vs.at[c + 1], sem),
                pltpu.make_async_copy(ssm_hbm.at[col, :], ssm.at[c], sem)]

    def wo_copy(i):
        return pltpu.make_async_copy(
            wo_hbm.at[pl.ds(_mo((i & 1) * S, S), S), pl.ds(_mo((i >> 1) * 128, 128), 128)],
            obuf.at[i], sems.at[1])

    def w_copy(t, g, slot):
        return pltpu.make_async_copy(w_hbm[t].at[:, pl.ds(_mo(g * 8, 8), 8), :], wraw.at[slot], sem_w.at[slot])

    def w0_copy(i):
        return pltpu.make_async_copy(wq_hbm.at[pl.ds(i * 256, 256), pl.ds(0, 8), :],
                                     wraw.at[0, pl.ds(i * 256, 256)], sems.at[5 + i])

    small_copies = [pltpu.make_async_copy(a, b, sems.at[9]) for a, b in (
        (shift_hbm, shift_ref), (dskip_hbm, dskip_ref), (gate_hbm, gate_ref),
        (mem0_hbm, mem0_ref), (fwd_hbm, fwd_ref), (inv_hbm, inv_ref))]

    for i in range(4):
        w0_copy(i).start()
    for c in range(NC):
        x_copy(c, 0).start()

    zero_ref[0] = 0
    for c in range(NC):
        ks[c, 0:KPAD, :] = jnp.zeros((KPAD, 128), BF16)

    def gate_block(r0, n):
        z = None
        for c in range(NC):
            t = xs[c, r0:r0 + n, :].astype(F32) * small[NC + c:NC + c + 1, :]
            z = t if z is None else z + t
        z = jnp.sum(z, axis=1, keepdims=True)
        gbuf[r0:r0 + n, :] = jnp.broadcast_to(0.5 * jnp.tanh(0.5 * z) + 0.5, (n, 128))

    def relayout_piece(c, slot, q):
        o = (q % 2) * 128
        blk = wraw[slot, q * 16:(q + 1) * 16]
        wts[STG, o:o + 128, :] = pltpu.bitcast(blk.astype(F32).reshape(16 * 8, 128), U32)
        vals = [pltpu.bitcast(wts[STG, pl.ds(o + j, 16, stride=8), :], F32) for j in range(8)]
        for j in range(8):
            wts[c * 8 + j, q * 8:(q + 1) * 8, :] = pltpu.bitcast(vals[j].astype(BF16), U32)

    def pre_mm(c, j, r):
        w = pltpu.bitcast(wts[c * 8 + j], BF16)
        xp = jnp.concatenate([xs[cc, r:r + MB, :] for cc in range(NC)], axis=1)
        y = _dot(xp, w)
        ring[c * 8 + j, r:r + MB, :] = y.astype(BF16)
        return pltpu.bitcast(y[MB - 8:MB], U32)

    for i in range(4):
        for c in range(2 * i, 2 * i + 2):
            outb[c + 1] = jnp.zeros((S, 128), BF16)
        w0_copy(i).wait()
        if i == 0:
            w_copy(0, 1, 1).start()
            w_copy(0, 2, 2).start()
            for cp in small_copies:
                cp.start()
        for q in range(16 * i, 16 * i + 16):
            relayout_piece(0, 0, q)
    w_copy(0, 3, 0).start()
    for c in range(NC):
        x_copy(c, 0).wait()
    if not MIDW:
        w_copy(0, 1, 1).wait()

    def pre_chunk(c, carry):
        cn, slot = carry
        nslot = jnp.where(slot == NSLOT - 1, 0, slot + 1)
        q = 0
        for d in range(32):
            pre_mm(c, d // 4, (d % 4) * MB)
            if MIDW and d == MIDW - 1:
                w_copy(0, 0, slot).wait()
            if d >= MIDW - 1:
                while q < (64 * (d + 2 - MIDW) // (33 - MIDW - TAILD) if MIDW else 2 * (d + 1)) and q < 64:
                    relayout_piece(cn, slot, q)
                    q += 1
        assert q == 64
        n = cn + NSLOT
        for t in range(1, 3):
            @pl.when((n >> 2) == t)
            def _():
                w_copy(t, n & 3, slot).start()

        @pl.when(c < NC)
        def _():
            wo_copy(2 * c).start()
            wo_copy(2 * c + 1).start()
            x_copy(c, 1).start()

        @pl.when(c == NC)
        def _():
            for cp in conv_copies(0) + conv_copies(1):
                cp.start()

        if not MIDW:
            @pl.when(cn + 1 < NCH)
            def _():
                w_copy(0, 0, nslot).wait()
        return cn + 1, nslot
    c_last = jax.lax.fori_loop(0, NCH - 1, pre_chunk, (1, 1))[0] - 1

    for cp in small_copies:
        cp.wait()
    small[0:NC, :] = dskip_ref[...].astype(F32)
    small[NC:2 * NC, :] = gate_ref[...].astype(F32)
    mem[...] = mem0_ref[...].astype(F32)
    for i in range(2 * NC):
        wo_copy(i).wait()
    for c in range(NC):
        x_copy(c, 1).wait()
    q = 0
    for j in range(8):
        for r in range(0, PRE, MB):
            pre_mm(c_last, j, r)
            wts[WO0 + q] = pltpu.bitcast(obuf[q // 2, (q % 2) * 1024:(q % 2 + 1) * 1024, :], U32)
            q += 1

    def gate_rows(r0, n):
        return gbuf[pl.ds(r0, n), :]

    def accumulate(slab, rows, val):
        outb[slab, rows, :] = (outb[slab, rows, :].astype(F32) + val.astype(BF16).astype(F32)).astype(BF16)

    for cp in conv_copies(0) + conv_copies(1):
        cp.wait()
    for c in range(2, NC):
        for cp in conv_copies(c):
            cp.start()

    def conv_fwd(t, j):
        tr = t if isinstance(t, int) else jnp.minimum(t, NC - 1)
        slot = t & 1
        r0 = _mo(j * 2 * CB, 2 * CB)
        shift = shift_ref[tr].astype(F32)
        kf[...] = ks[tr, pl.ds(r0, 2 * CB + KPAD), :].astype(F32)
        fwd = fwd_ref[...]
        for i in range(2):
            o = KPAD + i * CB
            acc = kf[o:o + CB, :] * shift[0:1, :]
            for l in range(1, KS):
                acc = acc + kf[o - l:o - l + CB, :] * shift[l:l + 1, :]
            rows = pl.ds(_mo(r0 + i * CB, CB), CB)
            kv = (acc * vs[tr + 1, rows, :].astype(F32)).astype(BF16)
            vs[t + 1, rows, :] = kv
            sr = _mo((2 * j + i) * 32, 32)
            for off, res in ((0, _dot(fwd, kv)), (512, _dot_nt(fwd, ssm[tr, :, rows]))):
                for ri in range(2):
                    for fj in range(8):
                        spec[slot * 8 + fj, pl.ds(sr + (off + ri * 16), 16), :] = (
                            res[ri * CB + fj * 16:ri * CB + (fj + 1) * 16])

    def tie(x, gate):
        return x if gate is None else pltpu.bitcast(pltpu.bitcast(x, jnp.int32) | gate, F32)

    def conv_mac(t, j):
        slot = t & 1
        sign = jnp.where(j < 4, 1.0, -1.0).astype(F32)
        base0 = slot * 8 + j
        zero = zero_ref[0]
        zbase = pl.multiple_of(slot * (NB * CB) + j * 8, 8)
        prev = None
        gate = yield None
        for i in range(NB):
            base = base0 + zero * (i + 1)
            ys = []
            for hv in range(2):
                yr = yi = None
                for jj in range(i + 1):
                    uo = jj * 32 + hv * 8
                    ko = 512 + (i - jj) * 32 + hv * 8
                    ur = spec[base, uo:uo + 8, :]
                    ui = spec[base, uo + 16:uo + 24, :]
                    kr = spec[base, ko:ko + 8, :]
                    ki = spec[base, ko + 16:ko + 24, :]
                    if GATE_OPS:
                        ur, ui = tie(ur, gate), tie(ui, gate)
                        tr, ti = ur * kr - ui * ki, ur * ki + ui * kr
                    else:
                        tr, ti = tie(ur * kr - ui * ki, gate), tie(ur * ki + ui * kr, gate)
                    yr, yi = (tr, ti) if yr is None else (yr + tr, yi + ti)
                    if jj < i or hv == 0:
                        gate = yield yr
                ys.append((yr, yi))
            yr = jnp.concatenate([ys[0][0], ys[1][0]], axis=0)
            yi = jnp.concatenate([ys[0][1], ys[1][1]], axis=0)
            zr, zi = (yr, yi) if prev is None else (yr - sign * prev[1], yi + sign * prev[0])
            prev = (yr, yi)
            zspec[pl.ds(zbase + i * CB, 8), :] = pltpu.bitcast(zr.astype(BF16), U32)
            zspec[pl.ds(zbase + (i * CB + CB // 2), 8), :] = pltpu.bitcast(zi.astype(BF16), U32)
            gate = yield ys[1][0]

    def conv_inv(t, j):
        tr = t if isinstance(t, int) else jnp.maximum(t, 0)
        slot = t & 1
        dsk = small[pl.ds(tr, 1), :]
        inv = inv_ref[...]
        for i in range(2):
            r0 = _mo((2 * j + i) * CB, CB)
            rows = pl.ds(r0, CB)
            z = zspec[pl.ds(_mo((slot * NB + 2 * j + i) * CB, CB), CB), :]
            y = _dot(inv, pltpu.bitcast(z, BF16))
            y = y + vs[t + 1, rows, :].astype(F32) * dsk
            accumulate(t + 1, rows, gate_rows(r0, CB) * (xs[tr, rows, :].astype(F32) * y))

    for j in range(NB // 2):
        conv_fwd(0, j)
        for r in range(j * 256, (j + 1) * 256, 64):
            gate_block(r, 64)

    scale = float(DH) ** -0.5
    NR = 2 * (SEG + MEM)

    def wrap(r):
        return jnp.where(r >= RING, r - RING, r)

    def step(s, carry):
        wr0, rd0 = carry
        ct = jax.lax.shift_right_logical(s, 3)
        cj = jnp.bitwise_and(s, 7)
        ri = jax.lax.broadcasted_iota(jnp.int32, (NR, NR), 0)
        ci = jax.lax.broadcasted_iota(jnp.int32, (NR, NR), 1)
        r_mem = ri >= 2 * SEG
        c_mem = ci >= 2 * SEG
        r_head = jnp.where(r_mem, (ri - 2 * SEG) // MEM, ri // SEG)
        c_head = jnp.where(c_mem, (ci - 2 * SEG) // MEM, ci // SEG)
        same = r_head == c_head
        allowed = same & (r_mem | c_mem | (ci <= ri))
        fill = jnp.where(same, -1000000000.0, -jnp.inf).astype(F32)

        xr0 = pl.multiple_of(PRE + s * XR, 8)
        h_lhs = jnp.concatenate(
            [jnp.concatenate([mem[:, c * 128:(c + 1) * 128], xs[c, pl.ds(xr0, XR), :].astype(F32)],
                             axis=0).astype(BF16) for c in range(NC)], axis=1)
        wr = [pl.multiple_of(wrap(wr0 + 8 * i), 8) for i in range(XR // 8)]
        rd = pl.multiple_of(rd0, SEG)
        orow = pl.multiple_of(s * SEG, SEG)
        lag = pl.multiple_of(s * XR, 8)

        macs = conv_mac(ct, cj)
        next(macs)
        left = [NB * (NB + 1)]
        zvec = jnp.full((8, 128), zero_ref[0], jnp.int32)
        dead = []

        def side_work(token):
            if left[0] > 0 and CONV_IN & 2:
                gate = pltpu.bitcast(token, jnp.int32) & zvec
                for n in range(min(MAC_G, left[0])):
                    out = macs.send(gate if (n == 0 or GATE_ALL) else None)
                    left[0] -= 1
                dead.append(out)

        def proj(p):
            res = []
            for t in range(3):
                ms = []
                for hh in (2 * p, 2 * p + 1):
                    y = _dot(h_lhs, pltpu.bitcast(wts[t * H + hh], BF16))
                    for i in range(XR // 8):
                        yy = y[MEM + 8 * i:MEM + 8 * (i + 1)]
                        if DEADL and i == XR // 8 - 1 and len(dead) >= DEADL:
                            yy = tie(yy, pltpu.bitcast(dead.pop(0), jnp.int32) & zvec)
                        ring[t * H + hh, pl.ds(wr[i], 8), :] = yy.astype(BF16)
                    ms.append(y[0:MEM])
                    if p >= MAC_T0:
                        side_work(y[0:MEM])
                res.append(jnp.concatenate(ms, axis=0).astype(BF16))
            return res

        def xrows(t, p):
            return [ring[t * H + 2 * p, pl.ds(rd, SEG), :], ring[t * H + 2 * p + 1, pl.ds(rd, SEG), :]]

        def scores(q, k):
            sc = _dot_nt(q, k) * scale
            sc = jnp.where(allowed, sc, fill)
            m = jnp.max(sc, axis=1, keepdims=True)
            e = jnp.exp(sc - m)
            l = jnp.sum(e, axis=1, keepdims=True)
            r = pl.reciprocal(l, approx=True)
            r = r * (2.0 - l * r)
            return e.astype(BF16), r

        def values(p, v, e, r):
            o = _dot(e, v) * r
            for i, hh in enumerate((2 * p, 2 * p + 1)):
                obuf[hh, pl.ds(orow, SEG), :] = o[i * SEG:(i + 1) * SEG].astype(BF16)
                lagged = obuf[hh, pl.ds(lag, XR), :].astype(F32)
                om = o[2 * SEG + i * MEM:2 * SEG + (i + 1) * MEM]
                olhs[hh] = jnp.concatenate([om, lagged], axis=0).astype(BF16)

        def oproj(g):
            lhs = jnp.concatenate([olhs[hh] for hh in range(4 * g, 4 * g + 4)], axis=1)
            if g == H // 4 - 1:
                omg = 1.0 - gate_rows(lag, XR)
            for n in range(NC):
                w = wts[WO0 + 4 * n + g // 2, (g % 2) * 256:(g % 2 + 1) * 256, :]
                y = _dot(lhs, pltpu.bitcast(w, BF16))
                if g > 0:
                    y = y + oacc[n]
                if g < H // 4 - 1:
                    oacc[n] = y
                else:
                    mem[:, n * 128:(n + 1) * 128] = y[0:MEM].astype(BF16).astype(F32)
                    accumulate(n + 1, pl.ds(lag, XR), omg * y[MEM:].astype(BF16).astype(F32))

        NP = H // 2
        mrows = [None] * NP
        er = [None] * NP
        qk = [None] * NP
        vv = [None] * NP
        for item in PROGRAM.split():
            op, arg = item[0], int(item[1:] or 0)
            if op == "P":
                mrows[arg] = proj(arg)
            elif op == "q":
                qk[arg] = [jnp.concatenate(xrows(t, arg) + [mrows[arg][t]], axis=0) for t in range(2)]
            elif op == "v":
                vv[arg] = jnp.concatenate(xrows(2, arg) + [mrows[arg][2]], axis=0)
            elif op == "S":
                er[arg] = scores(*qk[arg])
            elif op == "V":
                values(arg, vv[arg], *er[arg])
            elif op == "O":
                oproj(arg)
            elif op == "I" and CONV_IN & 4:
                conv_inv(ct - 1, cj)
            elif op == "F" and CONV_IN & 1:
                conv_fwd(ct + 1, cj)
        assert left[0] == 0 or not CONV_IN & 2

        @pl.when(s == 6)
        def _():
            for c in range(2, NC):
                for cp in conv_copies(c):
                    cp.wait()
        return wrap(wr0 + XR), wrap(rd0 + SEG)
    jax.lax.fori_loop(0, NST, step, (PRE, 0))

    for j in range(NB // 2):
        conv_inv(NC - 1, j)

    def out_copies(r0, n):
        return [pltpu.make_async_copy(outb.at[c + 1, pl.ds(r0, n), :],
                                      out_hbm.at[pl.ds(r0, n), pl.ds(c * 128, 128)], sems.at[4])
                for c in range(NC)]

    for cp in out_copies(0, S - PRE):
        cp.start()

    def post_chunk(i, carry):
        r = pl.multiple_of(S - PRE + i * MB, MB)
        op = jnp.concatenate([obuf[hh, pl.ds(r, MB), :] for hh in range(H)], axis=1)
        omg = 1.0 - gate_rows(r, MB)
        for n in range(NC):
            w = jnp.concatenate([wts[WO0 + 4 * n + kq] for kq in range(4)], axis=0)
            y = _dot(op, pltpu.bitcast(w, BF16))
            accumulate(n + 1, pl.ds(r, MB), omg * y.astype(BF16).astype(F32))
        for cp in out_copies(r, MB):
            cp.start()
        return carry
    jax.lax.fori_loop(0, PRE // MB, post_chunk, 0)
    for cp in out_copies(0, S):
        cp.wait()


@functools.partial(jax.jit, static_argnames=("B_seg_len",))
def pallas_gated_mix__ssm_conv_h3__memory_aug_recurrent_mem_tr__prompt_kernel(
    A_q, A_k, A_v, A_shift_k, A_ssm_k, A_ssm_D, B_x, B_mem0, B_Wq, B_Wk, B_Wv, B_Wo,
    B_seg_len, gate_w,
):
    del B_x
    assert B_seg_len == SEG and A_q.shape == (1, S, D) and B_Wq.shape == (D, H, DH)
    fwd, inv = _dft_tables()
    hbm = pl.BlockSpec(memory_space=pl.ANY)
    vmem = pl.BlockSpec(memory_space=pltpu.VMEM)
    out = pl.pallas_call(
        _kernel,
        out_shape=jax.ShapeDtypeStruct((S, D), BF16),
        in_specs=[hbm] * 14,
        out_specs=hbm,
        scratch_shapes=[
            pltpu.VMEM((NC, S, 128), BF16),
            pltpu.VMEM((NC, KPAD + S, 128), BF16),
            pltpu.VMEM((NC + 2, S, 128), BF16),
            pltpu.VMEM((NC, 128, S), BF16),
            pltpu.VMEM((NSLOT, D, 8, 128), BF16),
            pltpu.VMEM((G0, D // 2, 128), U32),
            pltpu.VMEM((3 * H, RING, 128), BF16),
            pltpu.VMEM((H, S, 128), BF16),
            pltpu.VMEM((NC + 1, S, 128), BF16),
            pltpu.VMEM((H, MEM + XR, 128), BF16),
            pltpu.VMEM((NC, MEM + XR, 128), F32),
            pltpu.VMEM((MEM, D), F32),
            pltpu.VMEM((2 * NC, 128), F32),
            pltpu.VMEM((2 * CB + KPAD, 128), F32),
            pltpu.VMEM((16, 1024, 128), F32),
            pltpu.VMEM((2 * NB * CB, 128), U32),
            pltpu.VMEM((S, 128), F32),
            pltpu.VMEM((NC, KS, 128), BF16),
            pltpu.VMEM((NC, 128), BF16),
            pltpu.VMEM((NC, 128), BF16),
            pltpu.VMEM((MEM, D), BF16),
            pltpu.VMEM((2 * CB, CB), BF16),
            pltpu.VMEM((CB, 2 * CB), BF16),
            pltpu.SMEM((1,), jnp.int32),
            pltpu.SemaphoreType.DMA((10,)),
            pltpu.SemaphoreType.DMA((NSLOT,)),
        ],
        compiler_params=pltpu.CompilerParams(vmem_limit_bytes=120 * 1024 * 1024),
    )(
        A_q.reshape(S, D), A_k.reshape(S, D), A_v.reshape(S, D), A_ssm_k,
        B_Wq, B_Wk, B_Wv, B_Wo.reshape(H * DH, D),
        A_shift_k.T.reshape(KS, NC, 128).transpose(1, 0, 2),
        A_ssm_D.reshape(NC, 128), gate_w.reshape(NC, 128),
        B_mem0.reshape(MEM, D),
        jnp.asarray(fwd, BF16), jnp.asarray(inv, BF16),
    )
    return out.reshape(1, S, D)
```

```python
import functools

import jax
import jax.numpy as jnp
import numpy as np
import jax.experimental.pallas as pl
import jax.experimental.pallas.tpu as pltpu

F32 = jnp.float32
BF16 = jnp.bfloat16
U32 = jnp.uint32
I32 = jnp.int32

S = 2048
D = 1024
NC = D // 128
H = 32
DH = 128
MEM = 8
SEG = 32
NSEG = S // SEG
XR = 24
PRE = S - NSEG * XR
RING = PRE + 2 * SEG
NR = 2 * (SEG + MEM)
CB = 128
NB = S // CB
KS = 4
KPAD = 16
MB = 128
SST = 9
MAC_G = 3


def _expand(text):
    out = []
    for item in text.split():
        if "-" in item:
            a, b = item[1:].split("-")
            out += [(item[0], i) for i in range(int(a), int(b) + 1)]
        else:
            out.append((item[0], int(item[1:] or 0)))
    return out


PROGRAM = _expand("P0-4 S0-3 P5-8 V0-3 S4-7 P9-10 O0 P11-12 V4-7 S8-11 P13 O1 P14-15 "
                  "O2 V8-11 S12-15 O3 O4 V12-15 O5 O6 O7 I F")


def _dft_tables():
    f = np.concatenate([np.arange(0, CB, 2), np.arange(1, CB, 2)]).astype(np.float64)
    t = np.arange(CB, dtype=np.float64)
    ang = 2.0 * np.pi * (f[:, None] + 0.5) * t[None, :] / (2 * CB)
    fwd = np.concatenate([np.cos(ang), -np.sin(ang)], axis=0)
    inv = np.concatenate([np.cos(ang).T, -np.sin(ang).T], axis=1) / CB
    return fwd, inv


def _dot(a, b):
    return jnp.dot(a, b, preferred_element_type=F32)


def _dot_nt(a, b):
    return jax.lax.dot_general(a, b, (((1,), (1,)), ((), ())), preferred_element_type=F32)


def _mo(x, m):
    return x if isinstance(x, int) else pl.multiple_of(x, m)


def _tie(x, gate):
    return x if gate is None else pltpu.bitcast(pltpu.bitcast(x, I32) | gate, x.dtype)


def _gate(token, zero):
    return pltpu.bitcast(token, I32) & jnp.full((8, 128), zero, I32)


def _zero_of(counter):
    return jax.lax.shift_right_logical(counter, 16)


def _kernel(x_hbm, k_hbm, v_hbm, ssm_hbm, wq_hbm, wk_hbm, wv_hbm, wo_hbm,
            shift_hbm, dskip_hbm, gate_hbm, mem0_hbm, fwd_hbm, inv_hbm,
            out_hbm,
            xs, ks, vs, ssm, wraw, wts, wos, ring0, ring1, ring2, ring3, obuf, outb, olhs, oacc,
            mem, small, kf, stage, fbuf, ebuf, spec, zspec, gbuf,
            fwd_ref, inv_ref, mem0_ref, shift_ref, dskip_ref, gate_ref,
            sems, sem_w):
    w_hbm = (wq_hbm, wk_hbm, wv_hbm)
    rings = (ring0, ring1, ring2, ring3)

    def x_copy(c, part):
        r0, n, si = ((0, MB, 0), (MB, PRE - MB, 10), (PRE, S - PRE, 1))[part]
        return pltpu.make_async_copy(x_hbm.at[pl.ds(r0, n), pl.ds(_mo(c * 128, 128), 128)],
                                     xs.at[c, pl.ds(r0, n), :], sems.at[si])

    def conv_copies(c):
        col = pl.ds(c * 128, 128)
        sem = sems.at[2 if c < 2 else 3]
        return [pltpu.make_async_copy(k_hbm.at[:, col], ks.at[c, pl.ds(KPAD, S), :], sem),
                pltpu.make_async_copy(v_hbm.at[:, col], vs.at[c + 1], sem),
                pltpu.make_async_copy(ssm_hbm.at[col, :], ssm.at[c], sem)]

    def wo_copy(i):
        return pltpu.make_async_copy(
            wo_hbm.at[pl.ds(_mo((i & 1) * S, S), S), pl.ds(_mo((i >> 1) * 128, 128), 128)],
            obuf.at[i], sems.at[1])

    def w_copy(t, g, slot):
        return pltpu.make_async_copy(w_hbm[t].at[:, pl.ds(g * 8, 8), :], wraw.at[slot], sem_w.at[slot])

    def w0_copy(i):
        return pltpu.make_async_copy(wq_hbm.at[pl.ds(i * 256, 256), pl.ds(0, 8), :],
                                     wraw.at[0, pl.ds(i * 256, 256)], sems.at[5 + i])

    small_copies = [pltpu.make_async_copy(a, b, sems.at[9]) for a, b in (
        (shift_hbm, shift_ref), (dskip_hbm, dskip_ref), (gate_hbm, gate_ref),
        (mem0_hbm, mem0_ref), (fwd_hbm, fwd_ref), (inv_hbm, inv_ref))]

    def background(c):
        wo_copy(2 * c).start()
        wo_copy(2 * c + 1).start()
        x_copy(c, 2).start()

    for i in range(4):
        w0_copy(i).start()
    for c in range(NC):
        x_copy(c, 0).start()

    def clear(c, count):
        ks[c, 0:KPAD, :] = jnp.zeros((KPAD, 128), BF16)
        outb[c + 1] = jnp.zeros((S, 128), BF16)
        return count + 1

    def relayout_piece(c, slot, q, gate=None):
        st = stage.at[q % 2]
        blk = wraw[slot, q * 16:(q + 1) * 16].astype(F32)
        for i in range(16):
            st[i * SST:i * SST + 8, :] = _tie(blk[i], gate if i % 8 == 0 else None)
        for j in range(8):
            wts[c * 8 + j, q * 8:(q + 1) * 8, :] = pltpu.bitcast(
                st[pl.ds(j, 16, stride=SST), :].astype(BF16), U32)

    def relayout_with(y, zero, c, slot, d, span):
        qs = range(min(64 * d // span, 64), min(64 * (d + 1) // span, 64))
        for i, q in enumerate(qs):
            o = (i * MB // len(qs)) // 8 * 8
            relayout_piece(c, slot, q, _gate(y[o:o + 8], zero))

    def pre_mm(t, g, d):
        j, r = d // 4, (d % 4) * MB
        w = pltpu.bitcast(wts[t * 8 + (g * 24 + j)], BF16)
        xp = jnp.concatenate([xs[c, r:r + MB, :] for c in range(NC)], axis=1)
        y = _dot(xp, w)
        rings[g][t * 8 + j, r:r + MB, :] = y.astype(BF16)
        return y

    count = 0
    for i in range(4):
        count = jax.lax.fori_loop(2 * i, 2 * i + 2, clear, count)
        w0_copy(i).wait()
        if i == 0:
            for c in range(NC):
                x_copy(c, 1).start()
        if i == 1:
            for t in range(1, 3):
                w_copy(t, 0, t).start()
        for q in range(16 * i, 16 * i + 16):
            relayout_piece(0, 0, q)
    w_copy(0, 1, 0).start()
    for cp in small_copies:
        cp.start()
    for c in range(NC):
        x_copy(c, 0).wait()

    for e in range(32):
        if e == 8:
            for c in range(NC):
                x_copy(c, 1).wait()
        if e == 24:
            w_copy(1, 0, 1).wait()
        y = pre_mm(0, 0, (e % 8) * 4 + e // 8)
        if e >= 24:
            relayout_with(y, _zero_of(count), 1, 1, e - 24, 7)
    w_copy(1, 1, 1).start()
    background(0)

    def pre_chunk(t, count, g):
        zero = _zero_of(count)
        tn = jnp.where(t == 2, 0, t + 1)
        w_copy(0, 0, tn).wait()
        for d in range(32):
            y = pre_mm(t, g, d)
            relayout_with(y, zero, t + (3 * g + 1), tn, d, 31)
            if g == 3:
                for i in range(2):
                    gate = _gate(y[64 * i + 32:64 * i + 40], zero)
                    for r in range((d % 2) * 256 + i * 128, (d % 2) * 256 + (i + 1) * 128, 8):
                        o = ((d // 2) % 2) * 1024 + 2 * r
                        wos[t * 16 + d // 2, r:r + 8, :] = _tie(
                            pltpu.bitcast(obuf[t * 8 + d // 4, o:o + 16, :], U32), gate)
        for tt in range(3):
            gg = g + (2 if tt == 0 else 1)
            if gg < 4:
                @pl.when(tn == tt)
                def _():
                    w_copy(tt, gg, tt).start()

        if g < 3:
            @pl.when(t + 3 * g < NC)
            def _():
                background(t + 3 * g)

        if g == 2:
            @pl.when(t == 2)
            def _():
                for cp in conv_copies(0) + conv_copies(1):
                    cp.start()
        return count + 1

    for g in range(4):
        if g == 3:
            for i in range(2 * NC):
                wo_copy(i).wait()
            for c in range(NC):
                x_copy(c, 2).wait()
        count = jax.lax.fori_loop(1 if g == 0 else 0, 3 if g < 3 else 2,
                                  functools.partial(pre_chunk, g=g), count)

    for cp in small_copies:
        cp.wait()
    for cp in conv_copies(0) + conv_copies(1):
        cp.wait()
    small[0:NC, :] = dskip_ref[...].astype(F32)
    gate_w = gate_ref[...].astype(F32)
    for c in range(NC):
        small[NC + 8 * c:NC + 8 * (c + 1), :] = jnp.broadcast_to(gate_w[c:c + 1, :], (8, 128))
    mem[...] = mem0_ref[...].astype(F32)

    def mix_gate(r0, gate):
        z = None
        for c in range(NC):
            gw = small[NC + 8 * c:NC + 8 * (c + 1), :]
            t = xs[c, r0:r0 + 16, :].astype(F32) * jnp.concatenate([gw, gw], axis=0)
            z = _tie(t, jnp.concatenate([gate, gate], axis=0)) if z is None else z + t
        z = jnp.sum(z, axis=1, keepdims=True)
        gbuf[r0:r0 + 16, :] = jnp.broadcast_to(0.5 * jnp.tanh(0.5 * z) + 0.5, (16, 128))

    def accumulate(slab, rows, val):
        outb[slab, rows, :] = (outb[slab, rows, :].astype(F32) + val.astype(BF16).astype(F32)).astype(BF16)

    def conv_prep(t, j):
        tr = t if isinstance(t, int) else jnp.minimum(t, NC - 1)
        r0 = _mo(j * 2 * CB, 2 * CB)
        shift = shift_ref[tr].astype(F32)
        gate = yield
        for o in range(0, 2 * CB + KPAD, 16):
            kk = ks[tr, pl.ds(_mo(r0 + o, 16), 16), :].astype(F32)
            kf[o:o + 8, :] = _tie(kk[0:8], gate)
            kf[o + 8:o + 16, :] = _tie(kk[8:16], gate)
            if o == 0:
                continue
            acc = kf[o:o + 16, :] * shift[0:1, :]
            for l in range(1, KS):
                acc = acc + kf[o - l:o - l + 16, :] * shift[l:l + 1, :]
            rows = pl.ds(_mo(r0 + (o - KPAD), 16), 16)
            vs[t + 1, rows, :] = (acc * vs[tr + 1, rows, :].astype(F32)).astype(BF16)
            gate = yield

    def conv_fwd(t, j):
        tr = t if isinstance(t, int) else jnp.minimum(t, NC - 1)
        slot = t & 1
        fwd = fwd_ref[...]
        for i in range(2):
            rows = pl.ds(_mo((2 * j + i) * CB, CB), CB)
            sr = _mo((2 * j + i) * 32, 32)
            for off, res in ((0, _dot(fwd, vs[t + 1, rows, :])), (512, _dot_nt(fwd, ssm[tr, :, rows]))):
                for ri in range(2):
                    for fj in range(8):
                        spec[slot * 8 + fj, pl.ds(sr + (off + ri * 16), 16), :] = (
                            res[ri * CB + fj * 16:ri * CB + (fj + 1) * 16])

    def conv_mac(t, j, zero):
        slot = t & 1
        sign = jnp.where(j < 4, 1.0, -1.0).astype(F32)
        zbase = pl.multiple_of(slot * (NB * CB) + j * 8, 8)
        prev = None
        gate = yield
        for i in range(NB):
            base = slot * 8 + j + zero * (i + 1)
            ys = []
            for hv in range(2):
                yr = yi = None
                for jj in range(i + 1):
                    uo = jj * 32 + hv * 8
                    ko = 512 + (i - jj) * 32 + hv * 8
                    ur = spec[base, uo:uo + 8, :]
                    ui = spec[base, uo + 16:uo + 24, :]
                    kr = spec[base, ko:ko + 8, :]
                    ki = spec[base, ko + 16:ko + 24, :]
                    tr, ti = _tie(ur * kr - ui * ki, gate), _tie(ur * ki + ui * kr, gate)
                    yr, yi = (tr, ti) if yr is None else (yr + tr, yi + ti)
                    if jj < i or hv == 0:
                        gate = yield
                ys.append((yr, yi))
            yr = jnp.concatenate([ys[0][0], ys[1][0]], axis=0)
            yi = jnp.concatenate([ys[0][1], ys[1][1]], axis=0)
            zr, zi = (yr, yi) if prev is None else (yr - sign * prev[1], yi + sign * prev[0])
            prev = (yr, yi)
            zspec[pl.ds(zbase + i * CB, 8), :] = pltpu.bitcast(zr.astype(BF16), U32)
            zspec[pl.ds(zbase + (i * CB + CB // 2), 8), :] = pltpu.bitcast(zi.astype(BF16), U32)
            gate = yield

    def conv_inv(t, j):
        tr = t if isinstance(t, int) else jnp.maximum(t, 0)
        slot = t & 1
        dsk = small[pl.ds(tr, 1), :]
        inv = inv_ref[...]
        for i in range(2):
            rows = pl.ds(_mo((2 * j + i) * CB, CB), CB)
            z = zspec[pl.ds(_mo((slot * NB + 2 * j + i) * CB, CB), CB), :]
            y = _dot(inv, pltpu.bitcast(z, BF16))
            y = y + vs[t + 1, rows, :].astype(F32) * dsk
            accumulate(t + 1, rows, gbuf[rows, :] * (xs[tr, rows, :].astype(F32) * y))

    for q in range(32):
        if q % 4 == 0:
            preps = conv_prep(0, q // 4)
            next(preps)
        y = pre_mm(2, 3, q)
        if q % 4 == 1 and q >= 4:
            conv_fwd(0, q // 4 - 1)
        for i in range(4):
            gate = _gate(y[32 * i:32 * i + 8], _zero_of(count))
            preps.send(gate)
            mix_gate(q * 64 + i * 16, gate)
    conv_fwd(0, NB // 2 - 1)

    ri = jax.lax.broadcasted_iota(I32, (NR, NR), 0)
    ci = jax.lax.broadcasted_iota(I32, (NR, NR), 1)
    r_mem = ri >= 2 * SEG
    c_mem = ci >= 2 * SEG
    same = (jnp.where(r_mem, (ri - 2 * SEG) // MEM, ri // SEG)
            == jnp.where(c_mem, (ci - 2 * SEG) // MEM, ci // SEG))
    keep = same & (r_mem | c_mem | (ci <= ri))
    fbuf[0, 0:NR, 0:NR] = jnp.where(keep, 0.0, jnp.where(same, -1000000000.0, -jnp.inf)).astype(F32)
    scale = float(DH) ** -0.5

    def wrap(r):
        return jnp.where(r >= RING, r - RING, r)

    def step(it, u, wr0, rdi):
        s = it * 2 + u
        zero = _zero_of(rdi)
        ct = jax.lax.shift_right_logical(s, 3)
        cj = jnp.bitwise_and(s, 7)
        xr0 = pl.multiple_of(PRE + s * XR, 8)
        wr = [pl.multiple_of(wrap(wr0 + 8 * i), 8) for i in range(XR // 8)]
        rd = pl.multiple_of(rdi * (2 * SEG) + u * SEG, SEG)
        orow = pl.multiple_of(it * (2 * SEG) + u * SEG, SEG)
        lag = pl.multiple_of(s * XR, 8)
        h_lhs = jnp.concatenate(
            [jnp.concatenate([mem[:, c * 128:(c + 1) * 128], xs[c, pl.ds(xr0, XR), :].astype(F32)],
                             axis=0).astype(BF16) for c in range(NC)], axis=1)

        macs = conv_mac(ct, cj, zero)
        next(macs)
        preps = conv_prep(ct + 1, cj)
        next(preps)
        n_mac = NB * (NB + 1)
        queue = [(preps, 1)] * 16 + [(macs, min(MAC_G, n_mac - n)) for n in range(0, n_mac, MAC_G)]

        def side_work(token):
            if queue:
                gen, cnt = queue.pop(0)
                gen.send(_gate(token, zero))
                for _ in range(cnt - 1):
                    gen.send(None)

        def proj(p):
            res = []
            for t in range(3):
                ms = []
                for hh in (2 * p, 2 * p + 1):
                    y = _dot(h_lhs, pltpu.bitcast(wts[(hh // 8) * 24 + t * 8 + hh % 8], BF16))
                    for i in range(XR // 8):
                        rings[hh // 8][t * 8 + hh % 8, pl.ds(wr[i], 8), :] = (
                            y[MEM + 8 * i:MEM + 8 * (i + 1)].astype(BF16))
                    ms.append(y[0:MEM])
                    side_work(y[0:MEM])
                res.append(jnp.concatenate(ms, axis=0).astype(BF16))
            return res

        def rows_of(t, p, mrows):
            return jnp.concatenate(
                [rings[p // 4][t * 8 + (2 * p + i) % 8, pl.ds(rd, SEG), :] for i in range(2)] + [mrows[t]],
                axis=0)

        def scores(p, mrows):
            sc = _dot_nt(rows_of(0, p, mrows), rows_of(1, p, mrows)) * scale
            fill = fbuf[zero * (p + 1), 0:NR, 0:NR]
            sc = jnp.where(fill == 0.0, sc, fill)
            e = jnp.exp(sc - jnp.max(sc, axis=1, keepdims=True))
            l = jnp.sum(e, axis=1, keepdims=True)
            r = pl.reciprocal(l, approx=True)
            ebuf[p + zero, 0:NR // 2, :] = pltpu.bitcast(e.astype(BF16), U32)
            return r * (2.0 - l * r)

        def values(p, mrows, r):
            o = _dot(pltpu.bitcast(ebuf[p, 0:NR // 2, :], BF16), rows_of(2, p, mrows)) * r
            for i, hh in enumerate((2 * p, 2 * p + 1)):
                obuf[hh, pl.ds(orow, SEG), :] = o[i * SEG:(i + 1) * SEG].astype(BF16)
                lagged = obuf[hh, pl.ds(lag, XR), :].astype(F32)
                om = o[2 * SEG + i * MEM:2 * SEG + (i + 1) * MEM]
                olhs[hh] = jnp.concatenate([om, lagged], axis=0).astype(BF16)

        def oproj(g):
            lhs = jnp.concatenate([olhs[hh] for hh in range(4 * g, 4 * g + 4)], axis=1)
            for n in range(NC):
                w = wos[4 * n + g // 2, (g % 2) * 256:(g % 2 + 1) * 256, :]
                y = _dot(lhs, pltpu.bitcast(w, BF16))
                side_work(y[0:MEM])
                if g > 0:
                    y = y + oacc[n + zero]
                if g < H // 4 - 1:
                    oacc[n] = y
                else:
                    mem[:, n * 128:(n + 1) * 128] = y[0:MEM].astype(BF16).astype(F32)
                    accumulate(n + 1, pl.ds(lag, XR),
                               (1.0 - gbuf[pl.ds(lag, XR), :]) * y[MEM:].astype(BF16).astype(F32))

        mrows = [None] * (H // 2)
        recip = [None] * (H // 2)
        for op, arg in PROGRAM:
            if op == "P":
                mrows[arg] = proj(arg)
            elif op == "S":
                recip[arg] = scores(arg, mrows[arg])
            elif op == "V":
                values(arg, mrows[arg], recip[arg])
            elif op == "O":
                oproj(arg)
            elif op == "I":
                conv_inv(ct - 1, cj)
            else:
                assert not queue
                conv_fwd(ct + 1, cj)
        return wrap(wr0 + XR)

    def two_steps(it, carry):
        wr0, rdi = carry
        for u in range(2):
            wr0 = step(it, u, wr0, rdi)

        @pl.when(it == 0)
        def _():
            for c in range(2, NC):
                for cp in conv_copies(c):
                    cp.start()

        @pl.when(it == 3)
        def _():
            for c in range(2, NC):
                for cp in conv_copies(c):
                    cp.wait()
        return wr0, jnp.where(rdi == RING // (2 * SEG) - 1, 0, rdi + 1)
    jax.lax.fori_loop(0, NSEG // 2, two_steps, (PRE, 0))

    for j in range(NB // 2):
        conv_inv(NC - 1, j)

    def out_copies(r0, n):
        return [pltpu.make_async_copy(outb.at[c + 1, pl.ds(r0, n), :],
                                      out_hbm.at[pl.ds(r0, n), pl.ds(c * 128, 128)], sems.at[4])
                for c in range(NC)]

    for cp in out_copies(0, S - PRE):
        cp.start()

    def post_chunk(i, carry):
        rows = pl.ds(pl.multiple_of(S - PRE + i * MB, MB), MB)
        op = jnp.concatenate([obuf[hh, rows, :] for hh in range(H)], axis=1)
        omg = 1.0 - gbuf[rows, :]
        for n in range(NC):
            w = jnp.concatenate([wos[4 * n + kq] for kq in range(4)], axis=0)
            y = _dot(op, pltpu.bitcast(w, BF16))
            accumulate(n + 1, rows, omg * y.astype(BF16).astype(F32))
        for cp in out_copies(pl.multiple_of(S - PRE + i * MB, MB), MB):
            cp.start()
        return carry
    jax.lax.fori_loop(0, PRE // MB, post_chunk, 0)
    for cp in out_copies(0, S - PRE):
        cp.wait()
    for i in range(PRE // MB):
        for cp in out_copies(S - PRE + i * MB, MB):
            cp.wait()


@functools.partial(jax.jit, static_argnames=("B_seg_len",))
def pallas_gated_mix__ssm_conv_h3__memory_aug_recurrent_mem_tr__prompt_kernel(
    A_q, A_k, A_v, A_shift_k, A_ssm_k, A_ssm_D, B_x, B_mem0, B_Wq, B_Wk, B_Wv, B_Wo,
    B_seg_len, gate_w,
):
    del B_x
    assert B_seg_len == SEG and A_q.shape == (1, S, D) and B_Wq.shape == (D, H, DH)
    assert A_shift_k.shape == (D, KS) and B_mem0.shape == (1, MEM, D)
    fwd, inv = _dft_tables()
    hbm = pl.BlockSpec(memory_space=pl.ANY)
    out = pl.pallas_call(
        _kernel,
        out_shape=jax.ShapeDtypeStruct((S, D), BF16),
        in_specs=[hbm] * 14,
        out_specs=hbm,
        scratch_shapes=[
            pltpu.VMEM((NC, S, 128), BF16),
            pltpu.VMEM((NC, 64 + S, 128), BF16),
            pltpu.VMEM((NC + 2, S, 128), BF16),
            pltpu.VMEM((NC, 128, S), BF16),
            pltpu.VMEM((3, D, 8, 128), BF16),
            pltpu.VMEM((3 * H, D // 2, 128), U32),
            pltpu.VMEM((4 * NC, D // 2, 128), U32),
            pltpu.VMEM((24, RING, 128), BF16),
            pltpu.VMEM((24, RING, 128), BF16),
            pltpu.VMEM((24, RING, 128), BF16),
            pltpu.VMEM((24, RING, 128), BF16),
            pltpu.VMEM((H, S, 128), BF16),
            pltpu.VMEM((NC + 1, S, 128), BF16),
            pltpu.VMEM((H, MEM + XR, 128), BF16),
            pltpu.VMEM((NC, MEM + XR, 128), F32),
            pltpu.VMEM((MEM, D), F32),
            pltpu.VMEM((96, 128), F32),
            pltpu.VMEM((288, 128), F32),
            pltpu.VMEM((2, 160, 128), F32),
            pltpu.VMEM((1, 96, 128), F32),
            pltpu.VMEM((H // 2, 64, NR), U32),
            pltpu.VMEM((16, 1024, 128), F32),
            pltpu.VMEM((2 * NB * CB, 128), U32),
            pltpu.VMEM((S, 128), F32),
            pltpu.VMEM((2 * CB, CB), BF16),
            pltpu.VMEM((CB, 2 * CB), BF16),
            pltpu.VMEM((MEM, D), BF16),
            pltpu.VMEM((NC, KS, 128), BF16),
            pltpu.VMEM((NC, 128), BF16),
            pltpu.VMEM((NC, 128), BF16),
            pltpu.SemaphoreType.DMA((11,)),
            pltpu.SemaphoreType.DMA((3,)),
        ],
        compiler_params=pltpu.CompilerParams(vmem_limit_bytes=120 * 1024 * 1024),
    )(
        A_q.reshape(S, D), A_k.reshape(S, D), A_v.reshape(S, D), A_ssm_k,
        B_Wq, B_Wk, B_Wv, B_Wo.reshape(H * DH, D),
        A_shift_k.T.reshape(KS, NC, 128).transpose(1, 0, 2),
        A_ssm_D.reshape(NC, 128), gate_w.reshape(NC, 128),
        B_mem0.reshape(MEM, D),
        jnp.asarray(fwd, BF16), jnp.asarray(inv, BF16),
    )
    return out.reshape(1, S, D)
```

```python
import functools

import jax
import jax.numpy as jnp
import numpy as np
import jax.experimental.pallas as pl
import jax.experimental.pallas.tpu as pltpu

F32 = jnp.float32
BF16 = jnp.bfloat16
U32 = jnp.uint32
I32 = jnp.int32

S = 2048
D = 1024
NC = D // 128
H = 32
DH = 128
MEM = 8
SEG = 32
NSEG = S // SEG
XR = 24
PRE = S - NSEG * XR
TL = SEG - XR
NR = 2 * (SEG + MEM)
CB = 128
NB = S // CB
KS = 4
KPAD = 16
MB = 128
SST = 9
MAC_G = 3


def _expand(text):
    out = []
    for item in text.split():
        if "-" in item:
            a, b = item[1:].split("-")
            out += [(item[0], i) for i in range(int(a), int(b) + 1)]
        else:
            out.append((item[0], int(item[1:] or 0)))
    return out


PROGRAM = _expand("P0-4 S0-3 P5-8 V0-3 S4-7 P9-10 O0 P11-12 V4-7 S8-11 P13 O1 P14-15 "
                  "O2 V8-11 S12-15 O3 O4 V12-15 O5 O6 O7 I F")


def _dft_tables():
    f = np.concatenate([np.arange(0, CB, 2), np.arange(1, CB, 2)]).astype(np.float64)
    t = np.arange(CB, dtype=np.float64)
    ang = 2.0 * np.pi * (f[:, None] + 0.5) * t[None, :] / (2 * CB)
    fwd = np.concatenate([np.cos(ang), -np.sin(ang)], axis=0)
    inv = np.concatenate([np.cos(ang).T, -np.sin(ang).T], axis=1) / CB
    return fwd, inv


def _dot(a, b):
    return jnp.dot(a, b, preferred_element_type=F32)


def _dot_nt(a, b):
    return jax.lax.dot_general(a, b, (((1,), (1,)), ((), ())), preferred_element_type=F32)


def _mo(x, m):
    return x if isinstance(x, int) else pl.multiple_of(x, m)


def _tie(x, gate):
    return x if gate is None else pltpu.bitcast(pltpu.bitcast(x, I32) | gate, x.dtype)


def _gate(token, zero):
    return pltpu.bitcast(token, I32) & jnp.full((8, 128), zero, I32)


def _zero_of(counter):
    return jax.lax.shift_right_logical(counter, 16)


def _kernel(x_hbm, x3_hbm, k_hbm, v_hbm, ssm_hbm, wq_hbm, wk_hbm, wv_hbm, wo_hbm,
            shift_hbm, dskip_hbm, gate_hbm, mem0_hbm, fwd_hbm, inv_hbm,
            out_hbm,
            xs, xpre, ks, vs, ssm, wraw, wts, wos, wpark, prebuf, yb0, yb1, yb2, yb3, obuf, outb, olhs, oacc,
            mem, small, kf, stage, fbuf, ebuf, spec, zspec, gbuf,
            fwd_ref, inv_ref, mem0_ref, shift_ref, dskip_ref, gate_ref,
            sems, sem_w):
    w_hbm = (wq_hbm, wk_hbm, wv_hbm)
    ybufs = (yb0, yb1, yb2, yb3)

    def x_copy(c):
        return pltpu.make_async_copy(x_hbm.at[:, pl.ds(_mo(c * 128, 128), 128)], xs.at[c], sems.at[1])

    def xt_copy(c, part):
        s0, n, si = ((0, 16, 0), (16, NSEG - 16, 10))[part]
        return pltpu.make_async_copy(x3_hbm.at[pl.ds(s0, n), pl.ds(XR, TL), pl.ds(c * 128, 128)],
                                     xpre.at[c, pl.ds(s0, n)], sems.at[si])

    def conv_copies(c):
        col = pl.ds(c * 128, 128)
        sem = sems.at[2 if c < 2 else 3]
        return [pltpu.make_async_copy(k_hbm.at[:, col], ks.at[c, pl.ds(KPAD, S), :], sem),
                pltpu.make_async_copy(v_hbm.at[:, col], vs.at[c + 1], sem),
                pltpu.make_async_copy(ssm_hbm.at[col, :], ssm.at[c], sem)]

    def wo_copy(c):
        return pltpu.make_async_copy(wo_hbm.at[:, pl.ds(_mo(c * 128, 128), 128)], wpark.at[c], sems.at[1])

    def w_copy(t, g, slot):
        return pltpu.make_async_copy(w_hbm[t].at[:, pl.ds(_mo(g * 8, 8), 8), :], wraw.at[slot], sem_w.at[slot])

    def w0_copy(i):
        return pltpu.make_async_copy(wq_hbm.at[pl.ds(i * 256, 256), pl.ds(0, 8), :],
                                     wraw.at[0, pl.ds(i * 256, 256)], sems.at[5 + i])

    small_copies = [pltpu.make_async_copy(a, b, sems.at[9]) for a, b in (
        (shift_hbm, shift_ref), (dskip_hbm, dskip_ref), (gate_hbm, gate_ref),
        (mem0_hbm, mem0_ref), (fwd_hbm, fwd_ref), (inv_hbm, inv_ref))]

    def background(c):
        wo_copy(c).start()
        x_copy(c).start()

    for i in range(4):
        w0_copy(i).start()
    for c in range(NC):
        xt_copy(c, 0).start()

    vs[0] = jnp.zeros((S, 128), BF16)
    outb[0] = jnp.zeros((NSEG, SEG, 128), BF16)
    zspec[NB * CB:2 * NB * CB, :] = jnp.zeros((NB * CB, 128), U32)

    def clear(c, count):
        ks[c, 0:KPAD, :] = jnp.zeros((KPAD, 128), BF16)
        outb[c + 1] = jnp.zeros((NSEG, SEG, 128), BF16)
        return count + 1

    def relayout_piece(c, slot, q, gate=None):
        st = stage.at[q % 2]
        blk = wraw[slot, q * 16:(q + 1) * 16].astype(F32)
        for i in range(16):
            st[i * SST:i * SST + 8, :] = _tie(blk[i], gate if i % 8 == 0 else None)
        for j in range(8):
            wts[c * 8 + j, q * 8:(q + 1) * 8, :] = pltpu.bitcast(
                st[pl.ds(j, 16, stride=SST), :].astype(BF16), U32)

    def relayout_with(y, zero, c, slot, d, span):
        qs = range(min(64 * d // span, 64), min(64 * (d + 1) // span, 64))
        for i, q in enumerate(qs):
            o = (i * MB // len(qs)) // 8 * 8
            relayout_piece(c, slot, q, _gate(y[o:o + 8], zero))

    pend = [None]

    def pre_mm(c, d):
        pp, rb, hb = d // 8, (d // 2) % 4, d % 2
        w = pltpu.bitcast(wts[c * 8 + (2 * pp + hb)], BF16)
        xp = jnp.concatenate([xpre[cc, rb * 16:(rb + 1) * 16].reshape(MB, 128) for cc in range(NC)], axis=1)
        y = _dot(xp, w)
        if hb == 0:
            pend[0] = y
        else:
            for i in range(16):
                pair = jnp.concatenate([pend[0][8 * i:8 * i + 8], y[8 * i:8 * i + 8]], axis=0)
                prebuf[rb * 16 + i, pl.ds(_mo(c * 32 + pp * 8, 8), 8), :] = pltpu.bitcast(pair.astype(BF16), U32)
        return y

    count = 0
    for i in range(4):
        count = jax.lax.fori_loop(2 * i, 2 * i + 2, clear, count)
        w0_copy(i).wait()
        if i == 0:
            for c in range(NC):
                xt_copy(c, 1).start()
        if i == 1:
            for t in range(1, 3):
                w_copy(t, 0, t).start()
        for q in range(16 * i, 16 * i + 16):
            relayout_piece(0, 0, q)
    w_copy(0, 1, 0).start()
    for cp in small_copies:
        cp.start()
    for c in range(NC):
        xt_copy(c, 0).wait()

    for e in range(32):
        if e == 8:
            for c in range(NC):
                xt_copy(c, 1).wait()
        if e == 24:
            w_copy(1, 0, 1).wait()
        y = pre_mm(0, ((e % 8) // 2) * 8 + (e // 8) * 2 + e % 2)
        if e >= 24:
            relayout_with(y, _zero_of(count), 1, 1, e - 24, 7)
    w_copy(1, 1, 1).start()
    background(0)

    def pre_chunk(c, carry, pack):
        tn, gn = carry
        zero = _zero_of(tn)
        w_copy(0, 0, tn).wait()
        for d in range(32):
            y = pre_mm(c, d)
            relayout_with(y, zero, c + 1, tn, d, 31)
            if pack:
                for i in range(2):
                    gate = _gate(y[64 * i + 32:64 * i + 40], zero)
                    for r in range((d % 2) * 256 + i * 128, (d % 2) * 256 + (i + 1) * 128, 8):
                        o = ((d // 2) % 4) * 1024 + 2 * r
                        wos[(c - 9) * 16 + d // 2, r:r + 8, :] = _tie(
                            pltpu.bitcast(wpark[(c - 9) * 4 + d // 8, o:o + 16, :], U32), gate)
        if not pack:
            for t in range(3):
                @pl.when(jnp.logical_and(tn == t, gn < 3))
                def _():
                    w_copy(t, gn + 1, t).start()

            @pl.when(c < NC)
            def _():
                background(c)

            @pl.when(c == NC)
            def _():
                for cp in conv_copies(0) + conv_copies(1):
                    cp.start()
        return jnp.where(tn == 2, 0, tn + 1), jnp.where(tn == 2, gn + 1, gn)

    carry = jax.lax.fori_loop(1, 9, functools.partial(pre_chunk, pack=False), (2, 0))
    for c in range(NC):
        wo_copy(c).wait()
        x_copy(c).wait()
    count = jax.lax.fori_loop(9, 11, functools.partial(pre_chunk, pack=True), carry)[1]

    for cp in small_copies:
        cp.wait()
    for cp in conv_copies(0) + conv_copies(1):
        cp.wait()
    small[0:NC, :] = dskip_ref[...].astype(F32)
    gate_w = gate_ref[...].astype(F32)
    for c in range(NC):
        small[NC + 8 * c:NC + 8 * (c + 1), :] = jnp.broadcast_to(gate_w[c:c + 1, :], (8, 128))
    mem[...] = mem0_ref[...].astype(F32)

    def mix_gate(r0, gate):
        z = None
        for c in range(NC):
            gw = small[NC + 8 * c:NC + 8 * (c + 1), :]
            t = xs[c, r0:r0 + 16, :].astype(F32) * jnp.concatenate([gw, gw], axis=0)
            z = _tie(t, jnp.concatenate([gate, gate], axis=0)) if z is None else z + t
        z = jnp.sum(z, axis=1, keepdims=True)
        gbuf[r0 // SEG, r0 % SEG:r0 % SEG + 16, :] = jnp.broadcast_to(0.5 * jnp.tanh(0.5 * z) + 0.5, (16, 128))

    def accumulate(slab, segs, rows, val):
        old = outb[slab, segs, rows, :].astype(F32)
        outb[slab, segs, rows, :] = (old + val.astype(BF16).astype(F32).reshape(old.shape)).astype(BF16)

    def conv_prep(t, j):
        tr = t if isinstance(t, int) else jnp.minimum(t, NC - 1)
        r0 = _mo(j * 2 * CB, 2 * CB)
        shift = shift_ref[tr].astype(F32)
        gate = yield
        for o in range(0, 2 * CB + KPAD, 16):
            kk = ks[tr, pl.ds(_mo(r0 + o, 16), 16), :].astype(F32)
            kf[o:o + 8, :] = _tie(kk[0:8], gate)
            kf[o + 8:o + 16, :] = _tie(kk[8:16], gate)
            if o == 0:
                continue
            acc = kf[o:o + 16, :] * shift[0:1, :]
            for l in range(1, KS):
                acc = acc + kf[o - l:o - l + 16, :] * shift[l:l + 1, :]
            rows = pl.ds(_mo(r0 + (o - KPAD), 16), 16)
            vs[t + 1, rows, :] = (acc * vs[tr + 1, rows, :].astype(F32)).astype(BF16)
            gate = yield

    def conv_fwd(t, j):
        tr = t if isinstance(t, int) else jnp.minimum(t, NC - 1)
        slot = t & 1
        fwd = fwd_ref[...]
        for i in range(2):
            rows = pl.ds(_mo((2 * j + i) * CB, CB), CB)
            sr = _mo((2 * j + i) * 32, 32)
            for off, res in ((0, _dot(fwd, vs[t + 1, rows, :])), (512, _dot_nt(fwd, ssm[tr, :, rows]))):
                for ri in range(2):
                    for fj in range(8):
                        spec[slot * 8 + fj, pl.ds(sr + (off + ri * 16), 16), :] = (
                            res[ri * CB + fj * 16:ri * CB + (fj + 1) * 16])

    def conv_mac(t, j, zero):
        slot = t & 1
        sign = jnp.where(j < 4, 1.0, -1.0).astype(F32)
        zbase = pl.multiple_of(slot * (NB * CB) + j * 8, 8)
        prev = None
        gate = yield
        for i in range(NB):
            base = slot * 8 + j + zero * (i + 1)
            ys = []
            for hv in range(2):
                yr = yi = None
                for jj in range(i + 1):
                    uo = jj * 32 + hv * 8
                    ko = 512 + (i - jj) * 32 + hv * 8
                    ur = spec[base, uo:uo + 8, :]
                    ui = spec[base, uo + 16:uo + 24, :]
                    kr = spec[base, ko:ko + 8, :]
                    ki = spec[base, ko + 16:ko + 24, :]
                    tr, ti = _tie(ur * kr - ui * ki, gate), _tie(ur * ki + ui * kr, gate)
                    yr, yi = (tr, ti) if yr is None else (yr + tr, yi + ti)
                    if jj < i or hv == 0:
                        gate = yield
                ys.append((yr, yi))
            yr = jnp.concatenate([ys[0][0], ys[1][0]], axis=0)
            yi = jnp.concatenate([ys[0][1], ys[1][1]], axis=0)
            zr, zi = (yr, yi) if prev is None else (yr - sign * prev[1], yi + sign * prev[0])
            prev = (yr, yi)
            zspec[pl.ds(zbase + i * CB, 8), :] = pltpu.bitcast(zr.astype(BF16), U32)
            zspec[pl.ds(zbase + (i * CB + CB // 2), 8), :] = pltpu.bitcast(zi.astype(BF16), U32)
            gate = yield

    def conv_inv(t, j):
        tr = t if isinstance(t, int) else jnp.maximum(t, 0)
        slot = t & 1
        dsk = small[pl.ds(tr, 1), :]
        inv = inv_ref[...]
        for i in range(2):
            rows = pl.ds(_mo((2 * j + i) * CB, CB), CB)
            z = zspec[pl.ds(_mo((slot * NB + 2 * j + i) * CB, CB), CB), :]
            y = _dot(inv, pltpu.bitcast(z, BF16))
            y = y + vs[t + 1, rows, :].astype(F32) * dsk
            segs = pl.ds((2 * j + i) * (CB // SEG), CB // SEG)
            accumulate(t + 1, segs, slice(None), gbuf[segs].reshape(CB, 128) * (xs[tr, rows, :].astype(F32) * y))

    for q in range(32):
        if q % 4 == 0:
            preps = conv_prep(0, q // 4)
            next(preps)
        y = pre_mm(11, q)
        if q % 4 == 1 and q >= 4:
            conv_fwd(0, q // 4 - 1)
        for i in range(4):
            gate = _gate(y[32 * i:32 * i + 8], _zero_of(count))
            preps.send(gate)
            mix_gate(q * 64 + i * 16, gate)
    conv_fwd(0, NB // 2 - 1)

    ri = jax.lax.broadcasted_iota(I32, (NR, NR), 0)
    ci = jax.lax.broadcasted_iota(I32, (NR, NR), 1)
    LD = MEM + XR

    def head_pos(i):
        tail = i >= 2 * LD
        return (jnp.where(tail, (i - 2 * LD) // TL, i // LD),
                jnp.where(tail, LD + (i - 2 * LD) % TL, i % LD))
    (rh, rp), (ch, cp_) = head_pos(ri), head_pos(ci)
    same = rh == ch
    keep = same & ((rp < MEM) | (rp >= cp_))
    fbuf[0, 0:NR, 0:NR] = jnp.where(keep, 0.0, jnp.where(same, -1000000000.0, -jnp.inf)).astype(F32)
    scale = float(DH) ** -0.5

    def step(it, u, zero):
        s = it * 2 + u
        ct = jax.lax.shift_right_logical(s, 3)
        cj = jnp.bitwise_and(s, 7)
        xr0 = pl.multiple_of(it * (2 * SEG) + u * SEG, SEG)
        h_lhs = jnp.concatenate(
            [jnp.concatenate([mem[:, c * 128:(c + 1) * 128], xs[c, pl.ds(xr0, XR), :].astype(F32)],
                             axis=0).astype(BF16) for c in range(NC)], axis=1)

        macs = conv_mac(ct, cj, zero)
        next(macs)
        preps = conv_prep(ct + 1, cj)
        next(preps)
        n_mac = NB * (NB + 1)
        queue = [(preps, 1)] * 16 + [(macs, min(MAC_G, n_mac - n)) for n in range(0, n_mac, MAC_G)]

        def side_work(token):
            if queue:
                gen, cnt = queue.pop(0)
                gen.send(_gate(token, zero))
                for _ in range(cnt - 1):
                    gen.send(None)

        def proj(p):
            for t in range(3):
                for i, hh in enumerate((2 * p, 2 * p + 1)):
                    y = _dot(h_lhs, pltpu.bitcast(wts[(hh // 8) * 24 + t * 8 + hh % 8], BF16))
                    side_work(y[0:MEM])
                    ybufs[p // 4][t * 4 + p % 4 + zero, i * 16:(i + 1) * 16, :] = pltpu.bitcast(y.astype(BF16), U32)

        def rows_of(t, p):
            o = ((p // 4) * 12 + t * 4 + p % 4) * 8
            return pltpu.bitcast(jnp.concatenate([ybufs[p // 4][t * 4 + p % 4], prebuf[s, o:o + 8, :]], axis=0), BF16)

        def scores(p):
            sc = _dot_nt(rows_of(0, p), rows_of(1, p)) * scale
            fill = fbuf[zero * (p + 1), 0:NR, 0:NR]
            sc = jnp.where(fill == 0.0, sc, fill)
            e = jnp.exp(sc - jnp.max(sc, axis=1, keepdims=True))
            l = jnp.sum(e, axis=1, keepdims=True)
            r = pl.reciprocal(l, approx=True)
            ebuf[p + zero, 0:NR // 2, :] = pltpu.bitcast(e.astype(BF16), U32)
            return r * (2.0 - l * r)

        def values(p, r):
            o = _dot(pltpu.bitcast(ebuf[p, 0:NR // 2, :], BF16), rows_of(2, p)) * r
            for i, hh in enumerate((2 * p, 2 * p + 1)):
                olhs[hh] = pltpu.bitcast(o[i * LD:(i + 1) * LD].astype(BF16), U32)
                obuf[hh, pl.ds(pl.multiple_of(s * TL, TL), TL), :] = (
                    o[2 * LD + i * TL:2 * LD + (i + 1) * TL].astype(BF16))

        def oproj(g):
            lhs = pltpu.bitcast(jnp.concatenate([olhs[hh] for hh in range(4 * g, 4 * g + 4)], axis=1), BF16)
            for n in range(NC):
                w = wos[4 * n + g // 2, (g % 2) * 256:(g % 2 + 1) * 256, :]
                y = _dot(lhs, pltpu.bitcast(w, BF16))
                side_work(y[0:MEM])
                if g > 0:
                    y = y + oacc[n + zero]
                if g < H // 4 - 1:
                    oacc[n] = y
                else:
                    mem[:, n * 128:(n + 1) * 128] = y[0:MEM].astype(BF16).astype(F32)
                    accumulate(n + 1, s, slice(0, XR),
                               (1.0 - gbuf[s, 0:XR, :]) * y[MEM:].astype(BF16).astype(F32))

        recip = [None] * (H // 2)
        for op, arg in PROGRAM:
            if op == "P":
                proj(arg)
            elif op == "S":
                recip[arg] = scores(arg)
            elif op == "V":
                values(arg, recip[arg])
            elif op == "O":
                oproj(arg)
            elif op == "I":
                conv_inv(ct - 1, cj)
            else:
                assert not queue
                conv_fwd(ct + 1, cj)

    def two_steps(it, carry):
        for u in range(2):
            step(it, u, _zero_of(carry))

        @pl.when(it == 0)
        def _():
            for c in range(2, NC):
                for cp in conv_copies(c):
                    cp.start()

        @pl.when(it == 3)
        def _():
            for c in range(2, NC):
                for cp in conv_copies(c):
                    cp.wait()
        return carry + 1
    jax.lax.fori_loop(0, NSEG // 2, two_steps, count)

    for j in range(NB // 2):
        conv_inv(NC - 1, j)

    def out_copies(s0, n, r0, nr):
        return [pltpu.make_async_copy(outb.at[c + 1, pl.ds(s0, n), pl.ds(r0, nr), :],
                                      out_hbm.at[pl.ds(s0, n), pl.ds(r0, nr), pl.ds(c * 128, 128)], sems.at[4])
                for c in range(NC)]

    for cp in out_copies(0, NSEG, 0, XR):
        cp.start()

    def post_chunk(i, carry):
        rows = pl.ds(pl.multiple_of(i * MB, MB), MB)
        segs = pl.ds(i * 16, 16)
        op = jnp.concatenate([obuf[hh, rows, :] for hh in range(H)], axis=1)
        omg = 1.0 - gbuf[segs, XR:SEG, :].reshape(MB, 128)
        for n in range(NC):
            w = jnp.concatenate([wos[4 * n + kq] for kq in range(4)], axis=0)
            y = _dot(op, pltpu.bitcast(w, BF16))
            accumulate(n + 1, segs, slice(XR, SEG), omg * y.astype(BF16).astype(F32))
        for cp in out_copies(i * 16, 16, XR, TL):
            cp.start()
        return carry
    jax.lax.fori_loop(0, PRE // MB, post_chunk, 0)
    for cp in out_copies(0, NSEG, 0, XR):
        cp.wait()
    for i in range(PRE // MB):
        for cp in out_copies(i * 16, 16, XR, TL):
            cp.wait()


@functools.partial(jax.jit, static_argnames=("B_seg_len",))
def pallas_gated_mix__ssm_conv_h3__memory_aug_recurrent_mem_tr__prompt_kernel(
    A_q, A_k, A_v, A_shift_k, A_ssm_k, A_ssm_D, B_x, B_mem0, B_Wq, B_Wk, B_Wv, B_Wo,
    B_seg_len, gate_w,
):
    del B_x
    assert B_seg_len == SEG and A_q.shape == (1, S, D) and B_Wq.shape == (D, H, DH)
    assert A_shift_k.shape == (D, KS) and B_mem0.shape == (1, MEM, D)
    fwd, inv = _dft_tables()
    hbm = pl.BlockSpec(memory_space=pl.ANY)
    out = pl.pallas_call(
        _kernel,
        out_shape=jax.ShapeDtypeStruct((NSEG, SEG, D), BF16),
        in_specs=[hbm] * 15,
        out_specs=hbm,
        scratch_shapes=[
            pltpu.VMEM((NC, S, 128), BF16),
            pltpu.VMEM((NC, NSEG, TL, 128), BF16),
            pltpu.VMEM((NC, 64 + S, 128), BF16),
            pltpu.VMEM((NC + 2, S, 128), BF16),
            pltpu.VMEM((NC, 128, S), BF16),
            pltpu.VMEM((3, D, 8, 128), BF16),
            pltpu.VMEM((3 * H, D // 2, 128), U32),
            pltpu.VMEM((4 * NC, D // 2, 128), U32),
            pltpu.VMEM((NC, H * DH, 128), BF16),
            pltpu.VMEM((NSEG, 3 * H // 2 * 8, 128), U32),
            pltpu.VMEM((12, 32, 128), U32),
            pltpu.VMEM((12, 32, 128), U32),
            pltpu.VMEM((12, 32, 128), U32),
            pltpu.VMEM((12, 32, 128), U32),
            pltpu.VMEM((H, PRE, 128), BF16),
            pltpu.VMEM((NC + 1, NSEG, SEG, 128), BF16),
            pltpu.VMEM((H, 16, 128), U32),
            pltpu.VMEM((NC, MEM + XR, 128), F32),
            pltpu.VMEM((MEM, D), F32),
            pltpu.VMEM((96, 128), F32),
            pltpu.VMEM((288, 128), F32),
            pltpu.VMEM((2, 160, 128), F32),
            pltpu.VMEM((1, 96, 128), F32),
            pltpu.VMEM((H // 2, 64, NR), U32),
            pltpu.VMEM((16, 1024, 128), F32),
            pltpu.VMEM((2 * NB * CB, 128), U32),
            pltpu.VMEM((NSEG, SEG, 128), F32),
            pltpu.VMEM((2 * CB, CB), BF16),
            pltpu.VMEM((CB, 2 * CB), BF16),
            pltpu.VMEM((MEM, D), BF16),
            pltpu.VMEM((NC, KS, 128), BF16),
            pltpu.VMEM((NC, 128), BF16),
            pltpu.VMEM((NC, 128), BF16),
            pltpu.SemaphoreType.DMA((11,)),
            pltpu.SemaphoreType.DMA((3,)),
        ],
        compiler_params=pltpu.CompilerParams(vmem_limit_bytes=120 * 1024 * 1024, disable_bounds_checks=True, disable_semaphore_checks=True),
    )(
        A_q.reshape(S, D), A_q.reshape(NSEG, SEG, D), A_k.reshape(S, D), A_v.reshape(S, D), A_ssm_k,
        B_Wq, B_Wk, B_Wv, B_Wo.reshape(H * DH, D),
        A_shift_k.T.reshape(KS, NC, 128).transpose(1, 0, 2),
        A_ssm_D.reshape(NC, 128), gate_w.reshape(NC, 128),
        B_mem0.reshape(MEM, D),
        jnp.asarray(fwd, BF16), jnp.asarray(inv, BF16),
    )
    return out.reshape(1, S, D)
```

```python
import functools

import jax
import jax.numpy as jnp
import numpy as np
import jax.experimental.pallas as pl
import jax.experimental.pallas.tpu as pltpu

F32 = jnp.float32
BF16 = jnp.bfloat16
U32 = jnp.uint32
I32 = jnp.int32

S = 2048
D = 1024
NC = D // 128
H = 32
DH = 128
MEM = 8
SEG = 32
NSEG = S // SEG
XR = 24
PRE = S - NSEG * XR
TL = SEG - XR
NR = 2 * (SEG + MEM)
CB = 128
NB = S // CB
KS = 4
KPAD = 16
MB = 128
SST = 9
MAC_G = 3


def _expand(text):
    out = []
    for item in text.split():
        if "-" in item:
            a, b = item[1:].split("-")
            out += [(item[0], i) for i in range(int(a), int(b) + 1)]
        else:
            out.append((item[0], int(item[1:] or 0)))
    return out


PROGRAM = _expand("P0-4 S0-3 P5-8 V0-3 S4-7 P9-10 O0 P11-12 V4-7 S8-11 P13 O1 P14-15 "
                  "O2 V8-11 S12-15 O3 O4 V12-15 O5 O6 O7 I F")


def _dft_tables():
    f = np.concatenate([np.arange(0, CB, 2), np.arange(1, CB, 2)]).astype(np.float64)
    t = np.arange(CB, dtype=np.float64)
    ang = 2.0 * np.pi * (f[:, None] + 0.5) * t[None, :] / (2 * CB)
    fwd = np.concatenate([np.cos(ang), -np.sin(ang)], axis=0)
    inv = np.concatenate([np.cos(ang).T, -np.sin(ang).T], axis=1) / CB
    return fwd, inv


def _dot(a, b):
    return jnp.dot(a, b, preferred_element_type=F32)


def _dot_nt(a, b):
    return jax.lax.dot_general(a, b, (((1,), (1,)), ((), ())), preferred_element_type=F32)


def _mo(x, m):
    return x if isinstance(x, int) else pl.multiple_of(x, m)


def _tie(x, gate):
    return x if gate is None else pltpu.bitcast(pltpu.bitcast(x, I32) | gate, x.dtype)


def _gate(token, zero):
    return pltpu.bitcast(token, I32) & jnp.full((8, 128), zero, I32)


def _zero_of(counter):
    return jax.lax.shift_right_logical(counter, 16)


def _kernel(x_hbm, x3_hbm, k_hbm, v_hbm, ssm_hbm, wq_hbm, wk_hbm, wv_hbm, wo_hbm,
            shift_hbm, dskip_hbm, gate_hbm, mem0_hbm, fwd_hbm, inv_hbm,
            out_hbm,
            xs, xpre, xpk, ks, vs, ssm, wraw, wts, wos, wpark, prebuf, yb0, yb1, yb2, yb3, obuf, outb, olhs, oacc,
            mem, small, kf, stage, fbuf, ebuf, spec, zspec, gbuf,
            fwd_ref, inv_ref, mem0_ref, shift_ref, dskip_ref, gate_ref,
            sems, sem_w):
    w_hbm = (wq_hbm, wk_hbm, wv_hbm)
    ybufs = (yb0, yb1, yb2, yb3)

    def x_copy(c):
        return pltpu.make_async_copy(x_hbm.at[:, pl.ds(_mo(c * 128, 128), 128)], xs.at[c], sems.at[1])

    def xt_copy(c, part):
        s0, n, si = ((0, 16, 0), (16, NSEG - 16, 10))[part]
        return pltpu.make_async_copy(x3_hbm.at[pl.ds(s0, n), pl.ds(XR, TL), pl.ds(c * 128, 128)],
                                     xpre.at[c, pl.ds(s0, n)], sems.at[si])

    def conv_copies(c):
        col = pl.ds(c * 128, 128)
        sem = sems.at[2 if c < 2 else 3]
        return [pltpu.make_async_copy(k_hbm.at[:, col], ks.at[c, pl.ds(KPAD, S), :], sem),
                pltpu.make_async_copy(v_hbm.at[:, col], vs.at[c + 1], sem),
                pltpu.make_async_copy(ssm_hbm.at[col, :], ssm.at[c], sem)]

    def wo_copy(c):
        return pltpu.make_async_copy(wo_hbm.at[:, pl.ds(_mo(c * 128, 128), 128)], wpark.at[c], sems.at[1])

    def w_copy(t, g, slot):
        return pltpu.make_async_copy(w_hbm[t].at[:, pl.ds(_mo(g * 8, 8), 8), :], wraw.at[slot], sem_w.at[slot])

    def w0_copy(i):
        return pltpu.make_async_copy(wq_hbm.at[pl.ds(i * 256, 256), pl.ds(0, 8), :],
                                     wraw.at[0, pl.ds(i * 256, 256)], sems.at[5 + i])

    small_copies = [pltpu.make_async_copy(a, b, sems.at[9]) for a, b in (
        (shift_hbm, shift_ref), (dskip_hbm, dskip_ref), (gate_hbm, gate_ref),
        (mem0_hbm, mem0_ref), (fwd_hbm, fwd_ref), (inv_hbm, inv_ref))]

    def background(c):
        wo_copy(c).start()
        x_copy(c).start()

    for i in range(4):
        w0_copy(i).start()
    for c in range(NC):
        xt_copy(c, 0).start()

    vs[0] = jnp.zeros((S, 128), BF16)
    outb[0] = jnp.zeros((NSEG, SEG, 128), BF16)
    zspec[NB * CB:2 * NB * CB, :] = jnp.zeros((NB * CB, 128), U32)

    def clear(c, count):
        ks[c, 0:KPAD, :] = jnp.zeros((KPAD, 128), BF16)
        outb[c + 1] = jnp.zeros((NSEG, SEG, 128), BF16)
        return count + 1

    def relayout_piece(c, slot, q, gate=None):
        st = stage.at[q % 2]
        blk = wraw[slot, q * 16:(q + 1) * 16].astype(F32)
        for i in range(16):
            st[i * SST:i * SST + 8, :] = _tie(blk[i], gate if i % 8 == 0 else None)
        for j in range(8):
            wts[c * 8 + j, q * 8:(q + 1) * 8, :] = pltpu.bitcast(
                st[pl.ds(j, 16, stride=SST), :].astype(BF16), U32)

    def relayout_with(y, zero, c, slot, d, span):
        qs = range(min(64 * d // span, 64), min(64 * (d + 1) // span, 64))
        for i, q in enumerate(qs):
            o = (i * MB // len(qs)) // 8 * 8
            relayout_piece(c, slot, q, _gate(y[o:o + 8], zero))

    pend = [None]

    def pre_mm(c, d, packed=True):
        pp, rb, hb = d // 8, (d // 2) % 4, d % 2
        w = pltpu.bitcast(wts[c * 8 + (2 * pp + hb)], BF16)
        if packed:
            xp = pltpu.bitcast(jnp.concatenate([xpk[cc, rb * 64:(rb + 1) * 64, :] for cc in range(NC)], axis=1), BF16)
        else:
            xp = jnp.concatenate([xpre[cc, rb * 16:(rb + 1) * 16].reshape(MB, 128) for cc in range(NC)], axis=1)
        y = _dot(xp, w)
        if hb == 0:
            pend[0] = y
        else:
            for i in range(16):
                pair = jnp.concatenate([pend[0][8 * i:8 * i + 8], y[8 * i:8 * i + 8]], axis=0)
                prebuf[rb * 16 + i, pl.ds(_mo(c * 32 + pp * 8, 8), 8), :] = pltpu.bitcast(pair.astype(BF16), U32)
        return y

    count = 0
    for i in range(4):
        count = jax.lax.fori_loop(2 * i, 2 * i + 2, clear, count)
        w0_copy(i).wait()
        if i == 0:
            for c in range(NC):
                xt_copy(c, 1).start()
        if i == 1:
            for t in range(1, 3):
                w_copy(t, 0, t).start()
        for q in range(16 * i, 16 * i + 16):
            relayout_piece(0, 0, q)
    w_copy(0, 1, 0).start()
    for cp in small_copies:
        cp.start()
    for c in range(NC):
        xt_copy(c, 0).wait()

    for e in range(32):
        if e == 8:
            for c in range(NC):
                xt_copy(c, 1).wait()
        if e == 24:
            w_copy(1, 0, 1).wait()
        y = pre_mm(0, ((e % 8) // 2) * 8 + (e // 8) * 2 + e % 2, packed=False)
        if 8 <= e < 24:
            gate = _gate(y[0:8], _zero_of(count))
            cc, s0 = (e - 8) // 2, (e % 2) * 32
            for sg in range(s0, s0 + 32, 2):
                xpk[cc, sg * 4:sg * 4 + 8, :] = _tie(pltpu.bitcast(xpre[cc, sg:sg + 2].reshape(16, 128), U32), gate)
        if e >= 24:
            relayout_with(y, _zero_of(count), 1, 1, e - 24, 7)
    w_copy(1, 1, 1).start()
    background(0)

    def pre_chunk(c, carry, pack):
        tn, gn = carry
        zero = _zero_of(tn)
        w_copy(0, 0, tn).wait()
        for d in range(32):
            y = pre_mm(c, d)
            relayout_with(y, zero, c + 1, tn, d, 31)
            if pack:
                for i in range(2):
                    gate = _gate(y[64 * i + 32:64 * i + 40], zero)
                    for r in range((d % 2) * 256 + i * 128, (d % 2) * 256 + (i + 1) * 128, 8):
                        o = ((d // 2) % 4) * 1024 + 2 * r
                        wos[(c - 9) * 16 + d // 2, r:r + 8, :] = _tie(
                            pltpu.bitcast(wpark[(c - 9) * 4 + d // 8, o:o + 16, :], U32), gate)
        if not pack:
            for t in range(3):
                @pl.when(jnp.logical_and(tn == t, gn < 3))
                def _():
                    w_copy(t, gn + 1, t).start()

            @pl.when(c < NC)
            def _():
                background(c)

            @pl.when(c == NC)
            def _():
                for cp in conv_copies(0) + conv_copies(1):
                    cp.start()
        return jnp.where(tn == 2, 0, tn + 1), jnp.where(tn == 2, gn + 1, gn)

    carry = jax.lax.fori_loop(1, 9, functools.partial(pre_chunk, pack=False), (2, 0))
    for c in range(NC):
        wo_copy(c).wait()
        x_copy(c).wait()
    count = jax.lax.fori_loop(9, 11, functools.partial(pre_chunk, pack=True), carry)[1]

    for cp in small_copies:
        cp.wait()
    for cp in conv_copies(0) + conv_copies(1):
        cp.wait()
    small[0:NC, :] = dskip_ref[...].astype(F32)
    gate_w = gate_ref[...].astype(F32)
    for c in range(NC):
        small[NC + 8 * c:NC + 8 * (c + 1), :] = jnp.broadcast_to(gate_w[c:c + 1, :], (8, 128))
    mem[...] = mem0_ref[...].astype(F32)

    def mix_gate(r0, gate):
        z = None
        for c in range(NC):
            gw = small[NC + 8 * c:NC + 8 * (c + 1), :]
            t = xs[c, r0:r0 + 16, :].astype(F32) * jnp.concatenate([gw, gw], axis=0)
            z = _tie(t, jnp.concatenate([gate, gate], axis=0)) if z is None else z + t
        z = jnp.sum(z, axis=1, keepdims=True)
        gbuf[r0 // SEG, r0 % SEG:r0 % SEG + 16, :] = jnp.broadcast_to(0.5 * jnp.tanh(0.5 * z) + 0.5, (16, 128))

    def accumulate(slab, segs, rows, val):
        old = outb[slab, segs, rows, :].astype(F32)
        outb[slab, segs, rows, :] = (old + val.astype(BF16).astype(F32).reshape(old.shape)).astype(BF16)

    def conv_prep(t, j):
        tr = t if isinstance(t, int) else jnp.minimum(t, NC - 1)
        r0 = _mo(j * 2 * CB, 2 * CB)
        shift = shift_ref[tr].astype(F32)
        gate = yield
        for o in range(0, 2 * CB + KPAD, 16):
            kk = ks[tr, pl.ds(_mo(r0 + o, 16), 16), :].astype(F32)
            kf[o:o + 8, :] = _tie(kk[0:8], gate)
            kf[o + 8:o + 16, :] = _tie(kk[8:16], gate)
            if o == 0:
                continue
            acc = kf[o:o + 16, :] * shift[0:1, :]
            for l in range(1, KS):
                acc = acc + kf[o - l:o - l + 16, :] * shift[l:l + 1, :]
            rows = pl.ds(_mo(r0 + (o - KPAD), 16), 16)
            vs[t + 1, rows, :] = (acc * vs[tr + 1, rows, :].astype(F32)).astype(BF16)
            gate = yield

    def conv_fwd(t, j):
        tr = t if isinstance(t, int) else jnp.minimum(t, NC - 1)
        slot = t & 1
        fwd = fwd_ref[...]
        for i in range(2):
            rows = pl.ds(_mo((2 * j + i) * CB, CB), CB)
            sr = _mo((2 * j + i) * 32, 32)
            for off, res in ((0, _dot(fwd, vs[t + 1, rows, :])), (512, _dot_nt(fwd, ssm[tr, :, rows]))):
                for ri in range(2):
                    for fj in range(8):
                        spec[slot * 8 + fj, pl.ds(sr + (off + ri * 16), 16), :] = (
                            res[ri * CB + fj * 16:ri * CB + (fj + 1) * 16])

    def conv_mac(t, j, zero):
        slot = t & 1
        sign = jnp.where(j < 4, 1.0, -1.0).astype(F32)
        zbase = pl.multiple_of(slot * (NB * CB) + j * 8, 8)
        prev = None
        gate = yield
        for i in range(NB):
            base = slot * 8 + j + zero * (i + 1)
            ys = []
            for hv in range(2):
                yr = yi = None
                for jj in range(i + 1):
                    uo = jj * 32 + hv * 8
                    ko = 512 + (i - jj) * 32 + hv * 8
                    ur = spec[base, uo:uo + 8, :]
                    ui = spec[base, uo + 16:uo + 24, :]
                    kr = spec[base, ko:ko + 8, :]
                    ki = spec[base, ko + 16:ko + 24, :]
                    tr, ti = _tie(ur * kr - ui * ki, gate), _tie(ur * ki + ui * kr, gate)
                    yr, yi = (tr, ti) if yr is None else (yr + tr, yi + ti)
                    if jj < i or hv == 0:
                        gate = yield
                ys.append((yr, yi))
            yr = jnp.concatenate([ys[0][0], ys[1][0]], axis=0)
            yi = jnp.concatenate([ys[0][1], ys[1][1]], axis=0)
            zr, zi = (yr, yi) if prev is None else (yr - sign * prev[1], yi + sign * prev[0])
            prev = (yr, yi)
            zspec[pl.ds(zbase + i * CB, 8), :] = pltpu.bitcast(zr.astype(BF16), U32)
            zspec[pl.ds(zbase + (i * CB + CB // 2), 8), :] = pltpu.bitcast(zi.astype(BF16), U32)
            gate = yield

    def conv_inv(t, j):
        tr = t if isinstance(t, int) else jnp.maximum(t, 0)
        slot = t & 1
        dsk = small[pl.ds(tr, 1), :]
        inv = inv_ref[...]
        for i in range(2):
            rows = pl.ds(_mo((2 * j + i) * CB, CB), CB)
            z = zspec[pl.ds(_mo((slot * NB + 2 * j + i) * CB, CB), CB), :]
            y = _dot(inv, pltpu.bitcast(z, BF16))
            y = y + vs[t + 1, rows, :].astype(F32) * dsk
            segs = pl.ds((2 * j + i) * (CB // SEG), CB // SEG)
            accumulate(t + 1, segs, slice(None), gbuf[segs].reshape(CB, 128) * (xs[tr, rows, :].astype(F32) * y))

    for q in range(32):
        if q % 4 == 0:
            preps = conv_prep(0, q // 4)
            next(preps)
        y = pre_mm(11, q)
        if q % 4 == 1 and q >= 4:
            conv_fwd(0, q // 4 - 1)
        for i in range(4):
            gate = _gate(y[32 * i:32 * i + 8], _zero_of(count))
            preps.send(gate)
            mix_gate(q * 64 + i * 16, gate)
    conv_fwd(0, NB // 2 - 1)

    ri = jax.lax.broadcasted_iota(I32, (NR, NR), 0)
    ci = jax.lax.broadcasted_iota(I32, (NR, NR), 1)
    LD = MEM + XR

    def head_pos(i):
        tail = i >= 2 * LD
        return (jnp.where(tail, (i - 2 * LD) // TL, i // LD),
                jnp.where(tail, LD + (i - 2 * LD) % TL, i % LD))
    (rh, rp), (ch, cp_) = head_pos(ri), head_pos(ci)
    same = rh == ch
    keep = same & ((rp < MEM) | (rp >= cp_))
    fbuf[0, 0:NR, 0:NR] = jnp.where(keep, 0.0, jnp.where(same, -1000000000.0, -jnp.inf)).astype(F32)
    scale = float(DH) ** -0.5

    def step(it, u, zero):
        s = it * 2 + u
        ct = jax.lax.shift_right_logical(s, 3)
        cj = jnp.bitwise_and(s, 7)
        xr0 = pl.multiple_of(it * (2 * SEG) + u * SEG, SEG)
        h_lhs = jnp.concatenate(
            [jnp.concatenate([mem[:, c * 128:(c + 1) * 128], xs[c, pl.ds(xr0, XR), :].astype(F32)],
                             axis=0).astype(BF16) for c in range(NC)], axis=1)

        macs = conv_mac(ct, cj, zero)
        next(macs)
        preps = conv_prep(ct + 1, cj)
        next(preps)
        n_mac = NB * (NB + 1)
        queue = [(preps, 1)] * 16 + [(macs, min(MAC_G, n_mac - n)) for n in range(0, n_mac, MAC_G)]

        def side_work(token):
            if queue:
                gen, cnt = queue.pop(0)
                gen.send(_gate(token, zero))
                for _ in range(cnt - 1):
                    gen.send(None)

        def proj(p):
            for t in range(3):
                for i, hh in enumerate((2 * p, 2 * p + 1)):
                    y = _dot(h_lhs, pltpu.bitcast(wts[(hh // 8) * 24 + t * 8 + hh % 8], BF16))
                    side_work(y[0:MEM])
                    ybufs[p // 4][t * 4 + p % 4 + zero, i * 16:(i + 1) * 16, :] = pltpu.bitcast(y.astype(BF16), U32)

        def rows_of(t, p):
            o = ((p // 4) * 12 + t * 4 + p % 4) * 8
            return pltpu.bitcast(jnp.concatenate([ybufs[p // 4][t * 4 + p % 4], prebuf[s, o:o + 8, :]], axis=0), BF16)

        def scores(p):
            sc = _dot_nt(rows_of(0, p), rows_of(1, p)) * scale
            fill = fbuf[zero * (p + 1), 0:NR, 0:NR]
            sc = jnp.where(fill == 0.0, sc, fill)
            e = jnp.exp(sc - jnp.max(sc, axis=1, keepdims=True))
            l = jnp.sum(e, axis=1, keepdims=True)
            r = pl.reciprocal(l, approx=True)
            ebuf[p + zero, 0:NR // 2, :] = pltpu.bitcast(e.astype(BF16), U32)
            return r * (2.0 - l * r)

        def values(p, r):
            o = _dot(pltpu.bitcast(ebuf[p, 0:NR // 2, :], BF16), rows_of(2, p)) * r
            for i, hh in enumerate((2 * p, 2 * p + 1)):
                olhs[hh] = pltpu.bitcast(o[i * LD:(i + 1) * LD].astype(BF16), U32)
                obuf[hh, pl.ds(pl.multiple_of(s * TL, TL), TL), :] = (
                    o[2 * LD + i * TL:2 * LD + (i + 1) * TL].astype(BF16))

        def oproj(g):
            lhs = pltpu.bitcast(jnp.concatenate([olhs[hh] for hh in range(4 * g, 4 * g + 4)], axis=1), BF16)
            for n in range(NC):
                w = wos[4 * n + g // 2, (g % 2) * 256:(g % 2 + 1) * 256, :]
                y = _dot(lhs, pltpu.bitcast(w, BF16))
                side_work(y[0:MEM])
                if g > 0:
                    y = y + oacc[n + zero]
                if g < H // 4 - 1:
                    oacc[n] = y
                else:
                    mem[:, n * 128:(n + 1) * 128] = y[0:MEM].astype(BF16).astype(F32)
                    accumulate(n + 1, s, slice(0, XR),
                               (1.0 - gbuf[s, 0:XR, :]) * y[MEM:].astype(BF16).astype(F32))

        recip = [None] * (H // 2)
        for op, arg in PROGRAM:
            if op == "P":
                proj(arg)
            elif op == "S":
                recip[arg] = scores(arg)
            elif op == "V":
                values(arg, recip[arg])
            elif op == "O":
                oproj(arg)
            elif op == "I":
                conv_inv(ct - 1, cj)
            else:
                assert not queue
                conv_fwd(ct + 1, cj)

    def two_steps(it, carry):
        for u in range(2):
            step(it, u, _zero_of(carry))

        @pl.when(it == 0)
        def _():
            for c in range(2, NC):
                for cp in conv_copies(c):
                    cp.start()

        @pl.when(it == 3)
        def _():
            for c in range(2, NC):
                for cp in conv_copies(c):
                    cp.wait()
        return carry + 1
    jax.lax.fori_loop(0, NSEG // 2, two_steps, count)

    for j in range(NB // 2):
        conv_inv(NC - 1, j)

    def out_copies(s0, n, r0, nr):
        return [pltpu.make_async_copy(outb.at[c + 1, pl.ds(s0, n), pl.ds(r0, nr), :],
                                      out_hbm.at[pl.ds(s0, n), pl.ds(r0, nr), pl.ds(c * 128, 128)], sems.at[4])
                for c in range(NC)]

    for cp in out_copies(0, NSEG, 0, XR):
        cp.start()

    def post_chunk(i, carry):
        rows = pl.ds(pl.multiple_of(i * MB, MB), MB)
        segs = pl.ds(i * 16, 16)
        op = jnp.concatenate([obuf[hh, rows, :] for hh in range(H)], axis=1)
        omg = 1.0 - gbuf[segs, XR:SEG, :].reshape(MB, 128)
        for n in range(NC):
            w = jnp.concatenate([wos[4 * n + kq] for kq in range(4)], axis=0)
            y = _dot(op, pltpu.bitcast(w, BF16))
            accumulate(n + 1, segs, slice(XR, SEG), omg * y.astype(BF16).astype(F32))
        for cp in out_copies(i * 16, 16, XR, TL):
            cp.start()
        return carry
    jax.lax.fori_loop(0, PRE // MB, post_chunk, 0)
    for cp in out_copies(0, NSEG, 0, XR):
        cp.wait()
    for i in range(PRE // MB):
        for cp in out_copies(i * 16, 16, XR, TL):
            cp.wait()


@functools.partial(jax.jit, static_argnames=("B_seg_len",))
def pallas_gated_mix__ssm_conv_h3__memory_aug_recurrent_mem_tr__prompt_kernel(
    A_q, A_k, A_v, A_shift_k, A_ssm_k, A_ssm_D, B_x, B_mem0, B_Wq, B_Wk, B_Wv, B_Wo,
    B_seg_len, gate_w,
):
    del B_x
    assert B_seg_len == SEG and A_q.shape == (1, S, D) and B_Wq.shape == (D, H, DH)
    assert A_shift_k.shape == (D, KS) and B_mem0.shape == (1, MEM, D)
    fwd, inv = _dft_tables()
    hbm = pl.BlockSpec(memory_space=pl.ANY)
    out = pl.pallas_call(
        _kernel,
        out_shape=jax.ShapeDtypeStruct((NSEG, SEG, D), BF16),
        in_specs=[hbm] * 15,
        out_specs=hbm,
        scratch_shapes=[
            pltpu.VMEM((NC, S, 128), BF16),
            pltpu.VMEM((NC, NSEG, TL, 128), BF16),
            pltpu.VMEM((NC, PRE // 2, 128), U32),
            pltpu.VMEM((NC, 64 + S, 128), BF16),
            pltpu.VMEM((NC + 2, S, 128), BF16),
            pltpu.VMEM((NC, 128, S), BF16),
            pltpu.VMEM((3, D, 8, 128), BF16),
            pltpu.VMEM((3 * H, D // 2, 128), U32),
            pltpu.VMEM((4 * NC, D // 2, 128), U32),
            pltpu.VMEM((NC, H * DH, 128), BF16),
            pltpu.VMEM((NSEG, 3 * H // 2 * 8, 128), U32),
            pltpu.VMEM((12, 32, 128), U32),
            pltpu.VMEM((12, 32, 128), U32),
            pltpu.VMEM((12, 32, 128), U32),
            pltpu.VMEM((12, 32, 128), U32),
            pltpu.VMEM((H, PRE, 128), BF16),
            pltpu.VMEM((NC + 1, NSEG, SEG, 128), BF16),
            pltpu.VMEM((H, 16, 128), U32),
            pltpu.VMEM((NC, MEM + XR, 128), F32),
            pltpu.VMEM((MEM, D), F32),
            pltpu.VMEM((96, 128), F32),
            pltpu.VMEM((288, 128), F32),
            pltpu.VMEM((2, 160, 128), F32),
            pltpu.VMEM((1, 96, 128), F32),
            pltpu.VMEM((H // 2, 64, NR), U32),
            pltpu.VMEM((16, 1024, 128), F32),
            pltpu.VMEM((2 * NB * CB, 128), U32),
            pltpu.VMEM((NSEG, SEG, 128), F32),
            pltpu.VMEM((2 * CB, CB), BF16),
            pltpu.VMEM((CB, 2 * CB), BF16),
            pltpu.VMEM((MEM, D), BF16),
            pltpu.VMEM((NC, KS, 128), BF16),
            pltpu.VMEM((NC, 128), BF16),
            pltpu.VMEM((NC, 128), BF16),
            pltpu.SemaphoreType.DMA((11,)),
            pltpu.SemaphoreType.DMA((3,)),
        ],
        compiler_params=pltpu.CompilerParams(vmem_limit_bytes=120 * 1024 * 1024, disable_bounds_checks=True, disable_semaphore_checks=True),
    )(
        A_q.reshape(S, D), A_q.reshape(NSEG, SEG, D), A_k.reshape(S, D), A_v.reshape(S, D), A_ssm_k,
        B_Wq, B_Wk, B_Wv, B_Wo.reshape(H * DH, D),
        A_shift_k.T.reshape(KS, NC, 128).transpose(1, 0, 2),
        A_ssm_D.reshape(NC, 128), gate_w.reshape(NC, 128),
        B_mem0.reshape(MEM, D),
        jnp.asarray(fwd, BF16), jnp.asarray(inv, BF16),
    )
    return out.reshape(1, S, D)
```

```python
import functools

import jax
import jax.numpy as jnp
import numpy as np
import jax.experimental.pallas as pl
import jax.experimental.pallas.tpu as pltpu

F32 = jnp.float32
BF16 = jnp.bfloat16
U32 = jnp.uint32
I32 = jnp.int32

S = 2048
D = 1024
NC = D // 128
H = 32
DH = 128
MEM = 8
SEG = 32
NSEG = S // SEG
XR = 24
PRE = S - NSEG * XR
TL = SEG - XR
NR = 2 * (SEG + MEM)
CB = 128
NB = S // CB
KS = 4
KPAD = 16
MB = 128
SST = 9
SB = 64
NEV = 28 * 256 // SB
MAC_G = 3


def _expand(text):
    out = []
    for item in text.split():
        if "-" in item:
            a, b = item[1:].split("-")
            out += [(item[0], i) for i in range(int(a), int(b) + 1)]
        else:
            out.append((item[0], int(item[1:] or 0)))
    return out


PROGRAM = _expand("P0-4 S0-3 P5-8 V0-3 S4-7 P9-10 O0 P11-12 V4-7 S8-11 P13 O1 P14-15 "
                  "O2 V8-11 S12-15 O3 O4 V12-15 O5 O6 O7 I F")


def _dft_tables():
    f = np.concatenate([np.arange(0, CB, 2), np.arange(1, CB, 2)]).astype(np.float64)
    t = np.arange(CB, dtype=np.float64)
    ang = 2.0 * np.pi * (f[:, None] + 0.5) * t[None, :] / (2 * CB)
    fwd = np.concatenate([np.cos(ang), -np.sin(ang)], axis=0)
    inv = np.concatenate([np.cos(ang).T, -np.sin(ang).T], axis=1) / CB

    def words(m):
        u = np.asarray(m, dtype=BF16).view(np.uint16).astype(np.uint32)
        return u[0::2] | (u[1::2] << 16)
    return words(fwd), np.stack([words(inv[:, :CB]), words(inv[:, CB:])])


def _dot(a, b):
    return jnp.dot(a, b, preferred_element_type=F32)


def _dot_nt(a, b):
    return jax.lax.dot_general(a, b, (((1,), (1,)), ((), ())), preferred_element_type=F32)


def _mo(x, m):
    return x if isinstance(x, int) else pl.multiple_of(x, m)


def _tie(x, gate):
    return x if gate is None else pltpu.bitcast(pltpu.bitcast(x, I32) | gate, x.dtype)


def _gate(token, zero):
    return pltpu.bitcast(token, I32) & jnp.full((8, 128), zero, I32)


def _halves(words):
    return [pltpu.unpack_elementwise(words, index=i, packed_dtype=BF16, unpacked_dtype=F32) for i in range(2)]


def _pack2(even, odd):
    return pltpu.pack_elementwise([even, odd], packed_dtype=BF16)


def _sum16(a, b, sign=1):
    return _pack2(*[(x + y if sign > 0 else x - y) for x, y in zip(a, b)])


def _zero_of(counter):
    return jax.lax.shift_right_logical(counter, 16)


def _kernel(x_hbm, x3_hbm, k_hbm, v_hbm, ssm_hbm, wq_hbm, wk_hbm, wv_hbm, wo_hbm,
            shift_hbm, dskip_hbm, gate_hbm, mem0_hbm, fwd_hbm, inv_hbm,
            out_hbm,
            xs, xpre, xpk, wsum, ks, vs, ssm, wraw, wts, wos, wosum, otail, wpark, prebuf, yb0, yb1, yb2, yb3, obuf, outb, olhs, oacc,
            mem, small, stage, fbuf, ebuf, spec, zspec, gbuf,
            fwd_ref, inv_ref, mem0_ref, shift_ref, dskip_ref, gate_ref,
            sems, sem_w):
    w_hbm = (wq_hbm, wk_hbm, wv_hbm)
    ybufs = (yb0, yb1, yb2, yb3)

    def x_copy(c):
        return pltpu.make_async_copy(x_hbm.at[:, pl.ds(c * 128, 128)], xs.at[c], sems.at[2])

    def xt_copy(c, part):
        s0, n, si = ((0, 16, 0), (16, NSEG - 16, 10))[part]
        return pltpu.make_async_copy(x3_hbm.at[pl.ds(s0, n), pl.ds(XR, TL), pl.ds(c * 128, 128)],
                                     xpre.at[c, pl.ds(s0, n)], sems.at[si])

    def conv_copies(c):
        col = pl.ds(c * 128, 128)
        sem = sems.at[(2, 0, 3)[min(c, 2)]]
        return [pltpu.make_async_copy(k_hbm.at[:, col], ks.at[c, pl.ds(KPAD, S), :], sem),
                pltpu.make_async_copy(v_hbm.at[:, col], vs.at[c + 1], sem),
                pltpu.make_async_copy(ssm_hbm.at[col, :], ssm.at[c], sem)]

    def wo_copy(c):
        return pltpu.make_async_copy(wo_hbm.at[:, pl.ds(_mo(c * 128, 128), 128)], wpark.at[c], sems.at[1])

    def w_copy(t, g, slot):
        return pltpu.make_async_copy(w_hbm[t].at[:, pl.ds(_mo(g * 8, 8), 8), :], wraw.at[slot], sem_w.at[slot])

    def w0_copy(i):
        return pltpu.make_async_copy(wq_hbm.at[pl.ds(i * 256, 256), pl.ds(0, 8), :],
                                     wraw.at[0, pl.ds(i * 256, 256)], sems.at[5 + i])

    small_copies = [pltpu.make_async_copy(a, b, sems.at[9]) for a, b in (
        (shift_hbm, shift_ref), (dskip_hbm, dskip_ref), (gate_hbm, gate_ref),
        (mem0_hbm, mem0_ref), (fwd_hbm, fwd_ref), (inv_hbm, inv_ref))]

    late_copies = conv_copies(0) + [x_copy(c) for c in range(NC)]

    for i in range(4):
        w0_copy(i).start()
    for c in range(NC):
        xt_copy(c, 0).start()

    vs[0] = jnp.zeros((S, 128), BF16)
    outb[0] = jnp.zeros((NSEG, SEG, 128), BF16)
    zspec[NB * CB:2 * NB * CB, :] = jnp.zeros((NB * CB, 128), U32)

    def clear(c, count):
        ks[c, 0:KPAD, :] = jnp.zeros((KPAD, 128), BF16)
        outb[c + 1] = jnp.zeros((NSEG, SEG, 128), BF16)
        return count + 1

    def relayout_piece(c, slot, q, gate=None):
        ws = [pltpu.bitcast(wraw[slot, q * 16 + 2 * i:q * 16 + 2 * i + 2].reshape(16, 128), U32)
              for i in range(8)]
        if isinstance(c, int):
            st = stage.at[q % 2]
            for i in range(8):
                st[i * SST:i * SST + 8, :] = _tie(ws[i], gate if i == 0 else None)
            tr = [st[pl.ds(j, 8, stride=SST), :] for j in range(8)]
        else:
            ws = [_tie(w, gate if i % 2 == 0 else None) for i, w in enumerate(ws)]
            tr = jnp.transpose(jnp.stack(ws, axis=0), (1, 0, 2))
        for j in range(4):
            ev, od = _halves(tr[j]), _halves(tr[4 + j])
            for hb in range(2):
                wts[c * 8 + (2 * j + hb), q * 8:(q + 1) * 8, :] = _pack2(ev[hb], od[hb])

    def relayout_with(y, zero, c, slot, d, span):
        qs = range(min(64 * d // span, 64), min(64 * (d + 1) // span, 64))
        for i, q in enumerate(qs):
            o = (i * MB // len(qs)) // 8 * 8
            relayout_piece(c, slot, q, _gate(y[o:o + 8], zero))

    pend = [None]

    def store_pair(c, pp, seg0, ya, yb):
        for i in range(ya.shape[0] // 8):
            pair = jnp.concatenate([ya[8 * i:8 * i + 8], yb[8 * i:8 * i + 8]], axis=0)
            prebuf[seg0 + i, pl.ds(_mo(c * 32, 32) + pp * 8, 8), :] = pltpu.bitcast(pair.astype(BF16), U32)

    def first_mm(d):
        pp, rb, hb = d // 8, (d // 2) % 4, d % 2
        w = pltpu.bitcast(wts[2 * pp + hb], BF16)
        xp = jnp.concatenate([xpre[cc, rb * 16:(rb + 1) * 16].reshape(MB, 128) for cc in range(NC)], axis=1)
        y = _dot(xp, w)
        if hb == 0:
            pend[0] = y
        else:
            store_pair(0, pp, rb * 16, pend[0], y)
        return y

    def lhs_piece(cc, sg, gate):
        def ld(c2, s2):
            return pltpu.bitcast(xpre[c2, s2:s2 + 2].reshape(16, 128), U32)
        w11, w12, w21, w22 = ld(cc, sg), ld(cc + 4, sg), ld(cc, sg + 32), ld(cc + 4, sg + 32)
        w11, w22 = _tie(w11, gate), _tie(w22, gate)
        a11, a12, a21, a22 = _halves(w11), _halves(w12), _halves(w21), _halves(w22)
        vals = (_sum16(a11, a12), _sum16(a21, a22), w11, w22, _sum16(a11, a22),
                _sum16(a12, a22, -1), _sum16(a21, a11, -1))
        for k, val in enumerate(vals):
            xpk[k * 4 + cc, sg * 4:sg * 4 + 8, :] = val

    def rhs_sums(w11, w12, w21, w22, gate):
        b11, b12, b21, b22 = _halves(_tie(w11, gate)), _halves(w12), _halves(w21), _halves(_tie(w22, gate))
        return (_sum16(b12, b22, -1), _sum16(b21, b11, -1), _sum16(b11, b22), _sum16(b21, b22), _sum16(b11, b12))

    def rhs_piece(hd, par, r, gate):
        sums = rhs_sums(wts[hd, r:r + 8, :], wts[hd + 1, r:r + 8, :],
                        wts[hd, 256 + r:264 + r, :], wts[hd + 1, 256 + r:264 + r, :], gate)
        for k, val in enumerate(sums):
            wsum[par * 5 + k, r:r + 8, :] = val

    def strassen_chunk(c, zero, extra, last=False):
        nrb = 256 // SB
        e = 0
        for pp in range(4):
            for rb in range(nrb):
                ms = []
                for k in range(7):
                    a = jnp.concatenate([xpk[k * 4 + cc, rb * (SB // 2):(rb + 1) * (SB // 2), :] for cc in range(4)], axis=1)
                    if k == 0:
                        b = wts[c * 8 + (2 * pp + 1), 256:512, :]
                    elif k == 1:
                        b = wts[c * 8 + 2 * pp, 0:256, :]
                    else:
                        b = wsum[(pp % 2) * 5 + k - 2]
                    y = _dot(pltpu.bitcast(a, BF16), pltpu.bitcast(b, BF16))
                    ms.append(y)
                    if k == 5:
                        m5, m2, m3, m4, m1, m7 = ms
                        store_pair(c, pp, rb * (SB // 8), ((m4 - m5) + m1) + m7, m5 + m3)
                    if k == 6:
                        store_pair(c, pp, 32 + rb * (SB // 8), m2 + m4, ((m3 - m2) + m1) + y)
                    extra(e, y)
                    le = e % (7 * nrb)
                    cbe = 6 * nrb
                    if not (last and pp == 3):
                        for i, r in enumerate(range(min(32 * le // cbe, 32), min(32 * (le + 1) // cbe, 32))):
                            o = (8 * (2 * i + 1)) % SB
                            rhs_piece(c * 8 + (2 * pp + 2), (pp + 1) % 2, r * 8, _gate(y[o:o + 8], zero))
                    e += 1

    count = 0
    for i in range(4):
        count = jax.lax.fori_loop(2 * i, 2 * i + 2, clear, count)
        w0_copy(i).wait()
        if i == 0:
            for c in range(NC):
                xt_copy(c, 1).start()
        if i == 1:
            for t in range(1, 3):
                w_copy(t, 0, t).start()
        for q in range(16 * i, 16 * i + 16):
            relayout_piece(0, 0, q)
    w_copy(0, 1, 0).start()
    for cp in small_copies:
        cp.start()
    for c in range(NC):
        xt_copy(c, 0).wait()

    for e in range(32):
        if e == 8:
            for c in range(NC):
                xt_copy(c, 1).wait()
        if e == 24:
            w_copy(1, 0, 1).wait()
        y = first_mm(((e % 8) // 2) * 8 + (e // 8) * 2 + e % 2)
        if 8 <= e < 24:
            for i in range(4):
                lhs_piece((e - 8) // 4, ((e % 4) * 4 + i) * 2, _gate(y[32 * i:32 * i + 8], _zero_of(count)))
        if e >= 24:
            relayout_with(y, _zero_of(count), 1, 1, e - 24, 7)
    for r in range(32):
        rhs_piece(8, 0, r * 8, None)
    w_copy(1, 1, 1).start()
    wo_copy(0).start()

    def pre_chunk(c, carry, packwo):
        tn, gn = carry
        zero = _zero_of(tn)
        w_copy(0, 0, tn).wait()

        def extra(e, y):
            rle = 78 * NEV // 112
            for i, q in enumerate(range(min(64 * e // rle, 64), min(64 * (e + 1) // rle, 64))):
                relayout_piece(c + 1, tn, q, _gate(y[16 * i:16 * i + 8], zero))
            if packwo:
                gate = _gate(y[SB - 8:SB], zero)
                for v in range(min(1024 * e // (NEV - 2), 1024), min(1024 * (e + 1) // (NEV - 2), 1024)):
                    sl, r = v // 64, (v % 64) * 8
                    o = (sl % 4) * 1024 + 2 * r
                    wos[(c - 9) * 16 + sl, r:r + 8, :] = _tie(
                        pltpu.bitcast(wpark[(c - 9) * 4 + sl // 4, o:o + 16, :], U32), gate)
        strassen_chunk(c, zero, extra)
        if not packwo:
            for t in range(3):
                @pl.when(jnp.logical_and(tn == t, gn < 3))
                def _():
                    w_copy(t, gn + 1, t).start()

            @pl.when(c < NC)
            def _():
                wo_copy(c).start()

        return jnp.where(tn == 2, 0, tn + 1), jnp.where(tn == 2, gn + 1, gn)

    carry = jax.lax.fori_loop(1, 9, functools.partial(pre_chunk, packwo=False), (2, 0))
    for cp in late_copies:
        cp.start()
    for c in range(NC):
        wo_copy(c).wait()
    count = jax.lax.fori_loop(9, 11, functools.partial(pre_chunk, packwo=True), carry)[1]

    for cp in small_copies:
        cp.wait()
    for cp in late_copies:
        cp.wait()
    for cp in conv_copies(1):
        cp.start()
    small[0:NC, :] = dskip_ref[...].astype(F32)
    gate_w = gate_ref[...].astype(F32)
    for c in range(NC):
        small[NC + 8 * c:NC + 8 * (c + 1), :] = jnp.broadcast_to(gate_w[c:c + 1, :], (8, 128))
    mem[...] = mem0_ref[...].astype(F32)

    def mix_gate(r0, gate):
        z = None
        for c in range(NC):
            gw = small[NC + 8 * c:NC + 8 * (c + 1), :]
            t = xs[c, r0:r0 + 16, :].astype(F32) * jnp.concatenate([gw, gw], axis=0)
            z = _tie(t, jnp.concatenate([gate, gate], axis=0)) if z is None else z + t
        z = jnp.sum(z, axis=1, keepdims=True)
        gbuf[r0 // SEG, r0 % SEG:r0 % SEG + 16, :] = jnp.broadcast_to(0.5 * jnp.tanh(0.5 * z) + 0.5, (16, 128))

    def accumulate(slab, segs, rows, val):
        old = outb[slab, segs, rows, :].astype(F32)
        outb[slab, segs, rows, :] = (old + val.astype(BF16).astype(F32).reshape(old.shape)).astype(BF16)

    def conv_prep(t, j):
        tr = t if isinstance(t, int) else jnp.minimum(t, NC - 1)
        r0 = _mo(j * 2 * CB, 2 * CB)
        shift = shift_ref[tr].astype(F32)
        gate = yield
        tail = None
        for o in range(0, 2 * CB + KPAD, 16):
            kk = ks[tr, pl.ds(r0 + o, 16), :].astype(F32)
            win = [tail, _tie(kk[0:8], gate), _tie(kk[8:16], gate)]
            tail = win[2]
            if o == 0:
                continue
            win = jnp.concatenate(win, axis=0)
            acc = win[8:24] * shift[0:1, :]
            for l in range(1, KS):
                acc = acc + win[8 - l:24 - l] * shift[l:l + 1, :]
            rows = pl.ds(r0 + (o - KPAD), 16)
            vs[t + 1, rows, :] = (acc * vs[tr + 1, rows, :].astype(F32)).astype(BF16)
            gate = yield

    def conv_fwd(t, j):
        tr = t if isinstance(t, int) else jnp.minimum(t, NC - 1)
        slot = t & 1
        fwd = pltpu.bitcast(fwd_ref[...], BF16)
        for i in range(2):
            rows = pl.ds(_mo((2 * j + i) * CB, CB), CB)
            sr = _mo((2 * j + i) * 32, 32)
            for off, res in ((0, _dot(fwd, vs[t + 1, rows, :])), (512, _dot_nt(fwd, ssm[tr, :, rows]))):
                for ri in range(2):
                    for fj in range(8):
                        spec[slot * 8 + fj, pl.ds(sr + (off + ri * 16), 16), :] = (
                            res[ri * CB + fj * 16:ri * CB + (fj + 1) * 16])

    def conv_mac(t, j, zero):
        slot = t & 1
        sign = jnp.where(j < 4, 1.0, -1.0).astype(F32)
        zbase = pl.multiple_of(slot * (NB * CB) + j * 8, 8)
        prev = None
        gate = yield
        for i in range(NB):
            base = slot * 8 + j + zero * (i + 1)
            ys = []
            for hv in range(2):
                yr = yi = None
                for jj in range(i + 1):
                    uo = jj * 32 + hv * 8
                    ko = 512 + (i - jj) * 32 + hv * 8
                    ur = spec[base, uo:uo + 8, :]
                    ui = spec[base, uo + 16:uo + 24, :]
                    kr = spec[base, ko:ko + 8, :]
                    ki = spec[base, ko + 16:ko + 24, :]
                    tr, ti = _tie(ur * kr - ui * ki, gate), _tie(ur * ki + ui * kr, gate)
                    yr, yi = (tr, ti) if yr is None else (yr + tr, yi + ti)
                    if jj < i or hv == 0:
                        gate = yield
                ys.append((yr, yi))
            yr = jnp.concatenate([ys[0][0], ys[1][0]], axis=0)
            yi = jnp.concatenate([ys[0][1], ys[1][1]], axis=0)
            zr, zi = (yr, yi) if prev is None else (yr - sign * prev[1], yi + sign * prev[0])
            prev = (yr, yi)
            zspec[pl.ds(zbase + i * CB, 8), :] = pltpu.bitcast(zr.astype(BF16), U32)
            zspec[pl.ds(zbase + (i * CB + CB // 2), 8), :] = pltpu.bitcast(zi.astype(BF16), U32)
            gate = yield

    def conv_inv(t, j):
        tr = t if isinstance(t, int) else jnp.maximum(t, 0)
        slot = t & 1
        dsk = small[pl.ds(tr, 1), :]
        inv = pltpu.bitcast(jnp.concatenate([inv_ref[0], inv_ref[1]], axis=1), BF16)
        for i in range(2):
            rows = pl.ds(_mo((2 * j + i) * CB, CB), CB)
            z = zspec[pl.ds(_mo((slot * NB + 2 * j + i) * CB, CB), CB), :]
            y = _dot(inv, pltpu.bitcast(z, BF16))
            y = y + vs[t + 1, rows, :].astype(F32) * dsk
            segs = pl.ds((2 * j + i) * (CB // SEG), CB // SEG)
            accumulate(t + 1, segs, slice(None), gbuf[segs].reshape(CB, 128) * (xs[tr, rows, :].astype(F32) * y))

    state = {}

    def last_extra(e, y):
        for i, q in enumerate(range(128 * e // NEV, 128 * (e + 1) // NEV)):
            if q % 16 == 0:
                state["prep"] = conv_prep(0, q // 16)
                next(state["prep"])
            if q % 16 == 5 and q >= 16:
                conv_fwd(0, q // 16 - 1)
            gate = _gate(y[16 * i:16 * i + 8], _zero_of(count))
            state["prep"].send(gate)
            mix_gate(q * 16, gate)
    strassen_chunk(11, _zero_of(count), last_extra, last=True)
    conv_fwd(0, NB // 2 - 1)

    ri = jax.lax.broadcasted_iota(I32, (NR, NR), 0)
    ci = jax.lax.broadcasted_iota(I32, (NR, NR), 1)
    LD = MEM + XR

    def head_pos(i):
        tail = i >= 2 * LD
        return (jnp.where(tail, (i - 2 * LD) // TL, i // LD),
                jnp.where(tail, LD + (i - 2 * LD) % TL, i % LD))
    (rh, rp), (ch, cp_) = head_pos(ri), head_pos(ci)
    same = rh == ch
    keep = same & ((rp < MEM) | (rp >= cp_))
    fbuf[0, 0:NR, 0:NR] = jnp.where(keep, 0.0, jnp.where(same, -1000000000.0, -jnp.inf)).astype(F32)
    scale = float(DH) ** -0.5

    def step(it, u, zero):
        s = it * 2 + u
        ct = jax.lax.shift_right_logical(s, 3)
        cj = jnp.bitwise_and(s, 7)
        xr0 = pl.multiple_of(it * (2 * SEG), 2 * SEG) + u * SEG
        h_lhs = jnp.concatenate(
            [jnp.concatenate([mem[:, c * 128:(c + 1) * 128], xs[c, pl.ds(xr0, XR), :].astype(F32)],
                             axis=0).astype(BF16) for c in range(NC)], axis=1)

        macs = conv_mac(ct, cj, zero)
        next(macs)
        preps = conv_prep(ct + 1, cj)
        next(preps)
        n_mac = NB * (NB + 1)

        def wo_sums():
            npair, kq = s >> 4, (s >> 3) & 1
            gate = yield
            for i in range(8):
                rows = pl.ds(pl.multiple_of((s & 7) * 64, 64) + 8 * i, 8)
                sl = npair * 8 + kq
                sums = rhs_sums(wos[sl, rows, :], wos[sl + 4, rows, :], wos[sl + 2, rows, :], wos[sl + 6, rows, :], gate)
                for k, val in enumerate(sums):
                    wosum[npair * 10 + kq + 2 * k, rows, :] = val
                gate = yield

        def tail_sums():
            rows = pl.ds(pl.multiple_of(it * TL, TL), TL)
            gate = yield
            for hh in range(H // 2):
                a11, a22 = _tie(otail[hh], gate), _tie(otail[H + H // 2 + hh], gate)
                a12, a21 = otail[H // 2 + hh], otail[H + hh]
                for k, val in enumerate((a11 + a12, a21 + a22, a11, a22, a11 + a22, a12 - a22, a21 - a11)):
                    obuf[k * (H // 2) + hh, rows, :] = val.astype(BF16)
                gate = yield

        wsums = wo_sums()
        next(wsums)
        queue = ([(preps, 1)] * 16 + [(macs, min(MAC_G, n_mac - n)) for n in range(0, n_mac, MAC_G)]
                 + [(wsums, 1)] * 8)

        def side_work(token):
            if queue:
                gen, cnt = queue.pop(0)
                if gen is None:
                    return
                gen.send(_gate(token, zero))
                for _ in range(cnt - 1):
                    gen.send(None)

        def proj(p):
            for t in range(3):
                for i, hh in enumerate((2 * p, 2 * p + 1)):
                    y = _dot(h_lhs, pltpu.bitcast(wts[(hh // 8) * 24 + t * 8 + hh % 8], BF16))
                    side_work(y[0:MEM])
                    ybufs[p // 4][t * 4 + p % 4 + zero, i * 16:(i + 1) * 16, :] = pltpu.bitcast(y.astype(BF16), U32)

        def rows_of(t, p):
            o = ((p // 4) * 12 + t * 4 + p % 4) * 8
            return pltpu.bitcast(jnp.concatenate([ybufs[p // 4][t * 4 + p % 4], prebuf[s, o:o + 8, :]], axis=0), BF16)

        def scores(p):
            sc = _dot_nt(rows_of(0, p), rows_of(1, p)) * scale
            fill = fbuf[zero * (p + 1), 0:NR, 0:NR]
            sc = jnp.where(fill == 0.0, sc, fill)
            e = jnp.exp(sc - jnp.max(sc, axis=1, keepdims=True))
            l = jnp.sum(e, axis=1, keepdims=True)
            r = pl.reciprocal(l, approx=True)
            ebuf[p + zero, 0:NR // 2, :] = pltpu.bitcast(e.astype(BF16), U32)
            return r * (2.0 - l * r)

        def values(p, r):
            o = _dot(pltpu.bitcast(ebuf[p, 0:NR // 2, :], BF16), rows_of(2, p)) * r
            for i, hh in enumerate((2 * p, 2 * p + 1)):
                olhs[hh] = pltpu.bitcast(o[i * LD:(i + 1) * LD].astype(BF16), U32)
                otail[u * H + hh + zero] = o[2 * LD + i * TL:2 * LD + (i + 1) * TL].astype(BF16).astype(F32)

        def oproj(g):
            lhs = pltpu.bitcast(jnp.concatenate([olhs[hh] for hh in range(4 * g, 4 * g + 4)], axis=1), BF16)
            for n in range(NC):
                w = wos[4 * n + g // 2, (g % 2) * 256:(g % 2 + 1) * 256, :]
                y = _dot(lhs, pltpu.bitcast(w, BF16))
                side_work(y[0:MEM])
                if g > 0:
                    y = y + oacc[n + zero]
                if g < H // 4 - 1:
                    oacc[n] = y
                else:
                    mem[:, n * 128:(n + 1) * 128] = y[0:MEM].astype(BF16).astype(F32)
                    accumulate(n + 1, s, slice(0, XR),
                               (1.0 - gbuf[s, 0:XR, :]) * y[MEM:].astype(BF16).astype(F32))

        recip = [None] * (H // 2)
        for op, arg in PROGRAM:
            if op == "P":
                proj(arg)
            elif op == "S":
                recip[arg] = scores(arg)
            elif op == "V":
                values(arg, recip[arg])
                if u == 1 and arg == H // 2 - 1:
                    assert not queue
                    tsums = tail_sums()
                    next(tsums)
                    queue.extend([(None, 0)] * 4 + [(tsums, 1)] * (H // 2))
            elif op == "O":
                oproj(arg)
            elif op == "I":
                conv_inv(ct - 1, cj)
            else:
                assert not queue
                conv_fwd(ct + 1, cj)

    def two_steps(it, carry):
        for u in range(2):
            step(it, u, _zero_of(carry))

        @pl.when(it == 3)
        def _():
            for c in range(2, NC):
                for cp in conv_copies(c):
                    cp.wait()
        return carry + 1
    for cp in conv_copies(1):
        cp.wait()
    for c in range(2, NC):
        for cp in conv_copies(c):
            cp.start()
    jax.lax.fori_loop(0, NSEG // 2, two_steps, count)

    for j in range(NB // 2):
        conv_inv(NC - 1, j)

    def out_copies(s0, n, r0, nr):
        return [pltpu.make_async_copy(outb.at[c + 1, pl.ds(s0, n), pl.ds(r0, nr), :],
                                      out_hbm.at[pl.ds(s0, n), pl.ds(r0, nr), pl.ds(c * 128, 128)], sems.at[4])
                for c in range(NC)]

    for cp in out_copies(0, NSEG, 0, XR):
        cp.start()

    def post_chunk(i, carry):
        rows = pl.ds(pl.multiple_of(i * 64, 64), 64)

        def finish(n, par, y):
            for j in range(8):
                sg = i * 16 + (2 * j + par)
                accumulate(n + 1, sg, slice(XR, SEG),
                           (1.0 - gbuf[sg, XR:SEG, :]) * y[8 * j:8 * j + 8].astype(BF16).astype(F32))

        for npair in range(NC // 2):
            ms = []
            for k in range(7):
                a = jnp.concatenate([obuf[k * (H // 2) + hh, rows, :] for hh in range(H // 2)], axis=1)
                if k == 0:
                    b = [wos[npair * 8 + 6], wos[npair * 8 + 7]]
                elif k == 1:
                    b = [wos[npair * 8], wos[npair * 8 + 1]]
                else:
                    b = [wosum[npair * 10 + 2 * (k - 2)], wosum[npair * 10 + 2 * (k - 2) + 1]]
                ms.append(_dot(a, pltpu.bitcast(jnp.concatenate(b, axis=0), BF16)))
                if k == 2:
                    finish(2 * npair + 1, 0, ms[0] + ms[2])
                if k == 3:
                    finish(2 * npair, 1, ms[1] + ms[3])
                if k == 5:
                    finish(2 * npair, 0, ((ms[3] - ms[0]) + ms[4]) + ms[5])
                if k == 6:
                    finish(2 * npair + 1, 1, ((ms[2] - ms[1]) + ms[4]) + ms[6])
        for cp in out_copies(i * 16, 16, XR, TL):
            cp.start()
        return carry
    jax.lax.fori_loop(0, PRE // MB, post_chunk, 0)
    for cp in out_copies(0, NSEG, 0, XR):
        cp.wait()
    for i in range(PRE // MB):
        for cp in out_copies(i * 16, 16, XR, TL):
            cp.wait()


@functools.partial(jax.jit, static_argnames=("B_seg_len",))
def pallas_gated_mix__ssm_conv_h3__memory_aug_recurrent_mem_tr__prompt_kernel(
    A_q, A_k, A_v, A_shift_k, A_ssm_k, A_ssm_D, B_x, B_mem0, B_Wq, B_Wk, B_Wv, B_Wo,
    B_seg_len, gate_w,
):
    del B_x
    assert B_seg_len == SEG and A_q.shape == (1, S, D) and B_Wq.shape == (D, H, DH)
    assert A_shift_k.shape == (D, KS) and B_mem0.shape == (1, MEM, D)
    fwd, inv = _dft_tables()
    hbm = pl.BlockSpec(memory_space=pl.ANY)
    out = pl.pallas_call(
        _kernel,
        out_shape=jax.ShapeDtypeStruct((NSEG, SEG, D), BF16),
        in_specs=[hbm] * 15,
        out_specs=hbm,
        scratch_shapes=[
            pltpu.VMEM((NC, S, 128), BF16),
            pltpu.VMEM((NC, NSEG, TL, 128), BF16),
            pltpu.VMEM((28, PRE // 4, 128), U32),
            pltpu.VMEM((10, D // 4, 128), U32),
            pltpu.VMEM((NC, 64 + S, 128), BF16),
            pltpu.VMEM((NC + 2, S, 128), BF16),
            pltpu.VMEM((NC, 128, S), BF16),
            pltpu.VMEM((3, D, 8, 128), BF16),
            pltpu.VMEM((3 * H, D // 2, 128), U32),
            pltpu.VMEM((4 * NC, D // 2, 128), U32),
            pltpu.VMEM((5 * NC, D // 2, 128), U32),
            pltpu.VMEM((2 * H, TL, 128), F32),
            pltpu.VMEM((NC, H * DH, 128), BF16),
            pltpu.VMEM((NSEG, 3 * H // 2 * 8, 128), U32),
            pltpu.VMEM((12, 32, 128), U32),
            pltpu.VMEM((12, 32, 128), U32),
            pltpu.VMEM((12, 32, 128), U32),
            pltpu.VMEM((12, 32, 128), U32),
            pltpu.VMEM((7 * H // 2, PRE // 2, 128), BF16),
            pltpu.VMEM((NC + 1, NSEG, SEG, 128), BF16),
            pltpu.VMEM((H, 16, 128), U32),
            pltpu.VMEM((NC, MEM + XR, 128), F32),
            pltpu.VMEM((MEM, D), F32),
            pltpu.VMEM((96, 128), F32),
            pltpu.VMEM((2, 96, 128), U32),
            pltpu.VMEM((1, 96, 128), F32),
            pltpu.VMEM((H // 2, 64, NR), U32),
            pltpu.VMEM((16, 1024, 128), F32),
            pltpu.VMEM((2 * NB * CB, 128), U32),
            pltpu.VMEM((NSEG, SEG, 128), F32),
            pltpu.VMEM((CB, CB), U32),
            pltpu.VMEM((2, CB // 2, CB), U32),
            pltpu.VMEM((MEM, D), BF16),
            pltpu.VMEM((NC, KS, 128), BF16),
            pltpu.VMEM((NC, 128), BF16),
            pltpu.VMEM((NC, 128), BF16),
            pltpu.SemaphoreType.DMA((11,)),
            pltpu.SemaphoreType.DMA((3,)),
        ],
        compiler_params=pltpu.CompilerParams(vmem_limit_bytes=120 * 1024 * 1024, disable_bounds_checks=True, disable_semaphore_checks=True),
    )(
        A_q.reshape(S, D), A_q.reshape(NSEG, SEG, D), A_k.reshape(S, D), A_v.reshape(S, D), A_ssm_k,
        B_Wq, B_Wk, B_Wv, B_Wo.reshape(H * DH, D),
        A_shift_k.T.reshape(KS, NC, 128).transpose(1, 0, 2),
        A_ssm_D.reshape(NC, 128), gate_w.reshape(NC, 128),
        B_mem0.reshape(MEM, D),
        jnp.asarray(fwd), jnp.asarray(inv),
    )
    return out.reshape(1, S, D)
```

```python
import functools

import jax
import jax.numpy as jnp
import numpy as np
import jax.experimental.pallas as pl
import jax.experimental.pallas.tpu as pltpu

F32 = jnp.float32
BF16 = jnp.bfloat16
U32 = jnp.uint32
I32 = jnp.int32

S = 2048
D = 1024
NC = D // 128
H = 32
DH = 128
MEM = 8
SEG = 32
NSEG = S // SEG
XR = 24
PRE = S - NSEG * XR
TL = SEG - XR
NR = 2 * (SEG + MEM)
CB = 128
NB = S // CB
KS = 4
KPAD = 16
MB = 128
SST = 9
SB = 64
NEV = 28 * 256 // SB
MAC_G = 3


def _expand(text):
    out = []
    for item in text.split():
        if "-" in item:
            a, b = item[1:].split("-")
            out += [(item[0], i) for i in range(int(a), int(b) + 1)]
        else:
            out.append((item[0], int(item[1:] or 0)))
    return out


PROGRAM = _expand("P0-4 S0-3 P5-8 V0-3 S4-7 P9-10 O0 P11-12 V4-7 S8-11 P13 O1 P14-15 "
                  "O2 V8-11 S12-15 O3 O4 V12-15 O5 O6 O7 I F")


def _dft_tables():
    f = np.concatenate([np.arange(0, CB, 2), np.arange(1, CB, 2)]).astype(np.float64)
    t = np.arange(CB, dtype=np.float64)
    ang = 2.0 * np.pi * (f[:, None] + 0.5) * t[None, :] / (2 * CB)
    fwd = np.concatenate([np.cos(ang), -np.sin(ang)], axis=0)
    inv = np.concatenate([np.cos(ang).T, -np.sin(ang).T], axis=1) / CB

    def words(m):
        u = np.asarray(m, dtype=BF16).view(np.uint16).astype(np.uint32)
        return u[0::2] | (u[1::2] << 16)
    return words(fwd), np.stack([words(inv[:, :CB]), words(inv[:, CB:])])


def _dot(a, b):
    return jnp.dot(a, b, preferred_element_type=F32)


def _dot_nt(a, b):
    return jax.lax.dot_general(a, b, (((1,), (1,)), ((), ())), preferred_element_type=F32)


def _mo(x, m):
    return x if isinstance(x, int) else pl.multiple_of(x, m)


def _tie(x, gate):
    return x if gate is None else pltpu.bitcast(pltpu.bitcast(x, I32) | gate, x.dtype)


def _gate(token, zero):
    return pltpu.bitcast(token, I32) & jnp.full((8, 128), zero, I32)


def _unpack(words):
    return pltpu.bitcast(words, BF16).astype(F32)


def _pack(val):
    return pltpu.bitcast(val.astype(BF16), U32)


def _zero_of(counter):
    return jax.lax.shift_right_logical(counter, 16)


def _kernel(x_hbm, x3_hbm, k_hbm, v_hbm, ssm_hbm, wq_hbm, wk_hbm, wv_hbm, wo_hbm,
            shift_hbm, dskip_hbm, gate_hbm, mem0_hbm, fwd_hbm, inv_hbm,
            out_hbm,
            xs, xpre, xpk, wsum, ks, vs, ssm, wraw, wts, wos, wosum, otail, wpark, prebuf, yb0, yb1, yb2, yb3, obuf, outb, olhs, oacc,
            mem, small, stage, fbuf, ebuf, spec, zspec, gbuf,
            fwd_ref, inv_ref, mem0_ref, shift_ref, dskip_ref, gate_ref,
            sems, sem_w):
    w_hbm = (wq_hbm, wk_hbm, wv_hbm)
    ybufs = (yb0, yb1, yb2, yb3)

    def x_copy(c):
        return pltpu.make_async_copy(x_hbm.at[:, pl.ds(c * 128, 128)], xs.at[c], sems.at[2])

    def xt_copy(c, part):
        s0, n, si = ((0, 16, 0), (16, NSEG - 16, 10))[part]
        return pltpu.make_async_copy(x3_hbm.at[pl.ds(s0, n), pl.ds(XR, TL), pl.ds(c * 128, 128)],
                                     xpre.at[c, pl.ds(s0, n)], sems.at[si])

    def conv_copies(c):
        col = pl.ds(c * 128, 128)
        sem = sems.at[(2, 0, 3)[min(c, 2)]]
        return [pltpu.make_async_copy(k_hbm.at[:, col], ks.at[c, pl.ds(KPAD, S), :], sem),
                pltpu.make_async_copy(v_hbm.at[:, col], vs.at[c + 1], sem),
                pltpu.make_async_copy(ssm_hbm.at[col, :], ssm.at[c], sem)]

    def wo_copy(c):
        return pltpu.make_async_copy(wo_hbm.at[:, pl.ds(_mo(c * 128, 128), 128)], wpark.at[c], sems.at[1])

    def w_copy(t, g, slot):
        return pltpu.make_async_copy(w_hbm[t].at[:, pl.ds(_mo(g * 8, 8), 8), :], wraw.at[slot], sem_w.at[slot])

    def w0_copy(i):
        return pltpu.make_async_copy(wq_hbm.at[pl.ds(i * 256, 256), pl.ds(0, 8), :],
                                     wraw.at[0, pl.ds(i * 256, 256)], sems.at[5 + i])

    small_copies = [pltpu.make_async_copy(a, b, sems.at[9]) for a, b in (
        (shift_hbm, shift_ref), (dskip_hbm, dskip_ref), (gate_hbm, gate_ref),
        (mem0_hbm, mem0_ref), (fwd_hbm, fwd_ref), (inv_hbm, inv_ref))]

    late_copies = conv_copies(0) + [x_copy(c) for c in range(NC)]

    for i in range(4):
        w0_copy(i).start()
    for c in range(NC):
        xt_copy(c, 0).start()

    vs[0] = jnp.zeros((S, 128), BF16)
    outb[0] = jnp.zeros((NSEG, SEG, 128), BF16)
    zspec[NB * CB:2 * NB * CB, :] = jnp.zeros((NB * CB, 128), U32)

    def clear(c, count):
        ks[c, 0:KPAD, :] = jnp.zeros((KPAD, 128), BF16)
        outb[c + 1] = jnp.zeros((NSEG, SEG, 128), BF16)
        return count + 1

    def relayout_piece(c, slot, q, gate=None):
        ws = [pltpu.bitcast(wraw[slot, q * 16 + 2 * i:q * 16 + 2 * i + 2].reshape(16, 128), U32)
              for i in range(8)]
        if isinstance(c, int):
            st = stage.at[q % 2]
            for i in range(8):
                st[i * SST:i * SST + 8, :] = _tie(ws[i], gate if i == 0 else None)
            tr = [st[pl.ds(j, 8, stride=SST), :] for j in range(8)]
        else:
            ws = [_tie(w, gate if i % 2 == 0 else None) for i, w in enumerate(ws)]
            tr = jnp.transpose(jnp.stack(ws, axis=0), (1, 0, 2))
        for j in range(4):
            ev, od = tr[j], tr[4 + j]
            wts[c * 8 + 2 * j, q * 8:(q + 1) * 8, :] = (ev & jnp.uint32(0xFFFF)) | (od << 16)
            wts[c * 8 + (2 * j + 1), q * 8:(q + 1) * 8, :] = (ev >> 16) | (od & jnp.uint32(0xFFFF0000))

    def relayout_with(y, zero, c, slot, d, span):
        qs = range(min(64 * d // span, 64), min(64 * (d + 1) // span, 64))
        for i, q in enumerate(qs):
            o = (i * MB // len(qs)) // 8 * 8
            relayout_piece(c, slot, q, _gate(y[o:o + 8], zero))

    pend = [None]

    def store_pair(c, pp, seg0, ya, yb):
        for i in range(ya.shape[0] // 8):
            pair = jnp.concatenate([ya[8 * i:8 * i + 8], yb[8 * i:8 * i + 8]], axis=0)
            prebuf[seg0 + i, pl.ds(_mo(c * 32, 32) + pp * 8, 8), :] = pltpu.bitcast(pair.astype(BF16), U32)

    def first_mm(d):
        pp, rb, hb = d // 8, (d // 2) % 4, d % 2
        w = pltpu.bitcast(wts[2 * pp + hb], BF16)
        xp = jnp.concatenate([xpre[cc, rb * 16:(rb + 1) * 16].reshape(MB, 128) for cc in range(NC)], axis=1)
        y = _dot(xp, w)
        if hb == 0:
            pend[0] = y
        else:
            store_pair(0, pp, rb * 16, pend[0], y)
        return y

    def lhs_piece(cc, sg, gate):
        def ld(c2, s2):
            return pltpu.bitcast(xpre[c2, s2:s2 + 2].reshape(16, 128), U32)
        w11, w12, w21, w22 = ld(cc, sg), ld(cc + 4, sg), ld(cc, sg + 32), ld(cc + 4, sg + 32)
        w11, w22 = _tie(w11, gate), _tie(w22, gate)
        a11, a12, a21, a22 = _unpack(w11), _unpack(w12), _unpack(w21), _unpack(w22)
        vals = (_pack(a11 + a12), _pack(a21 + a22), w11, w22, _pack(a11 + a22), _pack(a12 - a22), _pack(a21 - a11))
        for k, val in enumerate(vals):
            xpk[k * 4 + cc, sg * 4:sg * 4 + 8, :] = val

    def rhs_sums(w11, w12, w21, w22, gate):
        b11, b12, b21, b22 = _unpack(_tie(w11, gate)), _unpack(w12), _unpack(w21), _unpack(_tie(w22, gate))
        return [_pack(v) for v in (b12 - b22, b21 - b11, b11 + b22, b21 + b22, b11 + b12)]

    def rhs_piece(hd, par, r, gate):
        sums = rhs_sums(wts[hd, r:r + 8, :], wts[hd + 1, r:r + 8, :],
                        wts[hd, 256 + r:264 + r, :], wts[hd + 1, 256 + r:264 + r, :], gate)
        for k, val in enumerate(sums):
            wsum[par * 5 + k, r:r + 8, :] = val

    def strassen_chunk(c, zero, extra, last=False):
        nrb = 256 // SB
        e = 0
        for pp in range(4):
            for rb in range(nrb):
                ms = []
                for k in range(7):
                    a = jnp.concatenate([xpk[k * 4 + cc, rb * (SB // 2):(rb + 1) * (SB // 2), :] for cc in range(4)], axis=1)
                    if k == 0:
                        b = wts[c * 8 + (2 * pp + 1), 256:512, :]
                    elif k == 1:
                        b = wts[c * 8 + 2 * pp, 0:256, :]
                    else:
                        b = wsum[(pp % 2) * 5 + k - 2]
                    y = _dot(pltpu.bitcast(a, BF16), pltpu.bitcast(b, BF16))
                    ms.append(y)
                    if k == 5:
                        m5, m2, m3, m4, m1, m7 = ms
                        store_pair(c, pp, rb * (SB // 8), ((m4 - m5) + m1) + m7, m5 + m3)
                    if k == 6:
                        store_pair(c, pp, 32 + rb * (SB // 8), m2 + m4, ((m3 - m2) + m1) + y)
                    extra(e, y)
                    le = e % (7 * nrb)
                    cbe = 6 * nrb
                    if not (last and pp == 3):
                        for i, r in enumerate(range(min(32 * le // cbe, 32), min(32 * (le + 1) // cbe, 32))):
                            o = (8 * (2 * i + 1)) % SB
                            rhs_piece(c * 8 + (2 * pp + 2), (pp + 1) % 2, r * 8, _gate(y[o:o + 8], zero))
                    e += 1

    count = 0
    for i in range(4):
        count = jax.lax.fori_loop(2 * i, 2 * i + 2, clear, count)
        w0_copy(i).wait()
        if i == 0:
            for c in range(NC):
                xt_copy(c, 1).start()
        if i == 1:
            for t in range(1, 3):
                w_copy(t, 0, t).start()
        for q in range(16 * i, 16 * i + 16):
            relayout_piece(0, 0, q)
    w_copy(0, 1, 0).start()
    for cp in small_copies:
        cp.start()
    for c in range(NC):
        xt_copy(c, 0).wait()

    for e in range(32):
        if e == 8:
            for c in range(NC):
                xt_copy(c, 1).wait()
        if e == 24:
            w_copy(1, 0, 1).wait()
        y = first_mm(((e % 8) // 2) * 8 + (e // 8) * 2 + e % 2)
        if 8 <= e < 24:
            for i in range(4):
                lhs_piece((e - 8) // 4, ((e % 4) * 4 + i) * 2, _gate(y[32 * i:32 * i + 8], _zero_of(count)))
        if e >= 24:
            relayout_with(y, _zero_of(count), 1, 1, e - 24, 7)
    for r in range(32):
        rhs_piece(8, 0, r * 8, None)
    w_copy(1, 1, 1).start()
    wo_copy(0).start()

    def pre_chunk(c, carry, packwo):
        tn, gn = carry
        zero = _zero_of(tn)
        w_copy(0, 0, tn).wait()

        def extra(e, y):
            rle = 78 * NEV // 112
            for i, q in enumerate(range(min(64 * e // rle, 64), min(64 * (e + 1) // rle, 64))):
                relayout_piece(c + 1, tn, q, _gate(y[16 * i:16 * i + 8], zero))
            if packwo:
                gate = _gate(y[SB - 8:SB], zero)
                for v in range(min(1024 * e // (NEV - 2), 1024), min(1024 * (e + 1) // (NEV - 2), 1024)):
                    sl, r = v // 64, (v % 64) * 8
                    o = (sl % 4) * 1024 + 2 * r
                    wos[(c - 9) * 16 + sl, r:r + 8, :] = _tie(
                        pltpu.bitcast(wpark[(c - 9) * 4 + sl // 4, o:o + 16, :], U32), gate)
        strassen_chunk(c, zero, extra)
        if not packwo:
            for t in range(3):
                @pl.when(jnp.logical_and(tn == t, gn < 3))
                def _():
                    w_copy(t, gn + 1, t).start()

            @pl.when(c < NC)
            def _():
                wo_copy(c).start()

        return jnp.where(tn == 2, 0, tn + 1), jnp.where(tn == 2, gn + 1, gn)

    carry = jax.lax.fori_loop(1, 9, functools.partial(pre_chunk, packwo=False), (2, 0))
    for cp in late_copies:
        cp.start()
    for c in range(NC):
        wo_copy(c).wait()
    count = jax.lax.fori_loop(9, 11, functools.partial(pre_chunk, packwo=True), carry)[1]

    for cp in small_copies:
        cp.wait()
    for cp in late_copies:
        cp.wait()
    for cp in conv_copies(1):
        cp.start()
    small[0:NC, :] = dskip_ref[...].astype(F32)
    gate_w = gate_ref[...].astype(F32)
    for c in range(NC):
        small[NC + 8 * c:NC + 8 * (c + 1), :] = jnp.broadcast_to(gate_w[c:c + 1, :], (8, 128))
    mem[...] = mem0_ref[...].astype(F32)

    def mix_gate(r0, gate):
        z = None
        for c in range(NC):
            gw = small[NC + 8 * c:NC + 8 * (c + 1), :]
            t = xs[c, r0:r0 + 16, :].astype(F32) * jnp.concatenate([gw, gw], axis=0)
            z = _tie(t, jnp.concatenate([gate, gate], axis=0)) if z is None else z + t
        z = jnp.sum(z, axis=1, keepdims=True)
        gbuf[r0 // SEG, r0 % SEG:r0 % SEG + 16, :] = jnp.broadcast_to(0.5 * jnp.tanh(0.5 * z) + 0.5, (16, 128))

    def accumulate(slab, segs, rows, val):
        old = outb[slab, segs, rows, :].astype(F32)
        outb[slab, segs, rows, :] = (old + val.astype(BF16).astype(F32).reshape(old.shape)).astype(BF16)

    def conv_prep(t, j):
        tr = t if isinstance(t, int) else jnp.minimum(t, NC - 1)
        r0 = _mo(j * 2 * CB, 2 * CB)
        shift = shift_ref[tr].astype(F32)
        gate = yield
        tail = None
        for o in range(0, 2 * CB + KPAD, 16):
            kk = ks[tr, pl.ds(r0 + o, 16), :].astype(F32)
            win = [tail, _tie(kk[0:8], gate), _tie(kk[8:16], gate)]
            tail = win[2]
            if o == 0:
                continue
            win = jnp.concatenate(win, axis=0)
            acc = win[8:24] * shift[0:1, :]
            for l in range(1, KS):
                acc = acc + win[8 - l:24 - l] * shift[l:l + 1, :]
            rows = pl.ds(r0 + (o - KPAD), 16)
            vs[t + 1, rows, :] = (acc * vs[tr + 1, rows, :].astype(F32)).astype(BF16)
            gate = yield

    def conv_fwd(t, j):
        tr = t if isinstance(t, int) else jnp.minimum(t, NC - 1)
        slot = t & 1
        fwd = pltpu.bitcast(fwd_ref[...], BF16)
        for i in range(2):
            rows = pl.ds(_mo((2 * j + i) * CB, CB), CB)
            sr = _mo((2 * j + i) * 32, 32)
            for off, res in ((0, _dot(fwd, vs[t + 1, rows, :])), (512, _dot_nt(fwd, ssm[tr, :, rows]))):
                for ri in range(2):
                    for fj in range(8):
                        spec[slot * 8 + fj, pl.ds(sr + (off + ri * 16), 16), :] = (
                            res[ri * CB + fj * 16:ri * CB + (fj + 1) * 16])

    def conv_mac(t, j, zero):
        slot = t & 1
        sign = jnp.where(j < 4, 1.0, -1.0).astype(F32)
        zbase = pl.multiple_of(slot * (NB * CB) + j * 8, 8)
        prev = None
        gate = yield
        for i in range(NB):
            base = slot * 8 + j + zero * (i + 1)
            ys = []
            for hv in range(2):
                yr = yi = None
                for jj in range(i + 1):
                    uo = jj * 32 + hv * 8
                    ko = 512 + (i - jj) * 32 + hv * 8
                    ur = spec[base, uo:uo + 8, :]
                    ui = spec[base, uo + 16:uo + 24, :]
                    kr = spec[base, ko:ko + 8, :]
                    ki = spec[base, ko + 16:ko + 24, :]
                    tr, ti = _tie(ur * kr - ui * ki, gate), _tie(ur * ki + ui * kr, gate)
                    yr, yi = (tr, ti) if yr is None else (yr + tr, yi + ti)
                    if jj < i or hv == 0:
                        gate = yield
                ys.append((yr, yi))
            yr = jnp.concatenate([ys[0][0], ys[1][0]], axis=0)
            yi = jnp.concatenate([ys[0][1], ys[1][1]], axis=0)
            zr, zi = (yr, yi) if prev is None else (yr - sign * prev[1], yi + sign * prev[0])
            prev = (yr, yi)
            zspec[pl.ds(zbase + i * CB, 8), :] = pltpu.bitcast(zr.astype(BF16), U32)
            zspec[pl.ds(zbase + (i * CB + CB // 2), 8), :] = pltpu.bitcast(zi.astype(BF16), U32)
            gate = yield

    def conv_inv(t, j):
        tr = t if isinstance(t, int) else jnp.maximum(t, 0)
        slot = t & 1
        dsk = small[pl.ds(tr, 1), :]
        inv = pltpu.bitcast(jnp.concatenate([inv_ref[0], inv_ref[1]], axis=1), BF16)
        for i in range(2):
            rows = pl.ds(_mo((2 * j + i) * CB, CB), CB)
            z = zspec[pl.ds(_mo((slot * NB + 2 * j + i) * CB, CB), CB), :]
            y = _dot(inv, pltpu.bitcast(z, BF16))
            y = y + vs[t + 1, rows, :].astype(F32) * dsk
            segs = pl.ds((2 * j + i) * (CB // SEG), CB // SEG)
            accumulate(t + 1, segs, slice(None), gbuf[segs].reshape(CB, 128) * (xs[tr, rows, :].astype(F32) * y))

    state = {}

    def last_extra(e, y):
        for i, q in enumerate(range(128 * e // NEV, 128 * (e + 1) // NEV)):
            if q % 16 == 0:
                state["prep"] = conv_prep(0, q // 16)
                next(state["prep"])
            if q % 16 == 5 and q >= 16:
                conv_fwd(0, q // 16 - 1)
            gate = _gate(y[16 * i:16 * i + 8], _zero_of(count))
            state["prep"].send(gate)
            mix_gate(q * 16, gate)
    strassen_chunk(11, _zero_of(count), last_extra, last=True)
    conv_fwd(0, NB // 2 - 1)

    ri = jax.lax.broadcasted_iota(I32, (NR, NR), 0)
    ci = jax.lax.broadcasted_iota(I32, (NR, NR), 1)
    LD = MEM + XR

    def head_pos(i):
        tail = i >= 2 * LD
        return (jnp.where(tail, (i - 2 * LD) // TL, i // LD),
                jnp.where(tail, LD + (i - 2 * LD) % TL, i % LD))
    (rh, rp), (ch, cp_) = head_pos(ri), head_pos(ci)
    same = rh == ch
    keep = same & ((rp < MEM) | (rp >= cp_))
    fbuf[0, 0:NR, 0:NR] = jnp.where(keep, 0.0, jnp.where(same, -1000000000.0, -jnp.inf)).astype(F32)
    scale = float(DH) ** -0.5

    def step(it, u, zero):
        s = it * 2 + u
        ct = jax.lax.shift_right_logical(s, 3)
        cj = jnp.bitwise_and(s, 7)
        xr0 = pl.multiple_of(it * (2 * SEG), 2 * SEG) + u * SEG
        h_lhs = jnp.concatenate(
            [jnp.concatenate([mem[:, c * 128:(c + 1) * 128], xs[c, pl.ds(xr0, XR), :].astype(F32)],
                             axis=0).astype(BF16) for c in range(NC)], axis=1)

        macs = conv_mac(ct, cj, zero)
        next(macs)
        preps = conv_prep(ct + 1, cj)
        next(preps)
        n_mac = NB * (NB + 1)

        def wo_sums():
            npair, kq = s >> 4, (s >> 3) & 1
            gate = yield
            for i in range(8):
                rows = pl.ds(pl.multiple_of((s & 7) * 64, 64) + 8 * i, 8)
                sl = npair * 8 + kq
                sums = rhs_sums(wos[sl, rows, :], wos[sl + 4, rows, :], wos[sl + 2, rows, :], wos[sl + 6, rows, :], gate)
                for k, val in enumerate(sums):
                    wosum[npair * 10 + kq + 2 * k, rows, :] = val
                gate = yield

        def tail_sums():
            rows = pl.ds(pl.multiple_of(it * TL, TL), TL)
            gate = yield
            for hh in range(H // 2):
                a11, a22 = _tie(otail[hh], gate), _tie(otail[H + H // 2 + hh], gate)
                a12, a21 = otail[H // 2 + hh], otail[H + hh]
                for k, val in enumerate((a11 + a12, a21 + a22, a11, a22, a11 + a22, a12 - a22, a21 - a11)):
                    obuf[k * (H // 2) + hh, rows, :] = val.astype(BF16)
                gate = yield

        wsums = wo_sums()
        next(wsums)
        queue = ([(preps, 1)] * 16 + [(macs, min(MAC_G, n_mac - n)) for n in range(0, n_mac, MAC_G)]
                 + [(wsums, 1)] * 8)

        def side_work(token):
            if queue:
                gen, cnt = queue.pop(0)
                if gen is None:
                    return
                gen.send(_gate(token, zero))
                for _ in range(cnt - 1):
                    gen.send(None)

        def proj(p):
            for t in range(3):
                for i, hh in enumerate((2 * p, 2 * p + 1)):
                    y = _dot(h_lhs, pltpu.bitcast(wts[(hh // 8) * 24 + t * 8 + hh % 8], BF16))
                    side_work(y[0:MEM])
                    ybufs[p // 4][t * 4 + p % 4 + zero, i * 16:(i + 1) * 16, :] = pltpu.bitcast(y.astype(BF16), U32)

        def rows_of(t, p):
            o = ((p // 4) * 12 + t * 4 + p % 4) * 8
            return pltpu.bitcast(jnp.concatenate([ybufs[p // 4][t * 4 + p % 4], prebuf[s, o:o + 8, :]], axis=0), BF16)

        def scores(p):
            sc = _dot_nt(rows_of(0, p), rows_of(1, p)) * scale
            fill = fbuf[zero * (p + 1), 0:NR, 0:NR]
            sc = jnp.where(fill == 0.0, sc, fill)
            e = jnp.exp(sc - jnp.max(sc, axis=1, keepdims=True))
            l = jnp.sum(e, axis=1, keepdims=True)
            r = pl.reciprocal(l, approx=True)
            ebuf[p + zero, 0:NR // 2, :] = pltpu.bitcast(e.astype(BF16), U32)
            return r * (2.0 - l * r)

        def values(p, r):
            o = _dot(pltpu.bitcast(ebuf[p, 0:NR // 2, :], BF16), rows_of(2, p)) * r
            for i, hh in enumerate((2 * p, 2 * p + 1)):
                olhs[hh] = pltpu.bitcast(o[i * LD:(i + 1) * LD].astype(BF16), U32)
                otail[u * H + hh + zero] = o[2 * LD + i * TL:2 * LD + (i + 1) * TL].astype(BF16).astype(F32)

        def oproj(g):
            lhs = pltpu.bitcast(jnp.concatenate([olhs[hh] for hh in range(4 * g, 4 * g + 4)], axis=1), BF16)
            for n in range(NC):
                w = wos[4 * n + g // 2, (g % 2) * 256:(g % 2 + 1) * 256, :]
                y = _dot(lhs, pltpu.bitcast(w, BF16))
                side_work(y[0:MEM])
                if g > 0:
                    y = y + oacc[n + zero]
                if g < H // 4 - 1:
                    oacc[n] = y
                else:
                    mem[:, n * 128:(n + 1) * 128] = y[0:MEM].astype(BF16).astype(F32)
                    accumulate(n + 1, s, slice(0, XR),
                               (1.0 - gbuf[s, 0:XR, :]) * y[MEM:].astype(BF16).astype(F32))

        recip = [None] * (H // 2)
        for op, arg in PROGRAM:
            if op == "P":
                proj(arg)
            elif op == "S":
                recip[arg] = scores(arg)
            elif op == "V":
                values(arg, recip[arg])
                if u == 1 and arg == H // 2 - 1:
                    assert not queue
                    tsums = tail_sums()
                    next(tsums)
                    queue.extend([(None, 0)] * 4 + [(tsums, 1)] * (H // 2))
            elif op == "O":
                oproj(arg)
            elif op == "I":
                conv_inv(ct - 1, cj)
            else:
                assert not queue
                conv_fwd(ct + 1, cj)

    def two_steps(it, carry):
        for u in range(2):
            step(it, u, _zero_of(carry))

        @pl.when(it == 3)
        def _():
            for c in range(2, NC):
                for cp in conv_copies(c):
                    cp.wait()
        return carry + 1
    for cp in conv_copies(1):
        cp.wait()
    for c in range(2, NC):
        for cp in conv_copies(c):
            cp.start()
    jax.lax.fori_loop(0, NSEG // 2, two_steps, count)

    for j in range(NB // 2):
        conv_inv(NC - 1, j)

    def out_copies(s0, n, r0, nr):
        return [pltpu.make_async_copy(outb.at[c + 1, pl.ds(s0, n), pl.ds(r0, nr), :],
                                      out_hbm.at[pl.ds(s0, n), pl.ds(r0, nr), pl.ds(c * 128, 128)], sems.at[4])
                for c in range(NC)]

    for cp in out_copies(0, NSEG, 0, XR):
        cp.start()

    def post_chunk(i, carry):
        rows = pl.ds(pl.multiple_of(i * 64, 64), 64)

        def finish(n, par, y):
            for j in range(8):
                sg = i * 16 + (2 * j + par)
                accumulate(n + 1, sg, slice(XR, SEG),
                           (1.0 - gbuf[sg, XR:SEG, :]) * y[8 * j:8 * j + 8].astype(BF16).astype(F32))

        for npair in range(NC // 2):
            ms = []
            for k in range(7):
                a = jnp.concatenate([obuf[k * (H // 2) + hh, rows, :] for hh in range(H // 2)], axis=1)
                if k == 0:
                    b = [wos[npair * 8 + 6], wos[npair * 8 + 7]]
                elif k == 1:
                    b = [wos[npair * 8], wos[npair * 8 + 1]]
                else:
                    b = [wosum[npair * 10 + 2 * (k - 2)], wosum[npair * 10 + 2 * (k - 2) + 1]]
                ms.append(_dot(a, pltpu.bitcast(jnp.concatenate(b, axis=0), BF16)))
                if k == 2:
                    finish(2 * npair + 1, 0, ms[0] + ms[2])
                if k == 3:
                    finish(2 * npair, 1, ms[1] + ms[3])
                if k == 5:
                    finish(2 * npair, 0, ((ms[3] - ms[0]) + ms[4]) + ms[5])
                if k == 6:
                    finish(2 * npair + 1, 1, ((ms[2] - ms[1]) + ms[4]) + ms[6])
        for cp in out_copies(i * 16, 16, XR, TL):
            cp.start()
        return carry
    jax.lax.fori_loop(0, PRE // MB, post_chunk, 0)
    for cp in out_copies(0, NSEG, 0, XR):
        cp.wait()
    for i in range(PRE // MB):
        for cp in out_copies(i * 16, 16, XR, TL):
            cp.wait()


@functools.partial(jax.jit, static_argnames=("B_seg_len",))
def pallas_gated_mix__ssm_conv_h3__memory_aug_recurrent_mem_tr__prompt_kernel(
    A_q, A_k, A_v, A_shift_k, A_ssm_k, A_ssm_D, B_x, B_mem0, B_Wq, B_Wk, B_Wv, B_Wo,
    B_seg_len, gate_w,
):
    del B_x
    assert B_seg_len == SEG and A_q.shape == (1, S, D) and B_Wq.shape == (D, H, DH)
    assert A_shift_k.shape == (D, KS) and B_mem0.shape == (1, MEM, D)
    fwd, inv = _dft_tables()
    hbm = pl.BlockSpec(memory_space=pl.ANY)
    out = pl.pallas_call(
        _kernel,
        out_shape=jax.ShapeDtypeStruct((NSEG, SEG, D), BF16),
        in_specs=[hbm] * 15,
        out_specs=hbm,
        scratch_shapes=[
            pltpu.VMEM((NC, S, 128), BF16),
            pltpu.VMEM((NC, NSEG, TL, 128), BF16),
            pltpu.VMEM((28, PRE // 4, 128), U32),
            pltpu.VMEM((10, D // 4, 128), U32),
            pltpu.VMEM((NC, 64 + S, 128), BF16),
            pltpu.VMEM((NC + 2, S, 128), BF16),
            pltpu.VMEM((NC, 128, S), BF16),
            pltpu.VMEM((3, D, 8, 128), BF16),
            pltpu.VMEM((3 * H, D // 2, 128), U32),
            pltpu.VMEM((4 * NC, D // 2, 128), U32),
            pltpu.VMEM((5 * NC, D // 2, 128), U32),
            pltpu.VMEM((2 * H, TL, 128), F32),
            pltpu.VMEM((NC, H * DH, 128), BF16),
            pltpu.VMEM((NSEG, 3 * H // 2 * 8, 128), U32),
            pltpu.VMEM((12, 32, 128), U32),
            pltpu.VMEM((12, 32, 128), U32),
            pltpu.VMEM((12, 32, 128), U32),
            pltpu.VMEM((12, 32, 128), U32),
            pltpu.VMEM((7 * H // 2, PRE // 2, 128), BF16),
            pltpu.VMEM((NC + 1, NSEG, SEG, 128), BF16),
            pltpu.VMEM((H, 16, 128), U32),
            pltpu.VMEM((NC, MEM + XR, 128), F32),
            pltpu.VMEM((MEM, D), F32),
            pltpu.VMEM((96, 128), F32),
            pltpu.VMEM((2, 96, 128), U32),
            pltpu.VMEM((1, 96, 128), F32),
            pltpu.VMEM((H // 2, 64, NR), U32),
            pltpu.VMEM((16, 1024, 128), F32),
            pltpu.VMEM((2 * NB * CB, 128), U32),
            pltpu.VMEM((NSEG, SEG, 128), F32),
            pltpu.VMEM((CB, CB), U32),
            pltpu.VMEM((2, CB // 2, CB), U32),
            pltpu.VMEM((MEM, D), BF16),
            pltpu.VMEM((NC, KS, 128), BF16),
            pltpu.VMEM((NC, 128), BF16),
            pltpu.VMEM((NC, 128), BF16),
            pltpu.SemaphoreType.DMA((11,)),
            pltpu.SemaphoreType.DMA((3,)),
        ],
        compiler_params=pltpu.CompilerParams(vmem_limit_bytes=120 * 1024 * 1024, disable_bounds_checks=True, disable_semaphore_checks=True),
    )(
        A_q.reshape(S, D), A_q.reshape(NSEG, SEG, D), A_k.reshape(S, D), A_v.reshape(S, D), A_ssm_k,
        B_Wq, B_Wk, B_Wv, B_Wo.reshape(H * DH, D),
        A_shift_k.T.reshape(KS, NC, 128).transpose(1, 0, 2),
        A_ssm_D.reshape(NC, 128), gate_w.reshape(NC, 128),
        B_mem0.reshape(MEM, D),
        jnp.asarray(fwd), jnp.asarray(inv),
    )
    return out.reshape(1, S, D)
```

```python
import functools

import jax
import jax.numpy as jnp
import numpy as np
import jax.experimental.pallas as pl
import jax.experimental.pallas.tpu as pltpu

F32 = jnp.float32
BF16 = jnp.bfloat16
U32 = jnp.uint32
I32 = jnp.int32

S = 2048
D = 1024
NC = D // 128
H = 32
DH = 128
MEM = 8
SEG = 32
NSEG = S // SEG
XR = 24
PRE = S - NSEG * XR
TL = SEG - XR
NR = 2 * (SEG + MEM)
CB = 128
NB = S // CB
KS = 4
KPAD = 16
MB = 128
SST = 9
SB = 64
NEV = 28 * 256 // SB
MAC_G = 3


def _expand(text):
    out = []
    for item in text.split():
        if "-" in item:
            a, b = item[1:].split("-")
            out += [(item[0], i) for i in range(int(a), int(b) + 1)]
        else:
            out.append((item[0], int(item[1:] or 0)))
    return out


PROGRAM = _expand("P0-4 S0-3 P5-8 V0-3 S4-7 P9-10 O0 P11-12 V4-7 S8-11 P13 O1 P14-15 "
                  "O2 V8-11 S12-15 O3 O4 V12-15 O5 O6 O7 I F")


def _dft_tables():
    f = np.concatenate([np.arange(0, CB, 2), np.arange(1, CB, 2)]).astype(np.float64)
    t = np.arange(CB, dtype=np.float64)
    ang = 2.0 * np.pi * (f[:, None] + 0.5) * t[None, :] / (2 * CB)
    fwd = np.concatenate([np.cos(ang), -np.sin(ang)], axis=0)
    inv = np.concatenate([np.cos(ang).T, -np.sin(ang).T], axis=1) / CB

    def words(m):
        u = np.asarray(m, dtype=BF16).view(np.uint16).astype(np.uint32)
        return u[0::2] | (u[1::2] << 16)
    return words(fwd), np.stack([words(inv[:, :CB]), words(inv[:, CB:])])


def _dot(a, b):
    return jnp.dot(a, b, preferred_element_type=F32)


def _dot_nt(a, b):
    return jax.lax.dot_general(a, b, (((1,), (1,)), ((), ())), preferred_element_type=F32)


def _mo(x, m):
    return x if isinstance(x, int) else pl.multiple_of(x, m)


def _tie(x, gate):
    return x if gate is None else pltpu.bitcast(pltpu.bitcast(x, I32) | gate, x.dtype)


def _gate(token, zero):
    return pltpu.bitcast(token, I32) & jnp.full((8, 128), zero, I32)


def _unpack(words):
    return pltpu.bitcast(words, BF16).astype(F32)


def _pack(val):
    return pltpu.bitcast(val.astype(BF16), U32)


def _zero_of(counter):
    return jax.lax.shift_right_logical(counter, 16)


def _kernel(x_hbm, x3_hbm, k_hbm, v_hbm, ssm_hbm, wq_hbm, wk_hbm, wv_hbm, wo_hbm,
            shift_hbm, dskip_hbm, gate_hbm, mem0_hbm, fwd_hbm, inv_hbm,
            out_hbm,
            xs, xpre, xpk, wsum, ks, vs, ssm, wraw, wts, wos, wosum, otail, wpark, prebuf, yb0, yb1, yb2, yb3, obuf, outb, olhs, oacc,
            mem, small, stage, fbuf, ebuf, spec, zspec, gbuf,
            fwd_ref, inv_ref, mem0_ref, shift_ref, dskip_ref, gate_ref,
            sems, sem_w):
    w_hbm = (wq_hbm, wk_hbm, wv_hbm)
    ybufs = (yb0, yb1, yb2, yb3)

    def x_copy(c):
        return pltpu.make_async_copy(x_hbm.at[:, pl.ds(c * 128, 128)], xs.at[c], sems.at[2])

    def xt_copy(c, part):
        s0, n, si = ((0, 16, 0), (16, NSEG - 16, 10))[part]
        return pltpu.make_async_copy(x3_hbm.at[pl.ds(s0, n), pl.ds(XR, TL), pl.ds(c * 128, 128)],
                                     xpre.at[c, pl.ds(s0, n)], sems.at[si])

    def conv_copies(c):
        col = pl.ds(c * 128, 128)
        sem = sems.at[(2, 0, 3)[min(c, 2)]]
        return [pltpu.make_async_copy(k_hbm.at[:, col], ks.at[c, pl.ds(KPAD, S), :], sem),
                pltpu.make_async_copy(v_hbm.at[:, col], vs.at[c + 1], sem),
                pltpu.make_async_copy(ssm_hbm.at[col, :], ssm.at[c], sem)]

    def wo_copy(c):
        return pltpu.make_async_copy(wo_hbm.at[:, pl.ds(_mo(c * 128, 128), 128)], wpark.at[c], sems.at[1])

    def w_copy(t, g, slot):
        return pltpu.make_async_copy(w_hbm[t].at[:, pl.ds(_mo(g * 8, 8), 8), :], wraw.at[slot], sem_w.at[slot])

    def w0_copy(i):
        return pltpu.make_async_copy(wq_hbm.at[pl.ds(i * 256, 256), pl.ds(0, 8), :],
                                     wraw.at[0, pl.ds(i * 256, 256)], sems.at[5 + i])

    small_copies = [pltpu.make_async_copy(a, b, sems.at[9]) for a, b in (
        (shift_hbm, shift_ref), (dskip_hbm, dskip_ref), (gate_hbm, gate_ref),
        (mem0_hbm, mem0_ref), (fwd_hbm, fwd_ref), (inv_hbm, inv_ref))]

    late_copies = conv_copies(0) + [x_copy(c) for c in range(NC)]

    for i in range(4):
        w0_copy(i).start()
    for c in range(NC):
        xt_copy(c, 0).start()

    vs[0] = jnp.zeros((S, 128), BF16)
    outb[0] = jnp.zeros((NSEG, SEG, 128), BF16)
    zspec[NB * CB:2 * NB * CB, :] = jnp.zeros((NB * CB, 128), U32)

    def clear(c, count):
        ks[c, 0:KPAD, :] = jnp.zeros((KPAD, 128), BF16)
        outb[c + 1] = jnp.zeros((NSEG, SEG, 128), BF16)
        return count + 1

    def relayout_piece(c, slot, q, gate=None):
        ws = [pltpu.bitcast(wraw[slot, q * 16 + 2 * i:q * 16 + 2 * i + 2].reshape(16, 128), U32)
              for i in range(8)]
        if isinstance(c, int):
            st = stage.at[q % 2]
            for i in range(8):
                st[i * SST:i * SST + 8, :] = _tie(ws[i], gate if i == 0 else None)
            tr = [st[pl.ds(j, 8, stride=SST), :] for j in range(8)]
        else:
            ws = [_tie(w, gate if i % 2 == 0 else None) for i, w in enumerate(ws)]
            tr = jnp.transpose(jnp.stack(ws, axis=0), (1, 0, 2))
        for j in range(4):
            ev, od = tr[j], tr[4 + j]
            wts[c * 8 + 2 * j, q * 8:(q + 1) * 8, :] = (ev & jnp.uint32(0xFFFF)) | (od << 16)
            wts[c * 8 + (2 * j + 1), q * 8:(q + 1) * 8, :] = (ev >> 16) | (od & jnp.uint32(0xFFFF0000))

    def relayout_with(y, zero, c, slot, d, span):
        qs = range(min(64 * d // span, 64), min(64 * (d + 1) // span, 64))
        for i, q in enumerate(qs):
            o = (i * MB // len(qs)) // 8 * 8
            relayout_piece(c, slot, q, _gate(y[o:o + 8], zero))

    pend = [None]

    def store_pair(c, pp, seg0, ya, yb):
        for i in range(ya.shape[0] // 8):
            pair = jnp.concatenate([ya[8 * i:8 * i + 8], yb[8 * i:8 * i + 8]], axis=0)
            prebuf[seg0 + i, pl.ds(_mo(c * 32, 32) + pp * 8, 8), :] = pltpu.bitcast(pair.astype(BF16), U32)

    def first_mm(d):
        pp, rb, hb = d // 8, (d // 2) % 4, d % 2
        w = pltpu.bitcast(wts[2 * pp + hb], BF16)
        xp = jnp.concatenate([xpre[cc, rb * 16:(rb + 1) * 16].reshape(MB, 128) for cc in range(NC)], axis=1)
        y = _dot(xp, w)
        if hb == 0:
            pend[0] = y
        else:
            store_pair(0, pp, rb * 16, pend[0], y)
        return y

    def lhs_piece(cc, sg, gate):
        def ld(c2, s2):
            return pltpu.bitcast(xpre[c2, s2:s2 + 2].reshape(16, 128), U32)
        w11, w12, w21, w22 = ld(cc, sg), ld(cc + 4, sg), ld(cc, sg + 32), ld(cc + 4, sg + 32)
        w11, w22 = _tie(w11, gate), _tie(w22, gate)
        a11, a12, a21, a22 = _unpack(w11), _unpack(w12), _unpack(w21), _unpack(w22)
        vals = (_pack(a11 + a12), _pack(a21 + a22), w11, w22, _pack(a11 + a22), _pack(a12 - a22), _pack(a21 - a11))
        for k, val in enumerate(vals):
            xpk[k * 4 + cc, sg * 4:sg * 4 + 8, :] = val

    def rhs_sums(w11, w12, w21, w22, gate):
        b11, b12, b21, b22 = _unpack(_tie(w11, gate)), _unpack(w12), _unpack(w21), _unpack(_tie(w22, gate))
        return [_pack(v) for v in (b12 - b22, b21 - b11, b11 + b22, b21 + b22, b11 + b12)]

    def rhs_piece(hd, par, r, gate):
        sums = rhs_sums(wts[hd, r:r + 8, :], wts[hd + 1, r:r + 8, :],
                        wts[hd, 256 + r:264 + r, :], wts[hd + 1, 256 + r:264 + r, :], gate)
        for k, val in enumerate(sums):
            wsum[par * 5 + k, r:r + 8, :] = val

    def strassen_chunk(c, zero, extra, pairs, last=False):
        nrb = 256 // SB
        e = 0
        for pp in pairs:
            for rb in range(nrb):
                ms = []
                for k in range(7):
                    a = jnp.concatenate([xpk[k * 4 + cc, rb * (SB // 2):(rb + 1) * (SB // 2), :] for cc in range(4)], axis=1)
                    if k == 0:
                        b = wts[c * 8 + (2 * pp + 1), 256:512, :]
                    elif k == 1:
                        b = wts[c * 8 + 2 * pp, 0:256, :]
                    else:
                        b = wsum[(pp % 2) * 5 + k - 2]
                    y = _dot(pltpu.bitcast(a, BF16), pltpu.bitcast(b, BF16))
                    ms.append(y)
                    if k == 5:
                        m5, m2, m3, m4, m1, m7 = ms
                        store_pair(c, pp, rb * (SB // 8), ((m4 - m5) + m1) + m7, m5 + m3)
                    if k == 6:
                        store_pair(c, pp, 32 + rb * (SB // 8), m2 + m4, ((m3 - m2) + m1) + y)
                    extra(e, y)
                    le = e % (7 * nrb)
                    cbe = 6 * nrb
                    if not (last and pp == 3):
                        for i, r in enumerate(range(min(32 * le // cbe, 32), min(32 * (le + 1) // cbe, 32))):
                            o = (8 * (2 * i + 1)) % SB
                            rhs_piece(c * 8 + (2 * pp + 2), (pp + 1) % 2, r * 8, _gate(y[o:o + 8], zero))
                    e += 1

    count = 0
    for i in range(4):
        count = jax.lax.fori_loop(2 * i, 2 * i + 2, clear, count)
        w0_copy(i).wait()
        if i == 0:
            for c in range(NC):
                xt_copy(c, 1).start()
        if i == 1:
            for t in range(1, 3):
                w_copy(t, 0, t).start()
        for q in range(16 * i, 16 * i + 16):
            relayout_piece(0, 0, q)
    w_copy(0, 1, 0).start()
    for cp in small_copies:
        cp.start()
    for c in range(NC):
        xt_copy(c, 0).wait()

    for e in range(32):
        if e == 8:
            for c in range(NC):
                xt_copy(c, 1).wait()
        if e == 20:
            w_copy(1, 0, 1).wait()
        y = first_mm(((e % 8) // 2) * 8 + (e // 8) * 2 + e % 2)
        if 8 <= e < 24:
            for i in range(4):
                lhs_piece((e - 8) // 4, ((e % 4) * 4 + i) * 2, _gate(y[32 * i:32 * i + 8], _zero_of(count)))
        if e >= 20:
            relayout_with(y, _zero_of(count), 1, 1, e - 20, 11)
    for r in range(32):
        rhs_piece(8, 0, r * 8, None)
    w_copy(1, 1, 1).start()
    wo_copy(0).start()
    strassen_chunk(1, _zero_of(count), lambda e, y: None, range(1))

    def pre_chunk(c, carry, packwo):
        tn, gn = carry
        zero = _zero_of(tn)
        w_copy(0, 0, tn).wait()

        def extra(e, y):
            for i, q in enumerate(range(min(64 * e // 74, 64), min(64 * (e + 1) // 74, 64))):
                relayout_piece(c + 1, tn, (q % 2) * 32 + q // 2, _gate(y[16 * i:16 * i + 8], zero))
            if packwo:
                gate = _gate(y[SB - 8:SB], zero)
                for v in range(min(1024 * e // (NEV - 2), 1024), min(1024 * (e + 1) // (NEV - 2), 1024)):
                    sl, r = v // 64, (v % 64) * 8
                    o = (sl % 4) * 1024 + 2 * r
                    wos[(c - 9) * 16 + sl, r:r + 8, :] = _tie(
                        pltpu.bitcast(wpark[(c - 9) * 4 + sl // 4, o:o + 16, :], U32), gate)
        strassen_chunk(c, zero, extra, range(1, 5))
        if not packwo:
            for t in range(3):
                @pl.when(jnp.logical_and(tn == t, gn < 3))
                def _():
                    w_copy(t, gn + 1, t).start()

            @pl.when(c < NC)
            def _():
                wo_copy(c).start()

        return jnp.where(tn == 2, 0, tn + 1), jnp.where(tn == 2, gn + 1, gn)

    carry = jax.lax.fori_loop(1, 9, functools.partial(pre_chunk, packwo=False), (2, 0))
    for cp in late_copies:
        cp.start()
    for c in range(NC):
        wo_copy(c).wait()
    count = jax.lax.fori_loop(9, 11, functools.partial(pre_chunk, packwo=True), carry)[1]

    for cp in small_copies:
        cp.wait()
    for cp in late_copies:
        cp.wait()
    for cp in conv_copies(1):
        cp.start()
    small[0:NC, :] = dskip_ref[...].astype(F32)
    gate_w = gate_ref[...].astype(F32)
    for c in range(NC):
        small[NC + 8 * c:NC + 8 * (c + 1), :] = jnp.broadcast_to(gate_w[c:c + 1, :], (8, 128))
    mem[...] = mem0_ref[...].astype(F32)

    def mix_gate(r0, gate):
        z = None
        for c in range(NC):
            gw = small[NC + 8 * c:NC + 8 * (c + 1), :]
            t = xs[c, r0:r0 + 16, :].astype(F32) * jnp.concatenate([gw, gw], axis=0)
            z = _tie(t, jnp.concatenate([gate, gate], axis=0)) if z is None else z + t
        z = jnp.sum(z, axis=1, keepdims=True)
        gbuf[r0 // SEG, r0 % SEG:r0 % SEG + 16, :] = jnp.broadcast_to(0.5 * jnp.tanh(0.5 * z) + 0.5, (16, 128))

    def accumulate(slab, segs, rows, val):
        old = outb[slab, segs, rows, :].astype(F32)
        outb[slab, segs, rows, :] = (old + val.astype(BF16).astype(F32).reshape(old.shape)).astype(BF16)

    def conv_prep(t, j):
        tr = t if isinstance(t, int) else jnp.minimum(t, NC - 1)
        r0 = _mo(j * 2 * CB, 2 * CB)
        shift = shift_ref[tr].astype(F32)
        gate = yield
        tail = None
        for o in range(0, 2 * CB + KPAD, 16):
            kk = ks[tr, pl.ds(r0 + o, 16), :].astype(F32)
            win = [tail, _tie(kk[0:8], gate), _tie(kk[8:16], gate)]
            tail = win[2]
            if o == 0:
                continue
            win = jnp.concatenate(win, axis=0)
            acc = win[8:24] * shift[0:1, :]
            for l in range(1, KS):
                acc = acc + win[8 - l:24 - l] * shift[l:l + 1, :]
            rows = pl.ds(r0 + (o - KPAD), 16)
            vs[t + 1, rows, :] = (acc * vs[tr + 1, rows, :].astype(F32)).astype(BF16)
            gate = yield

    def conv_fwd(t, j):
        tr = t if isinstance(t, int) else jnp.minimum(t, NC - 1)
        slot = t & 1
        fwd = pltpu.bitcast(fwd_ref[...], BF16)
        for i in range(2):
            rows = pl.ds(_mo((2 * j + i) * CB, CB), CB)
            sr = _mo((2 * j + i) * 32, 32)
            for off, res in ((0, _dot(fwd, vs[t + 1, rows, :])), (512, _dot_nt(fwd, ssm[tr, :, rows]))):
                for ri in range(2):
                    for fj in range(8):
                        spec[slot * 8 + fj, pl.ds(sr + (off + ri * 16), 16), :] = (
                            res[ri * CB + fj * 16:ri * CB + (fj + 1) * 16])

    def conv_mac(t, j, zero):
        slot = t & 1
        sign = jnp.where(j < 4, 1.0, -1.0).astype(F32)
        zbase = pl.multiple_of(slot * (NB * CB) + j * 8, 8)
        prev = None
        gate = yield
        for i in range(NB):
            base = slot * 8 + j + zero * (i + 1)
            ys = []
            for hv in range(2):
                yr = yi = None
                for jj in range(i + 1):
                    uo = jj * 32 + hv * 8
                    ko = 512 + (i - jj) * 32 + hv * 8
                    ur = spec[base, uo:uo + 8, :]
                    ui = spec[base, uo + 16:uo + 24, :]
                    kr = spec[base, ko:ko + 8, :]
                    ki = spec[base, ko + 16:ko + 24, :]
                    tr, ti = _tie(ur * kr - ui * ki, gate), _tie(ur * ki + ui * kr, gate)
                    yr, yi = (tr, ti) if yr is None else (yr + tr, yi + ti)
                    if jj < i or hv == 0:
                        gate = yield
                ys.append((yr, yi))
            yr = jnp.concatenate([ys[0][0], ys[1][0]], axis=0)
            yi = jnp.concatenate([ys[0][1], ys[1][1]], axis=0)
            zr, zi = (yr, yi) if prev is None else (yr - sign * prev[1], yi + sign * prev[0])
            prev = (yr, yi)
            zspec[pl.ds(zbase + i * CB, 8), :] = pltpu.bitcast(zr.astype(BF16), U32)
            zspec[pl.ds(zbase + (i * CB + CB // 2), 8), :] = pltpu.bitcast(zi.astype(BF16), U32)
            gate = yield

    def conv_inv(t, j):
        tr = t if isinstance(t, int) else jnp.maximum(t, 0)
        slot = t & 1
        dsk = small[pl.ds(tr, 1), :]
        inv = pltpu.bitcast(jnp.concatenate([inv_ref[0], inv_ref[1]], axis=1), BF16)
        for i in range(2):
            rows = pl.ds(_mo((2 * j + i) * CB, CB), CB)
            z = zspec[pl.ds(_mo((slot * NB + 2 * j + i) * CB, CB), CB), :]
            y = _dot(inv, pltpu.bitcast(z, BF16))
            y = y + vs[t + 1, rows, :].astype(F32) * dsk
            segs = pl.ds((2 * j + i) * (CB // SEG), CB // SEG)
            accumulate(t + 1, segs, slice(None), gbuf[segs].reshape(CB, 128) * (xs[tr, rows, :].astype(F32) * y))

    state = {}

    def last_extra(e, y):
        for i, q in enumerate(range(128 * e // 84, 128 * (e + 1) // 84)):
            if q % 16 == 0:
                state["prep"] = conv_prep(0, q // 16)
                next(state["prep"])
            if q % 16 == 5 and q >= 16:
                conv_fwd(0, q // 16 - 1)
            gate = _gate(y[16 * i:16 * i + 8], _zero_of(count))
            state["prep"].send(gate)
            mix_gate(q * 16, gate)
    strassen_chunk(11, _zero_of(count), last_extra, range(1, 4), last=True)
    conv_fwd(0, NB // 2 - 1)

    ri = jax.lax.broadcasted_iota(I32, (NR, NR), 0)
    ci = jax.lax.broadcasted_iota(I32, (NR, NR), 1)
    LD = MEM + XR

    def head_pos(i):
        tail = i >= 2 * LD
        return (jnp.where(tail, (i - 2 * LD) // TL, i // LD),
                jnp.where(tail, LD + (i - 2 * LD) % TL, i % LD))
    (rh, rp), (ch, cp_) = head_pos(ri), head_pos(ci)
    same = rh == ch
    keep = same & ((rp < MEM) | (rp >= cp_))
    fbuf[0, 0:NR, 0:NR] = jnp.where(keep, 0.0, jnp.where(same, -1000000000.0, -jnp.inf)).astype(F32)
    scale = float(DH) ** -0.5

    def step(it, u, zero):
        s = it * 2 + u
        ct = jax.lax.shift_right_logical(s, 3)
        cj = jnp.bitwise_and(s, 7)
        xr0 = pl.multiple_of(it * (2 * SEG), 2 * SEG) + u * SEG
        h_lhs = jnp.concatenate(
            [jnp.concatenate([mem[:, c * 128:(c + 1) * 128], xs[c, pl.ds(xr0, XR), :].astype(F32)],
                             axis=0).astype(BF16) for c in range(NC)], axis=1)

        macs = conv_mac(ct, cj, zero)
        next(macs)
        preps = conv_prep(ct + 1, cj)
        next(preps)
        n_mac = NB * (NB + 1)

        def wo_sums():
            npair, kq = s >> 4, (s >> 3) & 1
            gate = yield
            for i in range(8):
                rows = pl.ds(pl.multiple_of((s & 7) * 64, 64) + 8 * i, 8)
                sl = npair * 8 + kq
                sums = rhs_sums(wos[sl, rows, :], wos[sl + 4, rows, :], wos[sl + 2, rows, :], wos[sl + 6, rows, :], gate)
                for k, val in enumerate(sums):
                    wosum[npair * 10 + kq + 2 * k, rows, :] = val
                gate = yield

        def tail_sums():
            rows = pl.ds(pl.multiple_of(it * TL, TL), TL)
            gate = yield
            for hh in range(H // 2):
                a11, a22 = _tie(otail[hh], gate), _tie(otail[H + H // 2 + hh], gate)
                a12, a21 = otail[H // 2 + hh], otail[H + hh]
                for k, val in enumerate((a11 + a12, a21 + a22, a11, a22, a11 + a22, a12 - a22, a21 - a11)):
                    obuf[k * (H // 2) + hh, rows, :] = val.astype(BF16)
                gate = yield

        wsums = wo_sums()
        next(wsums)
        queue = ([(preps, 1)] * 16 + [(macs, min(MAC_G, n_mac - n)) for n in range(0, n_mac, MAC_G)]
                 + [(wsums, 1)] * 8)

        def side_work(token):
            if queue:
                gen, cnt = queue.pop(0)
                if gen is None:
                    return
                gen.send(_gate(token, zero))
                for _ in range(cnt - 1):
                    gen.send(None)

        def proj(p):
            for t in range(3):
                for i, hh in enumerate((2 * p, 2 * p + 1)):
                    y = _dot(h_lhs, pltpu.bitcast(wts[(hh // 8) * 24 + t * 8 + hh % 8], BF16))
                    side_work(y[0:MEM])
                    ybufs[p // 4][t * 4 + p % 4 + zero, i * 16:(i + 1) * 16, :] = pltpu.bitcast(y.astype(BF16), U32)

        def rows_of(t, p):
            o = ((p // 4) * 12 + t * 4 + p % 4) * 8
            return pltpu.bitcast(jnp.concatenate([ybufs[p // 4][t * 4 + p % 4], prebuf[s, o:o + 8, :]], axis=0), BF16)

        def scores(p):
            sc = _dot_nt(rows_of(0, p), rows_of(1, p)) * scale
            fill = fbuf[zero * (p + 1), 0:NR, 0:NR]
            sc = jnp.where(fill == 0.0, sc, fill)
            e = jnp.exp(sc - jnp.max(sc, axis=1, keepdims=True))
            l = jnp.sum(e, axis=1, keepdims=True)
            r = pl.reciprocal(l, approx=True)
            ebuf[p + zero, 0:NR // 2, :] = pltpu.bitcast(e.astype(BF16), U32)
            return r * (2.0 - l * r)

        def values(p, r):
            o = _dot(pltpu.bitcast(ebuf[p, 0:NR // 2, :], BF16), rows_of(2, p)) * r
            for i, hh in enumerate((2 * p, 2 * p + 1)):
                olhs[hh] = pltpu.bitcast(o[i * LD:(i + 1) * LD].astype(BF16), U32)
                otail[u * H + hh + zero] = o[2 * LD + i * TL:2 * LD + (i + 1) * TL].astype(BF16).astype(F32)

        def oproj(g):
            lhs = pltpu.bitcast(jnp.concatenate([olhs[hh] for hh in range(4 * g, 4 * g + 4)], axis=1), BF16)
            for n in range(NC):
                w = wos[4 * n + g // 2, (g % 2) * 256:(g % 2 + 1) * 256, :]
                y = _dot(lhs, pltpu.bitcast(w, BF16))
                side_work(y[0:MEM])
                if g > 0:
                    y = y + oacc[n + zero]
                if g < H // 4 - 1:
                    oacc[n] = y
                else:
                    mem[:, n * 128:(n + 1) * 128] = y[0:MEM].astype(BF16).astype(F32)
                    accumulate(n + 1, s, slice(0, XR),
                               (1.0 - gbuf[s, 0:XR, :]) * y[MEM:].astype(BF16).astype(F32))

        recip = [None] * (H // 2)
        for op, arg in PROGRAM:
            if op == "P":
                proj(arg)
            elif op == "S":
                recip[arg] = scores(arg)
            elif op == "V":
                values(arg, recip[arg])
                if u == 1 and arg == H // 2 - 1:
                    assert not queue
                    tsums = tail_sums()
                    next(tsums)
                    queue.extend([(None, 0)] * 4 + [(tsums, 1)] * (H // 2))
            elif op == "O":
                oproj(arg)
            elif op == "I":
                conv_inv(ct - 1, cj)
            else:
                assert not queue
                conv_fwd(ct + 1, cj)

    def two_steps(it, carry):
        for u in range(2):
            step(it, u, _zero_of(carry))

        @pl.when(it == 3)
        def _():
            for c in range(2, NC):
                for cp in conv_copies(c):
                    cp.wait()
        return carry + 1
    for cp in conv_copies(1):
        cp.wait()
    for c in range(2, NC):
        for cp in conv_copies(c):
            cp.start()
    jax.lax.fori_loop(0, NSEG // 2, two_steps, count)

    def out_copy(c, s0, n, r0, nr):
        return pltpu.make_async_copy(outb.at[c + 1, pl.ds(s0, n), pl.ds(r0, nr), :],
                                     out_hbm.at[pl.ds(s0, n), pl.ds(r0, nr), pl.ds(c * 128, 128)], sems.at[4])

    def head_copies():
        return [out_copy(c, 0, NSEG, 0, XR) for c in range(NC - 1)]

    def tail_copies(i):
        return [out_copy(c, i * 16, 16, XR, TL) for c in range(NC - 1)] + [out_copy(NC - 1, i * 16, 16, 0, SEG)]

    for cp in head_copies():
        cp.start()

    def post_chunk(i, carry):
        rows = pl.ds(pl.multiple_of(i * 64, 64), 64)

        def finish(n, par, y):
            for j in range(8):
                sg = i * 16 + (2 * j + par)
                accumulate(n + 1, sg, slice(XR, SEG),
                           (1.0 - gbuf[sg, XR:SEG, :]) * y[8 * j:8 * j + 8].astype(BF16).astype(F32))

        copies = tail_copies(i)
        for npair in (0, 3, 1, 2):
            if npair == 3:
                conv_inv(NC - 1, 2 * i)
                conv_inv(NC - 1, 2 * i + 1)
            ms = []
            for k in range(7):
                a = jnp.concatenate([obuf[k * (H // 2) + hh, rows, :] for hh in range(H // 2)], axis=1)
                if k == 0:
                    b = [wos[npair * 8 + 6], wos[npair * 8 + 7]]
                elif k == 1:
                    b = [wos[npair * 8], wos[npair * 8 + 1]]
                else:
                    b = [wosum[npair * 10 + 2 * (k - 2)], wosum[npair * 10 + 2 * (k - 2) + 1]]
                ms.append(_dot(a, pltpu.bitcast(jnp.concatenate(b, axis=0), BF16)))
                if k == 2:
                    finish(2 * npair + 1, 0, ms[0] + ms[2])
                if k == 3:
                    finish(2 * npair, 1, ms[1] + ms[3])
                if k == 5:
                    finish(2 * npair, 0, ((ms[3] - ms[0]) + ms[4]) + ms[5])
                if k == 6:
                    finish(2 * npair + 1, 1, ((ms[2] - ms[1]) + ms[4]) + ms[6])
            copies[2 * npair].start()
            copies[2 * npair + 1].start()
        return carry
    jax.lax.fori_loop(0, PRE // MB, post_chunk, 0)
    for cp in head_copies():
        cp.wait()
    for i in range(PRE // MB):
        for cp in tail_copies(i):
            cp.wait()


@functools.partial(jax.jit, static_argnames=("B_seg_len",))
def pallas_gated_mix__ssm_conv_h3__memory_aug_recurrent_mem_tr__prompt_kernel(
    A_q, A_k, A_v, A_shift_k, A_ssm_k, A_ssm_D, B_x, B_mem0, B_Wq, B_Wk, B_Wv, B_Wo,
    B_seg_len, gate_w,
):
    del B_x
    assert B_seg_len == SEG and A_q.shape == (1, S, D) and B_Wq.shape == (D, H, DH)
    assert A_shift_k.shape == (D, KS) and B_mem0.shape == (1, MEM, D)
    fwd, inv = _dft_tables()
    hbm = pl.BlockSpec(memory_space=pl.ANY)
    out = pl.pallas_call(
        _kernel,
        out_shape=jax.ShapeDtypeStruct((NSEG, SEG, D), BF16),
        in_specs=[hbm] * 15,
        out_specs=hbm,
        scratch_shapes=[
            pltpu.VMEM((NC, S, 128), BF16),
            pltpu.VMEM((NC, NSEG, TL, 128), BF16),
            pltpu.VMEM((28, PRE // 4, 128), U32),
            pltpu.VMEM((10, D // 4, 128), U32),
            pltpu.VMEM((NC, 64 + S, 128), BF16),
            pltpu.VMEM((NC + 2, S, 128), BF16),
            pltpu.VMEM((NC, 128, S), BF16),
            pltpu.VMEM((3, D, 8, 128), BF16),
            pltpu.VMEM((3 * H, D // 2, 128), U32),
            pltpu.VMEM((4 * NC, D // 2, 128), U32),
            pltpu.VMEM((5 * NC, D // 2, 128), U32),
            pltpu.VMEM((2 * H, TL, 128), F32),
            pltpu.VMEM((NC, H * DH, 128), BF16),
            pltpu.VMEM((NSEG, 3 * H // 2 * 8, 128), U32),
            pltpu.VMEM((12, 32, 128), U32),
            pltpu.VMEM((12, 32, 128), U32),
            pltpu.VMEM((12, 32, 128), U32),
            pltpu.VMEM((12, 32, 128), U32),
            pltpu.VMEM((7 * H // 2, PRE // 2, 128), BF16),
            pltpu.VMEM((NC + 1, NSEG, SEG, 128), BF16),
            pltpu.VMEM((H, 16, 128), U32),
            pltpu.VMEM((NC, MEM + XR, 128), F32),
            pltpu.VMEM((MEM, D), F32),
            pltpu.VMEM((96, 128), F32),
            pltpu.VMEM((2, 96, 128), U32),
            pltpu.VMEM((1, 96, 128), F32),
            pltpu.VMEM((H // 2, 64, NR), U32),
            pltpu.VMEM((16, 1024, 128), F32),
            pltpu.VMEM((2 * NB * CB, 128), U32),
            pltpu.VMEM((NSEG, SEG, 128), F32),
            pltpu.VMEM((CB, CB), U32),
            pltpu.VMEM((2, CB // 2, CB), U32),
            pltpu.VMEM((MEM, D), BF16),
            pltpu.VMEM((NC, KS, 128), BF16),
            pltpu.VMEM((NC, 128), BF16),
            pltpu.VMEM((NC, 128), BF16),
            pltpu.SemaphoreType.DMA((11,)),
            pltpu.SemaphoreType.DMA((3,)),
        ],
        compiler_params=pltpu.CompilerParams(vmem_limit_bytes=120 * 1024 * 1024, disable_bounds_checks=True, disable_semaphore_checks=True),
    )(
        A_q.reshape(S, D), A_q.reshape(NSEG, SEG, D), A_k.reshape(S, D), A_v.reshape(S, D), A_ssm_k,
        B_Wq, B_Wk, B_Wv, B_Wo.reshape(H * DH, D),
        A_shift_k.T.reshape(KS, NC, 128).transpose(1, 0, 2),
        A_ssm_D.reshape(NC, 128), gate_w.reshape(NC, 128),
        B_mem0.reshape(MEM, D),
        jnp.asarray(fwd), jnp.asarray(inv),
    )
    return out.reshape(1, S, D)
```

```python
import functools

import jax
import jax.numpy as jnp
import numpy as np
import jax.experimental.pallas as pl
import jax.experimental.pallas.tpu as pltpu

F32 = jnp.float32
BF16 = jnp.bfloat16
U32 = jnp.uint32
I32 = jnp.int32

S = 2048
D = 1024
NC = D // 128
H = 32
DH = 128
MEM = 8
SEG = 32
NSEG = S // SEG
XR = 24
PRE = S - NSEG * XR
TL = SEG - XR
NR = 2 * (SEG + MEM)
CB = 128
NB = S // CB
KS = 4
KPAD = 16
MB = 128
SST = 9
SB = 64
NEV = 28 * 256 // SB
MAC_G = 3


def _expand(text):
    out = []
    for item in text.split():
        if "-" in item:
            a, b = item[1:].split("-")
            out += [(item[0], i) for i in range(int(a), int(b) + 1)]
        else:
            out.append((item[0], int(item[1:] or 0)))
    return out


PROGRAM = _expand("P0-4 S0-3 P5-8 V0-3 S4-7 P9-10 O0 P11-12 V4-7 S8-11 P13 O1 P14-15 "
                  "O2 V8-11 S12-15 O3 O4 V12-15 O5 O6 O7 I F")


def _dft_tables():
    fe = np.arange(0, CB, 2).reshape(-1, 8)
    f = np.concatenate([fe, CB - 1 - fe], axis=1).reshape(-1)
    ang = (2.0 * np.pi * (f + 0.5) / (2 * CB))[:, None] * np.arange(CB)[None, :]
    fwd = np.concatenate([np.cos(ang), -np.sin(ang)], axis=0)
    ang = np.arange(CB)[:, None, None] * (2.0 * np.pi * (fe + 0.5) / (2 * CB))[None]
    inv = np.concatenate([np.cos(ang), -np.sin(ang)], axis=2).reshape(CB, CB) / CB

    def words(m):
        u = np.asarray(m, dtype=BF16).view(np.uint16).astype(np.uint32)
        return u[0::2] | (u[1::2] << 16)
    return words(fwd), np.stack([words(inv[0::2]), words(inv[1::2])])


def _dot(a, b):
    return jnp.dot(a, b, preferred_element_type=F32)


def _dot_nt(a, b):
    return jax.lax.dot_general(a, b, (((1,), (1,)), ((), ())), preferred_element_type=F32)


def _mo(x, m):
    return x if isinstance(x, int) else pl.multiple_of(x, m)


def _tie(x, gate):
    return x if gate is None else pltpu.bitcast(pltpu.bitcast(x, I32) | gate, x.dtype)


def _gate(token, zero):
    return pltpu.bitcast(token, I32) & jnp.full((8, 128), zero, I32)


def _unpack(words):
    return pltpu.bitcast(words, BF16).astype(F32)


def _pack(val):
    return pltpu.bitcast(val.astype(BF16), U32)


def _even_odd(x):
    w = pltpu.bitcast(x, U32)
    return pltpu.bitcast(w << 16, F32), pltpu.bitcast(w & jnp.uint32(0xFFFF0000), F32)


def _zero_of(counter):
    return jax.lax.shift_right_logical(counter, 16)


def _kernel(x_hbm, x3_hbm, k_hbm, v_hbm, ssm_hbm, wq_hbm, wk_hbm, wv_hbm, wo_hbm,
            shift_hbm, dskip_hbm, gate_hbm, mem0_hbm, fwd_hbm, inv_hbm,
            out_hbm,
            xs, xpre, xpk, wsum, ks, vs, ssm, wraw, wts, wos, wosum, otail, wpark, prebuf,
            yb0, yb1, yb2, yb3, obuf, outb, olhs, oacc,
            mem, small, stage, fbuf, ebuf, spec, zspec, gbuf,
            fwd_ref, inv_ref, mem0_ref, shift_ref, dskip_ref, gate_ref,
            sems, sem_w):
    w_hbm = (wq_hbm, wk_hbm, wv_hbm)
    ybufs = (yb0, yb1, yb2, yb3)

    def x_copy(c):
        return pltpu.make_async_copy(x_hbm.at[:, pl.ds(c * 128, 128)], xs.at[c], sems.at[2])

    def xt_copy(c, part):
        s0, n, si = ((0, 16, 0), (16, NSEG - 16, 10))[part]
        return pltpu.make_async_copy(x3_hbm.at[pl.ds(s0, n), pl.ds(XR, TL), pl.ds(c * 128, 128)],
                                     xpre.at[c, pl.ds(s0, n)], sems.at[si])

    def conv_copies(c):
        col = pl.ds(c * 128, 128)
        sem = sems.at[(2, 0, 3)[min(c, 2)]]
        return [pltpu.make_async_copy(k_hbm.at[:, col], ks.at[c, pl.ds(KPAD, S), :], sem),
                pltpu.make_async_copy(v_hbm.at[:, col], vs.at[c + 1], sem),
                pltpu.make_async_copy(ssm_hbm.at[col, :], ssm.at[c], sem)]

    def wo_copy(c):
        return pltpu.make_async_copy(wo_hbm.at[:, pl.ds(_mo(c * 128, 128), 128)], wpark.at[c], sems.at[1])

    def w_copy(t, g, slot):
        return pltpu.make_async_copy(w_hbm[t].at[:, pl.ds(_mo(g * 8, 8), 8), :], wraw.at[slot], sem_w.at[slot])

    def w0_copy(i):
        return pltpu.make_async_copy(wq_hbm.at[pl.ds(i * 256, 256), pl.ds(0, 8), :],
                                     wraw.at[0, pl.ds(i * 256, 256)], sems.at[5 + i])

    small_copies = [pltpu.make_async_copy(a, b, sems.at[9]) for a, b in (
        (shift_hbm, shift_ref), (dskip_hbm, dskip_ref), (gate_hbm, gate_ref),
        (mem0_hbm, mem0_ref), (fwd_hbm, fwd_ref), (inv_hbm, inv_ref))]

    late_copies = conv_copies(0) + [x_copy(c) for c in range(NC)]

    for i in range(4):
        w0_copy(i).start()
    for c in range(NC):
        xt_copy(c, 0).start()

    vs[0] = jnp.zeros((S, 128), BF16)
    outb[0] = jnp.zeros((NSEG, SEG, 128), BF16)
    zspec[NB * CB:2 * NB * CB, :] = jnp.zeros((NB * CB, 128), U32)

    def clear(c, count):
        ks[c, 0:KPAD, :] = jnp.zeros((KPAD, 128), BF16)
        outb[c + 1] = jnp.zeros((NSEG, SEG, 128), BF16)
        return count + 1

    def relayout_piece(c, slot, q, gate=None):
        ws = [pltpu.bitcast(wraw[slot, q * 16 + 2 * i:q * 16 + 2 * i + 2].reshape(16, 128), U32)
              for i in range(8)]
        if isinstance(c, int):
            st = stage.at[q % 2]
            for i in range(8):
                st[i * SST:i * SST + 8, :] = _tie(ws[i], gate if i == 0 else None)
            tr = [st[pl.ds(j, 8, stride=SST), :] for j in range(8)]
        else:
            ws = [_tie(w, gate if i % 2 == 0 else None) for i, w in enumerate(ws)]
            tr = jnp.transpose(jnp.stack(ws, axis=0), (1, 0, 2))
        for j in range(4):
            ev, od = tr[j], tr[4 + j]
            wts[c * 8 + 2 * j, q * 8:(q + 1) * 8, :] = (ev & jnp.uint32(0xFFFF)) | (od << 16)
            wts[c * 8 + (2 * j + 1), q * 8:(q + 1) * 8, :] = (ev >> 16) | (od & jnp.uint32(0xFFFF0000))

    def relayout_with(y, zero, c, slot, d, span):
        qs = range(min(64 * d // span, 64), min(64 * (d + 1) // span, 64))
        for i, q in enumerate(qs):
            o = (i * MB // len(qs)) // 8 * 8
            relayout_piece(c, slot, q, _gate(y[o:o + 8], zero))

    pend = [None]

    def store_pair(c, pp, seg0, ya, yb):
        for i in range(ya.shape[0] // 8):
            pair = jnp.concatenate([ya[8 * i:8 * i + 8], yb[8 * i:8 * i + 8]], axis=0)
            prebuf[seg0 + i, pl.ds(_mo(c * 32, 32) + pp * 8, 8), :] = pltpu.bitcast(pair.astype(BF16), U32)

    def first_mm(d):
        pp, rb, hb = d // 8, (d // 2) % 4, d % 2
        w = pltpu.bitcast(wts[2 * pp + hb], BF16)
        xp = jnp.concatenate([xpre[cc, rb * 16:(rb + 1) * 16].reshape(MB, 128) for cc in range(NC)], axis=1)
        y = _dot(xp, w)
        if hb == 0:
            pend[0] = y
        else:
            store_pair(0, pp, rb * 16, pend[0], y)
        return y

    def lhs_piece(cc, sg, gate):
        def ld(c2, s2):
            return pltpu.bitcast(xpre[c2, s2:s2 + 2].reshape(16, 128), U32)
        w11, w12, w21, w22 = ld(cc, sg), ld(cc + 4, sg), ld(cc, sg + 32), ld(cc + 4, sg + 32)
        w11, w22 = _tie(w11, gate), _tie(w22, gate)
        a11, a12, a21, a22 = _unpack(w11), _unpack(w12), _unpack(w21), _unpack(w22)
        vals = (_pack(a11 + a12), _pack(a21 + a22), w11, w22, _pack(a11 + a22), _pack(a12 - a22), _pack(a21 - a11))
        for k, val in enumerate(vals):
            xpk[k * 4 + cc, sg * 4:sg * 4 + 8, :] = val

    def rhs_sums(w11, w12, w21, w22, gate):
        b11, b12, b21, b22 = _unpack(_tie(w11, gate)), _unpack(w12), _unpack(w21), _unpack(_tie(w22, gate))
        return [_pack(v) for v in (b12 - b22, b21 - b11, b11 + b22, b21 + b22, b11 + b12)]

    def rhs_piece(hd, par, r, gate):
        sums = rhs_sums(wts[hd, r:r + 8, :], wts[hd + 1, r:r + 8, :],
                        wts[hd, 256 + r:264 + r, :], wts[hd + 1, 256 + r:264 + r, :], gate)
        for k, val in enumerate(sums):
            wsum[par * 5 + k, r:r + 8, :] = val

    def strassen_chunk(c, zero, extra, pairs, last=False):
        nrb = 256 // SB
        e = 0
        for pp in pairs:
            for rb in range(nrb):
                ms = []
                for k in range(7):
                    a = jnp.concatenate([xpk[k * 4 + cc, rb * (SB // 2):(rb + 1) * (SB // 2), :] for cc in range(4)], axis=1)
                    if k == 0:
                        b = wts[c * 8 + (2 * pp + 1), 256:512, :]
                    elif k == 1:
                        b = wts[c * 8 + 2 * pp, 0:256, :]
                    else:
                        b = wsum[(pp % 2) * 5 + k - 2]
                    y = _dot(pltpu.bitcast(a, BF16), pltpu.bitcast(b, BF16))
                    ms.append(y)
                    if k == 5:
                        m5, m2, m3, m4, m1, m7 = ms
                        store_pair(c, pp, rb * (SB // 8), ((m4 - m5) + m1) + m7, m5 + m3)
                    if k == 6:
                        store_pair(c, pp, 32 + rb * (SB // 8), m2 + m4, ((m3 - m2) + m1) + y)
                    extra(e, y)
                    le = e % (7 * nrb)
                    cbe = 6 * nrb
                    if not (last and pp == 3):
                        for i, r in enumerate(range(min(32 * le // cbe, 32), min(32 * (le + 1) // cbe, 32))):
                            o = (8 * (2 * i + 1)) % SB
                            rhs_piece(c * 8 + (2 * pp + 2), (pp + 1) % 2, r * 8, _gate(y[o:o + 8], zero))
                    e += 1

    count = 0
    for i in range(4):
        count = jax.lax.fori_loop(2 * i, 2 * i + 2, clear, count)
        w0_copy(i).wait()
        if i == 0:
            for c in range(NC):
                xt_copy(c, 1).start()
        if i == 1:
            for t in range(1, 3):
                w_copy(t, 0, t).start()
        for q in range(16 * i, 16 * i + 16):
            relayout_piece(0, 0, q)
    w_copy(0, 1, 0).start()
    for cp in small_copies:
        cp.start()
    for c in range(NC):
        xt_copy(c, 0).wait()

    for e in range(32):
        if e == 8:
            for c in range(NC):
                xt_copy(c, 1).wait()
        if e == 20:
            w_copy(1, 0, 1).wait()
        y = first_mm(((e % 8) // 2) * 8 + (e // 8) * 2 + e % 2)
        if 8 <= e < 24:
            for i in range(4):
                lhs_piece((e - 8) // 4, ((e % 4) * 4 + i) * 2, _gate(y[32 * i:32 * i + 8], _zero_of(count)))
        if e >= 20:
            relayout_with(y, _zero_of(count), 1, 1, e - 20, 11)
    for r in range(32):
        rhs_piece(8, 0, r * 8, None)
    w_copy(1, 1, 1).start()
    wo_copy(0).start()
    strassen_chunk(1, _zero_of(count), lambda e, y: None, range(1))

    def pre_chunk(c, carry, packwo):
        tn, gn = carry
        zero = _zero_of(tn)
        w_copy(0, 0, tn).wait()

        def extra(e, y):
            for i, q in enumerate(range(min(64 * e // 74, 64), min(64 * (e + 1) // 74, 64))):
                relayout_piece(c + 1, tn, (q % 2) * 32 + q // 2, _gate(y[16 * i:16 * i + 8], zero))
            if packwo:
                gate = _gate(y[SB - 8:SB], zero)
                for v in range(min(1024 * e // (NEV - 2), 1024), min(1024 * (e + 1) // (NEV - 2), 1024)):
                    sl, r = v // 64, (v % 64) * 8
                    o = (sl % 4) * 1024 + 2 * r
                    wos[(c - 9) * 16 + sl, r:r + 8, :] = _tie(
                        pltpu.bitcast(wpark[(c - 9) * 4 + sl // 4, o:o + 16, :], U32), gate)
        strassen_chunk(c, zero, extra, range(1, 5))
        if not packwo:
            for t in range(3):
                @pl.when(jnp.logical_and(tn == t, gn < 3))
                def _():
                    w_copy(t, gn + 1, t).start()

            @pl.when(c < NC)
            def _():
                wo_copy(c).start()

        return jnp.where(tn == 2, 0, tn + 1), jnp.where(tn == 2, gn + 1, gn)

    carry = jax.lax.fori_loop(1, 9, functools.partial(pre_chunk, packwo=False), (2, 0))
    for cp in late_copies:
        cp.start()
    for c in range(NC):
        wo_copy(c).wait()
    count = jax.lax.fori_loop(9, 11, functools.partial(pre_chunk, packwo=True), carry)[1]

    for cp in small_copies:
        cp.wait()
    for cp in late_copies:
        cp.wait()
    for cp in conv_copies(1):
        cp.start()
    small[0:NC, :] = dskip_ref[...].astype(F32)
    gate_w = gate_ref[...].astype(F32)
    for c in range(NC):
        small[NC + 8 * c:NC + 8 * (c + 1), :] = jnp.broadcast_to(gate_w[c:c + 1, :], (8, 128))
    mem[...] = mem0_ref[...].astype(F32)

    def mix_gate(r0, gate):
        z = None
        for c in range(NC):
            gw = small[NC + 8 * c:NC + 8 * (c + 1), :]
            t = xs[c, r0:r0 + 16, :].astype(F32) * jnp.concatenate([gw, gw], axis=0)
            z = _tie(t, jnp.concatenate([gate, gate], axis=0)) if z is None else z + t
        z = jnp.sum(z, axis=1, keepdims=True)
        gbuf[r0 // SEG, r0 % SEG:r0 % SEG + 16, :] = jnp.broadcast_to(0.5 * jnp.tanh(0.5 * z) + 0.5, (16, 128)).astype(BF16)

    def accumulate(slab, segs, rows, val):
        old = outb[slab, segs, rows, :].astype(F32)
        outb[slab, segs, rows, :] = (old + val.astype(BF16).astype(F32).reshape(old.shape)).astype(BF16)

    def conv_prep(t, j):
        tr = t if isinstance(t, int) else jnp.minimum(t, NC - 1)
        r0 = _mo(j * 2 * CB, 2 * CB)
        shift = shift_ref[tr].astype(F32)
        gate = yield
        tail = None
        for o in range(0, 2 * CB + KPAD, 16):
            kk = ks[tr, pl.ds(r0 + o, 16), :].astype(F32)
            win = [tail, _tie(kk[0:8], gate), _tie(kk[8:16], gate)]
            tail = win[2]
            if o == 0:
                continue
            win = jnp.concatenate(win, axis=0)
            acc = win[8:24] * shift[0:1, :]
            for l in range(1, KS):
                acc = acc + win[8 - l:24 - l] * shift[l:l + 1, :]
            rows = pl.ds(r0 + (o - KPAD), 16)
            vs[t + 1, rows, :] = (acc * vs[tr + 1, rows, :].astype(F32)).astype(BF16)
            gate = yield

    def conv_fwd(t, j):
        tr = t if isinstance(t, int) else jnp.minimum(t, NC - 1)
        slot = t & 1
        fwd = pltpu.bitcast(fwd_ref[...], BF16)
        for i in range(2):
            rows = pl.ds(_mo((2 * j + i) * CB, CB), CB)
            sr = _mo((2 * j + i) * 32, 32)
            for off, res in ((0, _dot(fwd, vs[t + 1, rows, :])), (512, _dot_nt(fwd, ssm[tr, :, rows]))):
                for ri in range(2):
                    for fj in range(8):
                        spec[slot * 8 + fj, pl.ds(sr + (off + ri * 16), 16), :] = (
                            res[ri * CB + fj * 16:ri * CB + (fj + 1) * 16])
        return res

    def conv_mac(t, j, zero):
        slot = t & 1
        zbase = pl.multiple_of(slot * (NB * CB) + j * 8, 8)
        prev = None
        gate = yield
        for i in range(NB):
            base = slot * 8 + j + zero * (i + 1)
            ys = []
            for hv in range(2):
                yr = yi = None
                for jj in range(i + 1):
                    uo = jj * 32 + hv * 8
                    ko = 512 + (i - jj) * 32 + hv * 8
                    ur = spec[base, uo:uo + 8, :]
                    ui = spec[base, uo + 16:uo + 24, :]
                    kr = spec[base, ko:ko + 8, :]
                    ki = spec[base, ko + 16:ko + 24, :]
                    tr, ti = _tie(ur * kr - ui * ki, gate), _tie(ur * ki + ui * kr, gate)
                    yr, yi = (tr, ti) if yr is None else (yr + tr, yi + ti)
                    if jj < i or hv == 0:
                        gate = yield
                ys.append((yr, yi))
            (ar, ai), (br, bi) = ys
            if prev is not None:
                ar, ai, br, bi = ar - prev[0][1], ai + prev[0][0], br + prev[1][1], bi - prev[1][0]
            prev = ys
            zspec[pl.ds(zbase + i * CB, 8), :] = _pack(jnp.concatenate([ar + br, ai - bi], axis=0))
            zspec[pl.ds(zbase + (i * CB + CB // 2), 8), :] = _pack(jnp.concatenate([ar - br, ai + bi], axis=0))
            gate = yield

    def conv_inv(t, j):
        tr = t if isinstance(t, int) else jnp.maximum(t, 0)
        slot = t & 1
        ys = []
        for i in range(2):
            z = zspec[pl.ds(_mo((slot * NB + 2 * j + i) * CB, CB), CB), :]
            ys.append([_dot(pltpu.bitcast(inv_ref[h], BF16),
                            pltpu.bitcast(z[h * (CB // 2):(h + 1) * (CB // 2)], BF16)) for h in range(2)])
        gate = yield
        dsk = small[pl.ds(tr, 1), :]
        r0 = _mo(j * 2 * CB, 2 * CB)
        for m in range(2 * CB // 16):
            i, o = m % 2, (m // 2) * 16
            rows = pl.ds(r0 + (i * CB + o), 16)
            sg, part = j * (2 * CB // SEG) + (i * CB + o) // SEG, slice(o % SEG, o % SEG + 16)
            kv, q, g, old = [_even_odd(v) for v in (vs[t + 1, rows, :], xs[tr, rows, :], gbuf[sg, part, :],
                                                    outb[t + 1, sg, part, :])]
            res = []
            for h in range(2):
                y = _tie(ys[i][h][o // 2:o // 2 + 8], gate)
                y = old[h] + g[h] * (q[h] * (y + kv[h] * dsk))
                res.append(pltpu.bitcast(y.astype(BF16).astype(F32), U32))
            outb[t + 1, sg, part, :] = pltpu.bitcast((res[0] >> 16) | (res[1] & jnp.uint32(0xFFFF0000)), BF16)
            gate = yield

    state = {}

    def last_extra(e, y):
        for i, q in enumerate(range(128 * e // 84, 128 * (e + 1) // 84)):
            if q % 16 == 0:
                state["prep"] = conv_prep(0, q // 16)
                next(state["prep"])
            if q % 16 == 5 and q >= 16:
                conv_fwd(0, q // 16 - 1)
            gate = _gate(y[16 * i:16 * i + 8], _zero_of(count))
            state["prep"].send(gate)
            mix_gate(q * 16, gate)
    strassen_chunk(11, _zero_of(count), last_extra, range(1, 4), last=True)
    conv_fwd(0, NB // 2 - 1)

    ri = jax.lax.broadcasted_iota(I32, (NR, NR), 0)
    ci = jax.lax.broadcasted_iota(I32, (NR, NR), 1)
    LD = MEM + XR

    def head_pos(i):
        tail = i >= 2 * LD
        return (jnp.where(tail, (i - 2 * LD) // TL, i // LD),
                jnp.where(tail, LD + (i - 2 * LD) % TL, i % LD))
    (rh, rp), (ch, cp_) = head_pos(ri), head_pos(ci)
    same = rh == ch
    keep = same & ((rp < MEM) | (rp >= cp_))
    fbuf[0, 0:NR, 0:NR] = jnp.where(keep, 0.0, jnp.where(same, -1000000000.0, -jnp.inf)).astype(F32)
    scale = float(DH) ** -0.5

    def step(it, u, zero):
        s = it * 2 + u
        ct = jax.lax.shift_right_logical(s, 3)
        cj = jnp.bitwise_and(s, 7)
        xr0 = pl.multiple_of(it * (2 * SEG), 2 * SEG) + u * SEG
        h_lhs = jnp.concatenate(
            [jnp.concatenate([mem[:, c * 128:(c + 1) * 128], xs[c, pl.ds(xr0, XR), :].astype(F32)],
                             axis=0).astype(BF16) for c in range(NC)], axis=1)

        macs = conv_mac(ct, cj, zero)
        next(macs)
        preps = conv_prep(ct + 1, cj)
        next(preps)
        n_mac = NB * (NB + 1)

        def wo_sums():
            npair, kq = s >> 4, (s >> 3) & 1
            gate = yield
            for i in range(8):
                rows = pl.ds(pl.multiple_of((s & 7) * 64, 64) + 8 * i, 8)
                sl = npair * 8 + kq
                sums = rhs_sums(wos[sl, rows, :], wos[sl + 4, rows, :], wos[sl + 2, rows, :], wos[sl + 6, rows, :], gate)
                for k, val in enumerate(sums):
                    wosum[npair * 10 + kq + 2 * k, rows, :] = val
                gate = yield

        def tail_sums():
            rows = pl.ds(pl.multiple_of(it * TL, TL), TL)
            gate = yield
            for hh in range(H // 2):
                a11, a22 = _tie(otail[hh], gate), _tie(otail[H + H // 2 + hh], gate)
                a12, a21 = otail[H // 2 + hh], otail[H + hh]
                for k, val in enumerate((a11 + a12, a21 + a22, a11, a22, a11 + a22, a12 - a22, a21 - a11)):
                    obuf[k * (H // 2) + hh, rows, :] = val.astype(BF16)
                gate = yield

        wsums = wo_sums()
        next(wsums)
        queue = ([(preps, 1)] * 16 + [(macs, min(MAC_G, n_mac - n)) for n in range(0, n_mac, MAC_G)]
                 + [(wsums, 1)] * 8)

        def side_work(token):
            if queue:
                gen, cnt = queue.pop(0)
                if gen is None:
                    return
                gen.send(_gate(token, zero))
                for _ in range(cnt - 1):
                    gen.send(None)

        def proj(p):
            for t in range(3):
                for i, hh in enumerate((2 * p, 2 * p + 1)):
                    y = _dot(h_lhs, pltpu.bitcast(wts[(hh // 8) * 24 + t * 8 + hh % 8], BF16))
                    side_work(y[0:MEM])
                    ybufs[p // 4][t * 4 + p % 4 + zero, i * 16:(i + 1) * 16, :] = pltpu.bitcast(y.astype(BF16), U32)

        def rows_of(t, p):
            o = ((p // 4) * 12 + t * 4 + p % 4) * 8
            return pltpu.bitcast(jnp.concatenate([ybufs[p // 4][t * 4 + p % 4], prebuf[s, o:o + 8, :]], axis=0), BF16)

        def scores(p):
            sc = _dot_nt(rows_of(0, p), rows_of(1, p)) * scale
            fill = fbuf[zero * (p + 1), 0:NR, 0:NR]
            sc = jnp.where(fill == 0.0, sc, fill)
            e = jnp.exp(sc - jnp.max(sc, axis=1, keepdims=True))
            l = jnp.sum(e, axis=1, keepdims=True)
            r = pl.reciprocal(l, approx=True)
            ebuf[p + zero, 0:NR // 2, :] = pltpu.bitcast(e.astype(BF16), U32)
            return r * (2.0 - l * r)

        def values(p, r):
            o = _dot(pltpu.bitcast(ebuf[p, 0:NR // 2, :], BF16), rows_of(2, p)) * r
            for i, hh in enumerate((2 * p, 2 * p + 1)):
                olhs[hh] = pltpu.bitcast(o[i * LD:(i + 1) * LD].astype(BF16), U32)
                otail[u * H + hh + zero] = o[2 * LD + i * TL:2 * LD + (i + 1) * TL].astype(BF16).astype(F32)

        def oproj(g):
            lhs = pltpu.bitcast(jnp.concatenate([olhs[hh] for hh in range(4 * g, 4 * g + 4)], axis=1), BF16)
            for n in range(NC):
                w = wos[4 * n + g // 2, (g % 2) * 256:(g % 2 + 1) * 256, :]
                y = _dot(lhs, pltpu.bitcast(w, BF16))
                side_work(y[0:MEM])
                if g > 0:
                    y = y + oacc[n + zero]
                if g < H // 4 - 1:
                    oacc[n] = y
                else:
                    mem[:, n * 128:(n + 1) * 128] = y[0:MEM].astype(BF16).astype(F32)
                    accumulate(n + 1, s, slice(0, XR),
                               (1.0 - gbuf[s, 0:XR, :].astype(F32)) * y[MEM:].astype(BF16).astype(F32))

        recip = [None] * (H // 2)
        for op, arg in PROGRAM:
            if op == "P":
                proj(arg)
            elif op == "S":
                recip[arg] = scores(arg)
            elif op == "V":
                values(arg, recip[arg])
                if u == 1 and arg == H // 2 - 1:
                    assert not queue
                    tsums = tail_sums()
                    next(tsums)
                    queue.extend([(None, 0)] * 4 + [(tsums, 1)] * (H // 2))
            elif op == "O":
                oproj(arg)
            elif op == "I":
                invs = conv_inv(ct - 1, cj)
                next(invs)
            else:
                assert not queue
                res = conv_fwd(ct + 1, cj)
                for m in range(16):
                    o = (4 + m * 26 // 16) * 8
                    invs.send(_gate(res[o:o + 8], zero))

    def two_steps(it, carry):
        for u in range(2):
            step(it, u, _zero_of(carry))

        @pl.when(it == 3)
        def _():
            for c in range(2, NC):
                for cp in conv_copies(c):
                    cp.wait()
        return carry + 1
    for cp in conv_copies(1):
        cp.wait()
    for c in range(2, NC):
        for cp in conv_copies(c):
            cp.start()
    jax.lax.fori_loop(0, NSEG // 2, two_steps, count)

    def out_copy(c, s0, n, r0, nr):
        return pltpu.make_async_copy(outb.at[c + 1, pl.ds(s0, n), pl.ds(r0, nr), :],
                                     out_hbm.at[pl.ds(s0, n), pl.ds(r0, nr), pl.ds(c * 128, 128)], sems.at[4])

    def head_copies():
        return [out_copy(c, 0, NSEG, 0, XR) for c in range(NC - 1)]

    def tail_copies(i):
        return [out_copy(c, i * 16, 16, XR, TL) for c in range(NC - 1)] + [out_copy(NC - 1, i * 16, 16, 0, SEG)]

    for cp in head_copies():
        cp.start()

    def post_chunk(i, carry):
        rows = pl.ds(pl.multiple_of(i * 64, 64), 64)

        def finish(n, par, y):
            for j in range(8):
                sg = i * 16 + (2 * j + par)
                accumulate(n + 1, sg, slice(XR, SEG),
                           (1.0 - gbuf[sg, XR:SEG, :].astype(F32)) * y[8 * j:8 * j + 8].astype(BF16).astype(F32))

        copies = tail_copies(i)
        for npair in (0, 3, 1, 2):
            if npair == 3:
                invs = [conv_inv(NC - 1, 2 * i + jj) for jj in range(2)]
                for gen in invs:
                    next(gen)
            ms = []
            for k in range(7):
                a = jnp.concatenate([obuf[k * (H // 2) + hh, rows, :] for hh in range(H // 2)], axis=1)
                if k == 0:
                    b = [wos[npair * 8 + 6], wos[npair * 8 + 7]]
                elif k == 1:
                    b = [wos[npair * 8], wos[npair * 8 + 1]]
                else:
                    b = [wosum[npair * 10 + 2 * (k - 2)], wosum[npair * 10 + 2 * (k - 2) + 1]]
                ms.append(_dot(a, pltpu.bitcast(jnp.concatenate(b, axis=0), BF16)))
                if npair == 3 and k < 4:
                    for m in range(8):
                        invs[k // 2].send(_gate(ms[k][8 * m:8 * m + 8], _zero_of(carry)))
                if k == 2:
                    finish(2 * npair + 1, 0, ms[0] + ms[2])
                if k == 3:
                    finish(2 * npair, 1, ms[1] + ms[3])
                if k == 5:
                    finish(2 * npair, 0, ((ms[3] - ms[0]) + ms[4]) + ms[5])
                if k == 6:
                    finish(2 * npair + 1, 1, ((ms[2] - ms[1]) + ms[4]) + ms[6])
            copies[2 * npair].start()
            copies[2 * npair + 1].start()
        return carry + 1
    jax.lax.fori_loop(0, PRE // MB, post_chunk, 0)
    for cp in head_copies():
        cp.wait()
    for i in range(PRE // MB):
        for cp in tail_copies(i):
            cp.wait()


@functools.partial(jax.jit, static_argnames=("B_seg_len",))
def pallas_gated_mix__ssm_conv_h3__memory_aug_recurrent_mem_tr__prompt_kernel(
    A_q, A_k, A_v, A_shift_k, A_ssm_k, A_ssm_D, B_x, B_mem0, B_Wq, B_Wk, B_Wv, B_Wo,
    B_seg_len, gate_w,
):
    del B_x
    assert B_seg_len == SEG and A_q.shape == (1, S, D) and B_Wq.shape == (D, H, DH)
    assert A_shift_k.shape == (D, KS) and B_mem0.shape == (1, MEM, D)
    fwd, inv = _dft_tables()
    hbm = pl.BlockSpec(memory_space=pl.ANY)
    out = pl.pallas_call(
        _kernel,
        out_shape=jax.ShapeDtypeStruct((NSEG, SEG, D), BF16),
        in_specs=[hbm] * 15,
        out_specs=hbm,
        scratch_shapes=[
            pltpu.VMEM((NC, S, 128), BF16),
            pltpu.VMEM((NC, NSEG, TL, 128), BF16),
            pltpu.VMEM((28, PRE // 4, 128), U32),
            pltpu.VMEM((10, D // 4, 128), U32),
            pltpu.VMEM((NC, 64 + S, 128), BF16),
            pltpu.VMEM((NC + 2, S, 128), BF16),
            pltpu.VMEM((NC, 128, S), BF16),
            pltpu.VMEM((3, D, 8, 128), BF16),
            pltpu.VMEM((3 * H, D // 2, 128), U32),
            pltpu.VMEM((4 * NC, D // 2, 128), U32),
            pltpu.VMEM((5 * NC, D // 2, 128), U32),
            pltpu.VMEM((2 * H, TL, 128), F32),
            pltpu.VMEM((NC, H * DH, 128), BF16),
            pltpu.VMEM((NSEG, 3 * H // 2 * 8, 128), U32),
            pltpu.VMEM((12, 32, 128), U32),
            pltpu.VMEM((12, 32, 128), U32),
            pltpu.VMEM((12, 32, 128), U32),
            pltpu.VMEM((12, 32, 128), U32),
            pltpu.VMEM((7 * H // 2, PRE // 2, 128), BF16),
            pltpu.VMEM((NC + 1, NSEG, SEG, 128), BF16),
            pltpu.VMEM((H, 16, 128), U32),
            pltpu.VMEM((NC, MEM + XR, 128), F32),
            pltpu.VMEM((MEM, D), F32),
            pltpu.VMEM((96, 128), F32),
            pltpu.VMEM((2, 96, 128), U32),
            pltpu.VMEM((1, 96, 128), F32),
            pltpu.VMEM((H // 2, 64, NR), U32),
            pltpu.VMEM((16, 1024, 128), F32),
            pltpu.VMEM((2 * NB * CB, 128), U32),
            pltpu.VMEM((NSEG, SEG, 128), BF16),
            pltpu.VMEM((CB, CB), U32),
            pltpu.VMEM((2, CB // 4, CB), U32),
            pltpu.VMEM((MEM, D), BF16),
            pltpu.VMEM((NC, KS, 128), BF16),
            pltpu.VMEM((NC, 128), BF16),
            pltpu.VMEM((NC, 128), BF16),
            pltpu.SemaphoreType.DMA((11,)),
            pltpu.SemaphoreType.DMA((3,)),
        ],
        compiler_params=pltpu.CompilerParams(vmem_limit_bytes=120 * 1024 * 1024, disable_bounds_checks=True, disable_semaphore_checks=True),
    )(
        A_q.reshape(S, D), A_q.reshape(NSEG, SEG, D), A_k.reshape(S, D), A_v.reshape(S, D), A_ssm_k,
        B_Wq, B_Wk, B_Wv, B_Wo.reshape(H * DH, D),
        A_shift_k.T.reshape(KS, NC, 128).transpose(1, 0, 2),
        A_ssm_D.reshape(NC, 128), gate_w.reshape(NC, 128),
        B_mem0.reshape(MEM, D),
        jnp.asarray(fwd), jnp.asarray(inv),
    )
    return out.reshape(1, S, D)
```

```python
import functools

import jax
import jax.numpy as jnp
import numpy as np
import jax.experimental.pallas as pl
import jax.experimental.pallas.tpu as pltpu

F32 = jnp.float32
BF16 = jnp.bfloat16
U32 = jnp.uint32
I32 = jnp.int32

S = 2048
D = 1024
NC = D // 128
H = 32
DH = 128
MEM = 8
SEG = 32
NSEG = S // SEG
XR = 24
PRE = S - NSEG * XR
TL = SEG - XR
NR = 2 * (SEG + MEM)
CB = 128
NB = S // CB
KS = 4
KPAD = 16
MB = 128
SST = 9
SB = 64
NEV = 28 * 256 // SB
NEND = 8
MAC_G = 3


def _expand(text):
    out = []
    for item in text.split():
        if "-" in item:
            a, b = item[1:].split("-")
            out += [(item[0], i) for i in range(int(a), int(b) + 1)]
        else:
            out.append((item[0], int(item[1:] or 0)))
    return out


_HEAD = "P0-4 S0-3 P5-8 V0-3 S4-7 P9-10 O0 P11-12 V4-7 S8-11 P13 O1 P14-15 O2 V8-11 S12-15 "
PROGRAM = _expand(_HEAD + "O3 O4 V12-15 O5 O6 O7 I F")
PROGRAM_END = _expand(_HEAD + "I O3 O4 V12-15 O5 O6 O7")


def _dft_tables():
    fe = np.arange(0, CB, 2).reshape(-1, 8)
    f = np.concatenate([fe, CB - 1 - fe], axis=1).reshape(-1)
    ang = (2.0 * np.pi * (f + 0.5) / (2 * CB))[:, None] * np.arange(CB)[None, :]
    fwd = np.concatenate([np.cos(ang), -np.sin(ang)], axis=0)
    ang = np.arange(CB)[:, None, None] * (2.0 * np.pi * (fe + 0.5) / (2 * CB))[None]
    inv = np.concatenate([np.cos(ang), -np.sin(ang)], axis=2).reshape(CB, CB) / CB

    def words(m):
        u = np.asarray(m, dtype=BF16).view(np.uint16).astype(np.uint32)
        return u[0::2] | (u[1::2] << 16)
    return words(fwd), np.stack([words(inv[0::2]), words(inv[1::2])])


def _dot(a, b):
    return jnp.dot(a, b, preferred_element_type=F32)


def _dot_nt(a, b):
    return jax.lax.dot_general(a, b, (((1,), (1,)), ((), ())), preferred_element_type=F32)


def _mo(x, m):
    return x if isinstance(x, int) else pl.multiple_of(x, m)


def _tie(x, gate):
    return x if gate is None else pltpu.bitcast(pltpu.bitcast(x, I32) | gate, x.dtype)


def _gate(token, zero):
    return pltpu.bitcast(token, I32) & jnp.full((8, 128), zero, I32)


def _unpack(words):
    return pltpu.bitcast(words, BF16).astype(F32)


def _pack(val):
    return pltpu.bitcast(val.astype(BF16), U32)


def _even_odd(x):
    w = pltpu.bitcast(x, U32)
    return pltpu.bitcast(w << 16, F32), pltpu.bitcast(w & jnp.uint32(0xFFFF0000), F32)


def _zero_of(counter):
    return jax.lax.shift_right_logical(counter, 16)


def _kernel(x_hbm, x3_hbm, k_hbm, v_hbm, ssm_hbm, wq_hbm, wk_hbm, wv_hbm, wo_hbm,
            shift_hbm, dskip_hbm, gate_hbm, mem0_hbm, fwd_hbm, inv_hbm,
            out_hbm,
            xs, xpre, xpk, wsum, ks, vs, ssm, wraw, wts, wos, wosum, otail, wpark, prebuf,
            yb0, yb1, yb2, yb3, obuf, outb, oacc,
            mem, small, stage, fbuf, ebuf, spec, zspec, gbuf,
            fwd_ref, inv_ref, mem0_ref, shift_ref, dskip_ref, gate_ref,
            sems, sem_w, sem_o):
    w_hbm = (wq_hbm, wk_hbm, wv_hbm)
    ybufs = (yb0, yb1, yb2, yb3)

    def x_copy(c):
        return pltpu.make_async_copy(x_hbm.at[:, pl.ds(c * 128, 128)], xs.at[c], sems.at[2])

    def xt_copy(c, part):
        s0, n, si = ((0, 16, 0), (16, NSEG - 16, 10))[part]
        return pltpu.make_async_copy(x3_hbm.at[pl.ds(s0, n), pl.ds(XR, TL), pl.ds(c * 128, 128)],
                                     xpre.at[c, pl.ds(s0, n)], sems.at[si])

    def conv_copies(c):
        col = pl.ds(c * 128, 128)
        sem = sems.at[(2, 0, 3)[min(c, 2)]]
        return [pltpu.make_async_copy(k_hbm.at[:, col], ks.at[c, pl.ds(KPAD, S), :], sem),
                pltpu.make_async_copy(v_hbm.at[:, col], vs.at[c + 1], sem),
                pltpu.make_async_copy(ssm_hbm.at[col, :], ssm.at[c], sem)]

    def wo_copy(c):
        return pltpu.make_async_copy(wo_hbm.at[:, pl.ds(_mo(c * 128, 128), 128)], wpark.at[c], sem_o.at[c])

    def w_copy(t, g, slot):
        return pltpu.make_async_copy(w_hbm[t].at[:, pl.ds(_mo(g * 8, 8), 8), :], wraw.at[slot], sem_w.at[slot])

    def w0_copy(i):
        return pltpu.make_async_copy(wq_hbm.at[pl.ds(i * 256, 256), pl.ds(0, 8), :],
                                     wraw.at[0, pl.ds(i * 256, 256)], sems.at[5 + i])

    small_copies = [pltpu.make_async_copy(a, b, sems.at[9]) for a, b in (
        (shift_hbm, shift_ref), (dskip_hbm, dskip_ref), (gate_hbm, gate_ref),
        (mem0_hbm, mem0_ref), (fwd_hbm, fwd_ref), (inv_hbm, inv_ref))]

    late_copies = conv_copies(0) + [x_copy(c) for c in range(NC)]

    for i in range(4):
        w0_copy(i).start()
    for c in range(NC):
        xt_copy(c, 0).start()

    def clear_spare(c, count):
        r = pl.multiple_of(c * 256, 256)
        vs[0, pl.ds(r, 256), :] = jnp.zeros((256, 128), BF16)
        outb[0, pl.ds(c * 8, 8)] = jnp.zeros((8, SEG, 128), BF16)
        zspec[pl.ds(NB * CB + r, 256), :] = jnp.zeros((256, 128), U32)
        wpark[NC, pl.ds(2 * r, 512), :] = jnp.zeros((512, 128), BF16)
        return count
    jax.lax.fori_loop(0, 8, clear_spare, 0)

    def clear(c, count):
        ks[c, 0:KPAD, :] = jnp.zeros((KPAD, 128), BF16)
        outb[c + 1] = jnp.zeros((NSEG, SEG, 128), BF16)
        return count + 1

    def relayout_piece(c, slot, q, gate=None):
        ws = [pltpu.bitcast(wraw[slot, q * 16 + 2 * i:q * 16 + 2 * i + 2].reshape(16, 128), U32)
              for i in range(8)]
        if isinstance(c, int):
            st = stage.at[q % 2]
            for i in range(8):
                st[i * SST:i * SST + 8, :] = _tie(ws[i], gate if i == 0 else None)
            tr = [st[pl.ds(j, 8, stride=SST), :] for j in range(8)]
        else:
            ws = [_tie(w, gate if i % 2 == 0 else None) for i, w in enumerate(ws)]
            tr = jnp.transpose(jnp.stack(ws, axis=0), (1, 0, 2))
        for j in range(4):
            ev, od = tr[j], tr[4 + j]
            wts[c * 8 + 2 * j, q * 8:(q + 1) * 8, :] = (ev & jnp.uint32(0xFFFF)) | (od << 16)
            wts[c * 8 + (2 * j + 1), q * 8:(q + 1) * 8, :] = (ev >> 16) | (od & jnp.uint32(0xFFFF0000))

    def relayout_with(y, zero, c, slot, d, span):
        qs = range(min(64 * d // span, 64), min(64 * (d + 1) // span, 64))
        for i, q in enumerate(qs):
            o = (i * MB // len(qs)) // 8 * 8
            relayout_piece(c, slot, q, _gate(y[o:o + 8], zero))

    pend = [None]

    def store_pair(c, pp, seg0, ya, yb):
        for i in range(ya.shape[0] // 8):
            pair = jnp.concatenate([ya[8 * i:8 * i + 8], yb[8 * i:8 * i + 8]], axis=0)
            prebuf[seg0 + i, pl.ds(_mo(c * 32, 32) + pp * 8, 8), :] = pltpu.bitcast(pair.astype(BF16), U32)

    def first_mm(d):
        pp, rb, hb = d // 8, (d // 2) % 4, d % 2
        w = pltpu.bitcast(wts[2 * pp + hb], BF16)
        xp = jnp.concatenate([xpre[cc, rb * 16:(rb + 1) * 16].reshape(MB, 128) for cc in range(NC)], axis=1)
        y = _dot(xp, w)
        if hb == 0:
            pend[0] = y
        else:
            store_pair(0, pp, rb * 16, pend[0], y)
        return y

    def lhs_piece(cc, sg, gate):
        def ld(c2, s2):
            return pltpu.bitcast(xpre[c2, s2:s2 + 2].reshape(16, 128), U32)
        w11, w12, w21, w22 = ld(cc, sg), ld(cc + 4, sg), ld(cc, sg + 32), ld(cc + 4, sg + 32)
        w11, w22 = _tie(w11, gate), _tie(w22, gate)
        a11, a12, a21, a22 = _unpack(w11), _unpack(w12), _unpack(w21), _unpack(w22)
        vals = (_pack(a11 + a12), _pack(a21 + a22), w11, w22, _pack(a11 + a22), _pack(a12 - a22), _pack(a21 - a11))
        for k, val in enumerate(vals):
            xpk[k * 4 + cc, sg * 4:sg * 4 + 8, :] = val

    def rhs_sums(w11, w12, w21, w22, gate):
        b11, b12, b21, b22 = _unpack(_tie(w11, gate)), _unpack(w12), _unpack(w21), _unpack(_tie(w22, gate))
        return [_pack(v) for v in (b12 - b22, b21 - b11, b11 + b22, b21 + b22, b11 + b12)]

    def rhs_piece(hd, par, r, gate):
        sums = rhs_sums(wts[hd, r:r + 8, :], wts[hd + 1, r:r + 8, :],
                        wts[hd, 256 + r:264 + r, :], wts[hd + 1, 256 + r:264 + r, :], gate)
        for k, val in enumerate(sums):
            wsum[par * 5 + k, r:r + 8, :] = val

    def strassen_chunk(c, zero, extra, pairs, last=False):
        nrb = 256 // SB
        e = 0
        for pp in pairs:
            for rb in range(nrb):
                ms = []
                for k in range(7):
                    a = jnp.concatenate([xpk[k * 4 + cc, rb * (SB // 2):(rb + 1) * (SB // 2), :] for cc in range(4)], axis=1)
                    if k == 0:
                        b = wts[c * 8 + (2 * pp + 1), 256:512, :]
                    elif k == 1:
                        b = wts[c * 8 + 2 * pp, 0:256, :]
                    else:
                        b = wsum[(pp % 2) * 5 + k - 2]
                    y = _dot(pltpu.bitcast(a, BF16), pltpu.bitcast(b, BF16))
                    ms.append(y)
                    if k == 5:
                        m5, m2, m3, m4, m1, m7 = ms
                        store_pair(c, pp, rb * (SB // 8), ((m4 - m5) + m1) + m7, m5 + m3)
                    if k == 6:
                        store_pair(c, pp, 32 + rb * (SB // 8), m2 + m4, ((m3 - m2) + m1) + y)
                    extra(e, y)
                    le = e % (7 * nrb)
                    cbe = 6 * nrb
                    if not (last and pp == 3):
                        for i, r in enumerate(range(min(32 * le // cbe, 32), min(32 * (le + 1) // cbe, 32))):
                            o = (8 * (2 * i + 1)) % SB
                            rhs_piece(c * 8 + (2 * pp + 2), (pp + 1) % 2, r * 8, _gate(y[o:o + 8], zero))
                    e += 1

    count = 0
    for i in range(4):
        count = jax.lax.fori_loop(2 * i, 2 * i + 2, clear, count)
        w0_copy(i).wait()
        if i == 0:
            for c in range(NC):
                xt_copy(c, 1).start()
        if i == 1:
            for t in range(1, 3):
                w_copy(t, 0, t).start()
        for q in range(16 * i, 16 * i + 16):
            relayout_piece(0, 0, q)
    w_copy(0, 1, 0).start()
    for cp in small_copies:
        cp.start()
    for c in range(NC):
        xt_copy(c, 0).wait()

    for e in range(32):
        if e == 8:
            for c in range(NC):
                xt_copy(c, 1).wait()
        if e == 20:
            w_copy(1, 0, 1).wait()
        y = first_mm(((e % 8) // 2) * 8 + (e // 8) * 2 + e % 2)
        if 8 <= e < 24:
            for i in range(4):
                lhs_piece((e - 8) // 4, ((e % 4) * 4 + i) * 2, _gate(y[32 * i:32 * i + 8], _zero_of(count)))
        if e >= 20:
            relayout_with(y, _zero_of(count), 1, 1, e - 20, 11)
    for r in range(32):
        rhs_piece(8, 0, r * 8, None)
    w_copy(1, 1, 1).start()
    wo_copy(0).start()
    strassen_chunk(1, _zero_of(count), lambda e, y: None, range(1))

    def pre_chunk(c, carry):
        tn, gn = carry
        zero = _zero_of(tn)
        ws = jnp.where(c < 3, NC, c - 3)
        w_copy(0, 0, tn).wait()

        @pl.when(c >= 3)
        def _():
            wo_copy(ws).wait()

        def extra(e, y):
            for i, q in enumerate(range(min(64 * e // 74, 64), min(64 * (e + 1) // 74, 64))):
                relayout_piece(c + 1, tn, (q % 2) * 32 + q // 2, _gate(y[16 * i:16 * i + 8], zero))
            if e >= 74:
                gate = _gate(y[SB - 8:SB], zero)
                span = NEV - 76
                for v in range(min(256 * (e - 74) // span, 256), min(256 * (e - 73) // span, 256)):
                    wos[ws * 4 + v // 64, (v % 64) * 8:(v % 64) * 8 + 8, :] = _tie(
                        pltpu.bitcast(wpark[ws, v * 16:v * 16 + 16, :], U32), gate)
        strassen_chunk(c, zero, extra, range(1, 5))
        for t in range(3):
            @pl.when(jnp.logical_and(tn == t, gn < 3))
            def _():
                w_copy(t, gn + 1, t).start()

        @pl.when(c < NC)
        def _():
            wo_copy(c).start()

        @pl.when(c == NC)
        def _():
            for cp in late_copies:
                cp.start()
        return jnp.where(tn == 2, 0, tn + 1), jnp.where(tn == 2, gn + 1, gn)

    count = jax.lax.fori_loop(1, 11, pre_chunk, (2, 0))[1]

    for cp in small_copies:
        cp.wait()
    for cp in late_copies:
        cp.wait()
    for cp in conv_copies(1):
        cp.start()
    small[0:NC, :] = dskip_ref[...].astype(F32)
    gate_w = gate_ref[...].astype(F32)
    for c in range(NC):
        small[NC + 8 * c:NC + 8 * (c + 1), :] = jnp.broadcast_to(gate_w[c:c + 1, :], (8, 128))
    mem[...] = mem0_ref[...].astype(F32)

    def mix_gate(r0, gate):
        z = None
        for c in range(NC):
            gw = small[NC + 8 * c:NC + 8 * (c + 1), :]
            t = xs[c, r0:r0 + 16, :].astype(F32) * jnp.concatenate([gw, gw], axis=0)
            z = _tie(t, jnp.concatenate([gate, gate], axis=0)) if z is None else z + t
        z = jnp.sum(z, axis=1, keepdims=True)
        gbuf[r0 // SEG, r0 % SEG:r0 % SEG + 16, :] = jnp.broadcast_to(0.5 * jnp.tanh(0.5 * z) + 0.5, (16, 128)).astype(BF16)

    def accumulate(slab, segs, rows, val):
        old = outb[slab, segs, rows, :].astype(F32)
        outb[slab, segs, rows, :] = (old + val.astype(BF16).astype(F32).reshape(old.shape)).astype(BF16)

    def conv_prep(t, j):
        r0 = _mo(j * 2 * CB, 2 * CB)
        shift = shift_ref[t].astype(F32)
        gate = yield
        tail = None
        for o in range(0, 2 * CB + KPAD, 16):
            kk = ks[t, pl.ds(r0 + o, 16), :].astype(F32)
            win = [tail, _tie(kk[0:8], gate), _tie(kk[8:16], gate)]
            tail = win[2]
            if o == 0:
                continue
            win = jnp.concatenate(win, axis=0)
            acc = win[8:24] * shift[0:1, :]
            for l in range(1, KS):
                acc = acc + win[8 - l:24 - l] * shift[l:l + 1, :]
            rows = pl.ds(r0 + (o - KPAD), 16)
            vs[t + 1, rows, :] = (acc * vs[t + 1, rows, :].astype(F32)).astype(BF16)
            gate = yield

    def conv_fwd(t, j):
        slot = t & 1
        fwd = pltpu.bitcast(fwd_ref[...], BF16)
        for i in range(2):
            rows = pl.ds(_mo((2 * j + i) * CB, CB), CB)
            sr = _mo((2 * j + i) * 32, 32)
            for off, res in ((0, _dot(fwd, vs[t + 1, rows, :])), (512, _dot_nt(fwd, ssm[t, :, rows]))):
                for ri in range(2):
                    for fj in range(8):
                        spec[slot * 8 + fj, pl.ds(sr + (off + ri * 16), 16), :] = (
                            res[ri * CB + fj * 16:ri * CB + (fj + 1) * 16])
        return res

    def conv_mac(t, j, zero):
        slot = t & 1
        zbase = pl.multiple_of(slot * (NB * CB) + j * 8, 8)
        prev = None
        gate = yield
        for i in range(NB):
            base = slot * 8 + j + zero * (i + 1)
            ys = []
            for hv in range(2):
                yr = yi = None
                for jj in range(i + 1):
                    uo = jj * 32 + hv * 8
                    ko = 512 + (i - jj) * 32 + hv * 8
                    ur = spec[base, uo:uo + 8, :]
                    ui = spec[base, uo + 16:uo + 24, :]
                    kr = spec[base, ko:ko + 8, :]
                    ki = spec[base, ko + 16:ko + 24, :]
                    tr, ti = _tie(ur * kr - ui * ki, gate), _tie(ur * ki + ui * kr, gate)
                    yr, yi = (tr, ti) if yr is None else (yr + tr, yi + ti)
                    if jj < i or hv == 0:
                        gate = yield
                ys.append((yr, yi))
            (ar, ai), (br, bi) = ys
            if prev is not None:
                ar, ai, br, bi = ar - prev[0][1], ai + prev[0][0], br + prev[1][1], bi - prev[1][0]
            prev = ys
            zspec[pl.ds(zbase + i * CB, 8), :] = _pack(jnp.concatenate([ar + br, ai - bi], axis=0))
            zspec[pl.ds(zbase + (i * CB + CB // 2), 8), :] = _pack(jnp.concatenate([ar - br, ai + bi], axis=0))
            gate = yield

    def conv_inv(t, j):
        tr = t if isinstance(t, int) else jnp.maximum(t, 0)
        slot = t & 1
        ys = []
        for i in range(2):
            z = zspec[pl.ds(_mo((slot * NB + 2 * j + i) * CB, CB), CB), :]
            ys.append([_dot(pltpu.bitcast(inv_ref[h], BF16),
                            pltpu.bitcast(z[h * (CB // 2):(h + 1) * (CB // 2)], BF16)) for h in range(2)])
        gate = yield
        dsk = small[pl.ds(tr, 1), :]
        r0 = _mo(j * 2 * CB, 2 * CB)
        for m in range(2 * CB // 16):
            i, o = m % 2, (m // 2) * 16
            rows = pl.ds(r0 + (i * CB + o), 16)
            sg, part = j * (2 * CB // SEG) + (i * CB + o) // SEG, slice(o % SEG, o % SEG + 16)
            kv, q, g, old = [_even_odd(v) for v in (vs[t + 1, rows, :], xs[tr, rows, :], gbuf[sg, part, :],
                                                    outb[t + 1, sg, part, :])]
            res = []
            for h in range(2):
                y = _tie(ys[i][h][o // 2:o // 2 + 8], gate)
                y = old[h] + g[h] * (q[h] * (y + kv[h] * dsk))
                res.append(pltpu.bitcast(y.astype(BF16).astype(F32), U32))
            outb[t + 1, sg, part, :] = pltpu.bitcast((res[0] >> 16) | (res[1] & jnp.uint32(0xFFFF0000)), BF16)
            gate = yield

    state = {}

    def last_extra(e, y):
        for i, q in enumerate(range(128 * e // 84, 128 * (e + 1) // 84)):
            if q % 16 == 0:
                state["prep"] = conv_prep(0, q // 16)
                next(state["prep"])
            if q % 16 == 5 and q >= 16:
                conv_fwd(0, q // 16 - 1)
            gate = _gate(y[16 * i:16 * i + 8], _zero_of(count))
            state["prep"].send(gate)
            mix_gate(q * 16, gate)
    strassen_chunk(11, _zero_of(count), last_extra, range(1, 4), last=True)
    conv_fwd(0, NB // 2 - 1)

    ri = jax.lax.broadcasted_iota(I32, (NR, NR), 0)
    ci = jax.lax.broadcasted_iota(I32, (NR, NR), 1)
    LD = MEM + XR

    def head_pos(i):
        tail = i >= 2 * LD
        return (jnp.where(tail, (i - 2 * LD) // TL, i // LD),
                jnp.where(tail, LD + (i - 2 * LD) % TL, i % LD))
    (rh, rp), (ch, cp_) = head_pos(ri), head_pos(ci)
    same = rh == ch
    keep = same & ((rp < MEM) | (rp >= cp_))
    fbuf[0, 0:NR, 0:NR] = jnp.where(keep, 0.0, jnp.where(same, -1000000000.0 * float(DH) ** 0.5, -jnp.inf)).astype(F32)
    scale = float(DH) ** -0.5

    def step(it, u, zero):
        end = u is None
        if end:
            s, it, u = it, jax.lax.shift_right_logical(it, 1), it & 1
            xr0 = pl.multiple_of(s * SEG, SEG)
        else:
            s = it * 2 + u
            xr0 = pl.multiple_of(it * (2 * SEG), 2 * SEG) + u * SEG
        ct = jax.lax.shift_right_logical(s, 3)
        cj = jnp.bitwise_and(s, 7)
        h_lhs = jnp.concatenate(
            [jnp.concatenate([mem[:, c * 128:(c + 1) * 128], xs[c, pl.ds(xr0, XR), :].astype(F32)],
                             axis=0).astype(BF16) for c in range(NC)], axis=1)

        macs = conv_mac(ct, cj, zero)
        next(macs)
        preps = conv_prep(ct + 1, cj)
        if not end:
            next(preps)
        n_mac = NB * (NB + 1)

        def wo_sums():
            npair, kq = s >> 4, (s >> 3) & 1
            gate = yield
            for i in range(8):
                rows = pl.ds(pl.multiple_of((s & 7) * 64, 64) + 8 * i, 8)
                sl = npair * 8 + kq
                sums = rhs_sums(wos[sl, rows, :], wos[sl + 4, rows, :], wos[sl + 2, rows, :], wos[sl + 6, rows, :], gate)
                for k, val in enumerate(sums):
                    wosum[npair * 10 + kq + 2 * k, rows, :] = val
                gate = yield

        def tail_sums():
            rows = pl.ds(pl.multiple_of(it * TL, TL), TL)
            gate = yield
            for hh in range(H // 2):
                a11, a22 = _tie(otail[hh], gate), _tie(otail[H + H // 2 + hh], gate)
                a12, a21 = otail[H // 2 + hh], otail[H + hh]
                for k, val in enumerate((a11 + a12, a21 + a22, a11, a22, a11 + a22, a12 - a22, a21 - a11)):
                    obuf[k * (H // 2) + hh, rows, :] = val.astype(BF16)
                gate = yield

        wsums = wo_sums()
        next(wsums)
        queue = ([(preps, 1)] * (0 if end else 16)
                 + [(macs, min(MAC_G, n_mac - n)) for n in range(0, n_mac, MAC_G)] + [(wsums, 1)] * 8)

        def side_work(token):
            if queue:
                gen, cnt = queue.pop(0)
                if gen is None:
                    return
                gen.send(_gate(token, zero))
                for _ in range(cnt - 1):
                    gen.send(None)

        def proj(p):
            for t in range(3):
                for i, hh in enumerate((2 * p, 2 * p + 1)):
                    y = _dot(h_lhs, pltpu.bitcast(wts[(hh // 8) * 24 + t * 8 + hh % 8], BF16))
                    side_work(y[0:8])
                    ybufs[p // 4][t * 4 + p % 4 + zero, i * 16:(i + 1) * 16, :] = pltpu.bitcast(y.astype(BF16), U32)

        def rows_of(t, p):
            o = ((p // 4) * 12 + t * 4 + p % 4) * 8
            return pltpu.bitcast(jnp.concatenate([ybufs[p // 4][t * 4 + p % 4], prebuf[s, o:o + 8, :]], axis=0), BF16)

        def scores(p):
            sc = _dot_nt(rows_of(0, p), rows_of(1, p))
            fill = fbuf[zero * (p + 1), 0:NR, 0:NR]
            sc = jnp.where(fill == 0.0, sc, fill)
            e = jnp.exp2((sc - jnp.max(sc, axis=1, keepdims=True)) * (scale * 1.4426950408889634))
            l = jnp.sum(e, axis=1, keepdims=True)
            r = pl.reciprocal(l, approx=True)
            ebuf[p + zero, 0:NR // 2, :] = pltpu.bitcast(e.astype(BF16), U32)
            return r * (2.0 - l * r)

        olhs = [None] * H

        def values(p, r):
            o = _dot(pltpu.bitcast(ebuf[p, 0:NR // 2, :], BF16), rows_of(2, p)) * r
            for i, hh in enumerate((2 * p, 2 * p + 1)):
                olhs[hh] = pltpu.bitcast(o[i * LD:(i + 1) * LD].astype(BF16), U32)
                otail[u * H + hh + zero] = o[2 * LD + i * TL:2 * LD + (i + 1) * TL].astype(BF16).astype(F32)

        def oproj(g):
            lhs = pltpu.bitcast(jnp.concatenate([olhs[hh] for hh in range(4 * g, 4 * g + 4)], axis=1), BF16)
            for n in range(NC):
                w = wos[4 * n + g // 2, (g % 2) * 256:(g % 2 + 1) * 256, :]
                y = _dot(lhs, pltpu.bitcast(w, BF16))
                side_work(y[0:8])
                if g > 0:
                    y = y + oacc[n + zero]
                if g < H // 4 - 1:
                    oacc[n] = y
                else:
                    mem[:, n * 128:(n + 1) * 128] = y[0:MEM].astype(BF16).astype(F32)
                    accumulate(n + 1, s, slice(0, XR),
                               (1.0 - gbuf[s, 0:XR, :].astype(F32)) * y[MEM:].astype(BF16).astype(F32))

        recip = [None] * (H // 2)
        for op, arg in PROGRAM_END if end else PROGRAM:
            if op == "P":
                proj(arg)
            elif op == "S":
                recip[arg] = scores(arg)
            elif op == "V":
                values(arg, recip[arg])
                if (end or u == 1) and arg == H // 2 - 1:
                    assert not queue
                    tsums = tail_sums()
                    next(tsums)
                    queue.extend([(None, 0)] * 4 + [(tsums, 1)] * (H // 2))
            elif op == "O":
                oproj(arg)
            elif op == "I":
                invs = conv_inv(ct - 1, cj)
                next(invs)
                if end:
                    queue.extend([(invs, 1)] * 16)
            else:
                assert not queue
                res = conv_fwd(ct + 1, cj)
                for m in range(16):
                    o = (4 + m * 26 // 16) * 8
                    invs.send(_gate(res[o:o + 8], zero))

    def two_steps(it, carry):
        for u in range(2):
            step(it, u, _zero_of(carry))

        @pl.when(it == 3)
        def _():
            for c in range(2, NC):
                for cp in conv_copies(c):
                    cp.wait()
        return carry + 1

    def end_step(s, carry):
        step(s, None, _zero_of(carry))
        return carry + 1

    for cp in conv_copies(1):
        cp.wait()
    for c in range(2, NC):
        for cp in conv_copies(c):
            cp.start()
    jax.lax.fori_loop(0, (NSEG - NEND) // 2, two_steps, count)
    jax.lax.fori_loop(NSEG - NEND, NSEG, end_step, count)

    def out_copy(c, s0, n, r0, nr):
        return pltpu.make_async_copy(outb.at[c + 1, pl.ds(s0, n), pl.ds(r0, nr), :],
                                     out_hbm.at[pl.ds(s0, n), pl.ds(r0, nr), pl.ds(c * 128, 128)], sems.at[4])

    def head_copies():
        return [out_copy(c, 0, NSEG, 0, XR) for c in range(NC - 1)]

    def tail_copies(i):
        return [out_copy(c, i * 16, 16, XR, TL) for c in range(NC - 1)] + [out_copy(NC - 1, i * 16, 16, 0, SEG)]

    for cp in head_copies():
        cp.start()

    def post_chunk(i, carry):
        rows = pl.ds(pl.multiple_of(i * 64, 64), 64)

        def finish(n, par, y):
            for j in range(8):
                sg = i * 16 + (2 * j + par)
                accumulate(n + 1, sg, slice(XR, SEG),
                           (1.0 - gbuf[sg, XR:SEG, :].astype(F32)) * y[8 * j:8 * j + 8].astype(BF16).astype(F32))

        copies = tail_copies(i)
        for npair in (0, 3, 1, 2):
            if npair == 3:
                invs = [conv_inv(NC - 1, 2 * i + jj) for jj in range(2)]
                for gen in invs:
                    next(gen)
            ms = []
            for k in range(7):
                a = jnp.concatenate([obuf[k * (H // 2) + hh, rows, :] for hh in range(H // 2)], axis=1)
                if k == 0:
                    b = [wos[npair * 8 + 6], wos[npair * 8 + 7]]
                elif k == 1:
                    b = [wos[npair * 8], wos[npair * 8 + 1]]
                else:
                    b = [wosum[npair * 10 + 2 * (k - 2)], wosum[npair * 10 + 2 * (k - 2) + 1]]
                ms.append(_dot(a, pltpu.bitcast(jnp.concatenate(b, axis=0), BF16)))
                if npair == 3 and k < 4:
                    for m in range(8):
                        invs[k // 2].send(_gate(ms[k][8 * m:8 * m + 8], _zero_of(carry)))
                if k == 2:
                    finish(2 * npair + 1, 0, ms[0] + ms[2])
                if k == 3:
                    finish(2 * npair, 1, ms[1] + ms[3])
                if k == 5:
                    finish(2 * npair, 0, ((ms[3] - ms[0]) + ms[4]) + ms[5])
                if k == 6:
                    finish(2 * npair + 1, 1, ((ms[2] - ms[1]) + ms[4]) + ms[6])
            copies[2 * npair].start()
            copies[2 * npair + 1].start()
        return carry + 1
    jax.lax.fori_loop(0, PRE // MB, post_chunk, 0)
    for cp in head_copies():
        cp.wait()
    for i in range(PRE // MB):
        for cp in tail_copies(i):
            cp.wait()


@functools.partial(jax.jit, static_argnames=("B_seg_len",))
def pallas_gated_mix__ssm_conv_h3__memory_aug_recurrent_mem_tr__prompt_kernel(
    A_q, A_k, A_v, A_shift_k, A_ssm_k, A_ssm_D, B_x, B_mem0, B_Wq, B_Wk, B_Wv, B_Wo,
    B_seg_len, gate_w,
):
    del B_x
    assert B_seg_len == SEG and A_q.shape == (1, S, D) and B_Wq.shape == (D, H, DH)
    assert A_shift_k.shape == (D, KS) and B_mem0.shape == (1, MEM, D)
    fwd, inv = _dft_tables()
    hbm = pl.BlockSpec(memory_space=pl.ANY)
    out = pl.pallas_call(
        _kernel,
        out_shape=jax.ShapeDtypeStruct((NSEG, SEG, D), BF16),
        in_specs=[hbm] * 15,
        out_specs=hbm,
        scratch_shapes=[
            pltpu.VMEM((NC, S, 128), BF16),
            pltpu.VMEM((NC, NSEG, TL, 128), BF16),
            pltpu.VMEM((28, PRE // 4, 128), U32),
            pltpu.VMEM((10, D // 4, 128), U32),
            pltpu.VMEM((NC, 64 + S, 128), BF16),
            pltpu.VMEM((NC + 1, S, 128), BF16),
            pltpu.VMEM((NC, 128, S), BF16),
            pltpu.VMEM((3, D, 8, 128), BF16),
            pltpu.VMEM((3 * H, D // 2, 128), U32),
            pltpu.VMEM((4 * NC + 4, D // 2, 128), U32),
            pltpu.VMEM((5 * NC, D // 2, 128), U32),
            pltpu.VMEM((2 * H, TL, 128), F32),
            pltpu.VMEM((NC + 1, H * DH, 128), BF16),
            pltpu.VMEM((NSEG, 3 * H // 2 * 8, 128), U32),
            pltpu.VMEM((12, 32, 128), U32),
            pltpu.VMEM((12, 32, 128), U32),
            pltpu.VMEM((12, 32, 128), U32),
            pltpu.VMEM((12, 32, 128), U32),
            pltpu.VMEM((7 * H // 2, PRE // 2, 128), BF16),
            pltpu.VMEM((NC + 1, NSEG, SEG, 128), BF16),
            pltpu.VMEM((NC, MEM + XR, 128), F32),
            pltpu.VMEM((MEM, D), F32),
            pltpu.VMEM((96, 128), F32),
            pltpu.VMEM((2, 96, 128), U32),
            pltpu.VMEM((1, 96, 128), F32),
            pltpu.VMEM((H // 2, 64, NR), U32),
            pltpu.VMEM((16, 1024, 128), F32),
            pltpu.VMEM((2 * NB * CB, 128), U32),
            pltpu.VMEM((NSEG, SEG, 128), BF16),
            pltpu.VMEM((CB, CB), U32),
            pltpu.VMEM((2, CB // 4, CB), U32),
            pltpu.VMEM((MEM, D), BF16),
            pltpu.VMEM((NC, KS, 128), BF16),
            pltpu.VMEM((NC, 128), BF16),
            pltpu.VMEM((NC, 128), BF16),
            pltpu.SemaphoreType.DMA((11,)),
            pltpu.SemaphoreType.DMA((3,)),
            pltpu.SemaphoreType.DMA((NC,)),
        ],
        compiler_params=pltpu.CompilerParams(vmem_limit_bytes=120 * 1024 * 1024, disable_bounds_checks=True, disable_semaphore_checks=True),
    )(
        A_q.reshape(S, D), A_q.reshape(NSEG, SEG, D), A_k.reshape(S, D), A_v.reshape(S, D), A_ssm_k,
        B_Wq, B_Wk, B_Wv, B_Wo.reshape(H * DH, D),
        A_shift_k.T.reshape(KS, NC, 128).transpose(1, 0, 2),
        A_ssm_D.reshape(NC, 128), gate_w.reshape(NC, 128),
        B_mem0.reshape(MEM, D),
        jnp.asarray(fwd), jnp.asarray(inv),
    )
    return out.reshape(1, S, D)
```
